```python
import jax
import jax.numpy as jnp

def _softmax(x, axis=-1):
    return jax.nn.softmax(x, axis=axis)

def _gelu(x):
    return jax.nn.gelu(x, approximate=True)

def _silu(x):
    return jax.nn.silu(x)

def _sigmoid(x):
    return jax.nn.sigmoid(x)

def _layernorm(x, axis=-1, eps=1e-05):
    m = jnp.mean(x, axis=axis, keepdims=True)
    v = jnp.var(x, axis=axis, keepdims=True)
    return (x - m) / jnp.sqrt(v + eps)

def _scatter_add(tgt, idx, src, axis=0):
    return tgt.at[idx].add(src)

def _segment_sum(src, seg, n):
    return jax.ops.segment_sum(src, seg, n)

class _Rng:

    def __init__(self, key):
        self._k = key

    def _next(self):
        self._k, sub = jax.random.split(self._k)
        return sub

    def normal(self, shape):
        return jax.random.normal(self._next(), shape, dtype=jnp.bfloat16)

    def randint(self, lo, hi, shape):
        return jax.random.randint(self._next(), shape, lo, hi, dtype=jnp.int32)

    def uniform(self, shape, lo=0.0, hi=1.0):
        return jax.random.uniform(self._next(), shape, jnp.bfloat16, lo, hi)

    def permutation(self, n):
        return jax.random.permutation(self._next(), n)
kernel_name = 'interleave_layers__memory_aug_recurrent_mem_tr__sliding_local_dilated__prompt'

def setup_inputs():
    _rng = _Rng(jax.random.key(int.from_bytes(__import__("os").urandom(4), "little")))
    _w = lambda a: (lambda t: t.astype(jnp.bfloat16) if jnp.issubdtype(t.dtype, jnp.floating) else t)(jnp.asarray(a))

    def _A_setup():
        B, S, Dm = (1, 2048, 640)
        H, Dh = (32, 192)
        M, seg = (8, 32)
        seg = min(seg, S)
        S = S // seg * seg
        return {'x': _w((lambda *s: _rng.normal(s) * 0.05)(B, S, Dm)), 'mem0': _w((lambda *s: _rng.normal(s) * 0.05)(B, M, Dm)), 'Wq': _w((lambda *s: _rng.normal(s) * 0.05)(Dm, H, Dh) * Dm ** (-0.5)), 'Wk': _w((lambda *s: _rng.normal(s) * 0.05)(Dm, H, Dh) * Dm ** (-0.5)), 'Wv': _w((lambda *s: _rng.normal(s) * 0.05)(Dm, H, Dh) * Dm ** (-0.5)), 'Wo': _w((lambda *s: _rng.normal(s) * 0.05)(H, Dh, Dm) * (H * Dh) ** (-0.5)), 'seg_len': seg}
    _A_in = _A_setup()

    def _B_setup():
        B, S, D = (1, 2048, 640)
        return {'x': _w((lambda *s: _rng.normal(s) * 0.05)(B, S, D)), 'wqkv': _w((lambda *s: _rng.normal(s) * 0.05)(D, 3 * D)), 'wo': _w((lambda *s: _rng.normal(s) * 0.05)(D, D))}
    _B_in = _B_setup()
    return {'A_x': _A_in['x'], 'A_mem0': _A_in['mem0'], 'A_Wq': _A_in['Wq'], 'A_Wk': _A_in['Wk'], 'A_Wv': _A_in['Wv'], 'A_Wo': _A_in['Wo'], 'A_seg_len': _A_in['seg_len'], 'B_x': _B_in['x'], 'B_wqkv': _B_in['wqkv'], 'B_wo': _B_in['wo']}

def reference(A_x, A_mem0, A_Wq, A_Wk, A_Wv, A_Wo, A_seg_len, B_x, B_wqkv, B_wo):

    def _A_ref(x, mem0, Wq, Wk, Wv, Wo, seg_len):
        B, S, Dm = x.shape
        H, Dh = (Wq.shape[1], Wq.shape[2])
        M = mem0.shape[1]
        scale = Dh ** (-0.5)
        n_seg = S // seg_len
        L = M + seg_len
        idx = jnp.arange(L)
        mask = (idx[:, None] < M) | (idx[:, None] >= idx[None, :])
        mem = mem0
        outs = []
        for s in range(n_seg):
            xs = x[:, s * seg_len:(s + 1) * seg_len, :].copy()
            h = jnp.concatenate([mem, xs], axis=1)
            q = jnp.einsum('btd,dhe->bhte', h, Wq)
            k = jnp.einsum('btd,dhe->bhte', h, Wk)
            v = jnp.einsum('btd,dhe->bhte', h, Wv)
            scores = jnp.einsum('bhqe,bhke->bhqk', q, k) * scale
            scores = jnp.where(mask[None, None], scores, -1000000000.0)
            p = _softmax(scores, axis=-1)
            o = jnp.einsum('bhqk,bhke->bhqe', p, v)
            o = jnp.einsum('bhte,hed->btd', o, Wo)
            mem = o[:, :M, :].copy()
            outs.append(o[:, M:, :])
        return jnp.concatenate(outs, axis=1)

    def _B_ref(x, wqkv, wo):
        B, S, D = x.shape
        H = 32
        Dh = D // H
        W, dil = (8, 2)
        qkv = (lambda x, *d: x.transpose(*d))((x @ wqkv).reshape(B, S, 3, H, Dh), 2, 0, 3, 1, 4)
        q, k, v = (qkv[0], qkv[1], qkv[2])
        scale = Dh ** (-0.5)
        pos = jnp.arange(S)
        off = jnp.arange(W) * dil
        idx = pos[:, None] - off[None, :]
        mask = idx >= 0
        idx_c = jnp.where(mask, idx, 0).reshape(-1)
        kg = k[:, :, idx_c, :].reshape(B, H, S, W, Dh)
        vg = v[:, :, idx_c, :].reshape(B, H, S, W, Dh)
        logits = jnp.einsum('bhsd,bhswd->bhsw', q, kg) * scale
        logits = jnp.where(mask[None, None, :, :], logits, -1000000000.0)
        attn = _softmax(logits, axis=-1)
        o = jnp.einsum('bhsw,bhswd->bhsd', attn, vg)
        return (lambda x, *d: x.transpose(*d))(o, 0, 2, 1, 3).reshape(B, S, D) @ wo
    x = A_x
    x = x + _A_ref(_layernorm(x, axis=-1), A_mem0, A_Wq, A_Wk, A_Wv, A_Wo, A_seg_len)
    x = x + _B_ref(_layernorm(x, axis=-1), B_wqkv, B_wo)
    x = x + _A_ref(_layernorm(x, axis=-1), A_mem0, A_Wq, A_Wk, A_Wv, A_Wo, A_seg_len)
    x = x + _B_ref(_layernorm(x, axis=-1), B_wqkv, B_wo)
    return x
```

```python
import functools

import jax
import jax.numpy as jnp
import jax.experimental.pallas as pl
import jax.experimental.pallas.tpu as pltpu

f32 = jnp.float32
bf16 = jnp.bfloat16
u32 = jnp.uint32

DM = 640
NH = 32
DH = 192
NP = NH // 2
PW = 2 * DH
MEM = 8
SEG = 32
LL = MEM + SEG
BDH = DM // NH
BW, BDIL = 8, 2
LOG2E = 1.4426950408889634
EPS = 1e-5
NEG = -1e30


def _ln(x):
    m = jnp.mean(x, axis=-1, keepdims=True)
    d = x - m
    v = jnp.mean(d * d, axis=-1, keepdims=True)
    return d * jax.lax.rsqrt(v + EPS)


def _kernel(x_hbm, mem0_ref, wq_hbm, wk_hbm, wv_hbm, wo_hbm, bqkv_hbm, bwo_hbm,
            out_hbm,
            xst, wst, bst, bwo_st,
            wqkv, wo, bw, bwo, xres, hx, mem, obuf, kbuf, vbuf, outv,
            sems, out_sem, *, nseg):
    def cp_x():
        return pltpu.make_async_copy(x_hbm, xst, sems.at[0])

    def cp_b():
        return pltpu.make_async_copy(bqkv_hbm, bst, sems.at[1])

    def cp_bo():
        return pltpu.make_async_copy(bwo_hbm, bwo_st, sems.at[2])

    def cp_w(g, slot):
        return [pltpu.make_async_copy(w.at[pl.ds(g * PW, PW), :], wst.at[slot, j], sems.at[3 + slot * 3 + j])
                for j, w in enumerate((wq_hbm, wk_hbm, wv_hbm))]

    def cp_wo():
        return pltpu.make_async_copy(wo_hbm, wo, sems.at[12])

    cp_x().start()
    cp_b().start()
    cp_bo().start()
    for c in cp_w(0, 0):
        c.start()
    for c in cp_w(1, 1):
        c.start()

    cp_x().wait()

    def ln_body(i, c):
        r = pl.ds(pl.multiple_of(i * 64, 64), 64)
        xv = xst[r, :].astype(f32)
        xres[r, :] = xv
        hx[r, :] = _ln(xv)
        return c
    jax.lax.fori_loop(0, nseg * SEG // 64, ln_body, 0)
    zseg = jnp.zeros((SEG, DM), f32)
    xres[pl.ds(nseg * SEG, SEG), :] = zseg
    mem[...] = mem0_ref[...].astype(f32)
    kbuf[...] = jnp.zeros(kbuf.shape, f32)
    vbuf[...] = jnp.zeros(vbuf.shape, f32)

    cp_b().wait()
    cp_bo().wait()
    r_i = jax.lax.broadcasted_iota(jnp.int32, (DM, DM), 0)
    c_i = jax.lax.broadcasted_iota(jnp.int32, (DM, DM), 1)
    perm = (r_i == BDH * (c_i & (NH - 1)) + (c_i >> 5)).astype(bf16)
    perm_t = (c_i == BDH * (r_i & (NH - 1)) + (r_i >> 5)).astype(bf16)
    for j in range(3):
        t = jnp.dot(bst[:, j * DM:(j + 1) * DM], perm, preferred_element_type=f32)
        bw[:, j * DM:(j + 1) * DM] = pltpu.bitcast(t.astype(bf16), u32)
    t = jnp.dot(perm_t, bwo_st[...], preferred_element_type=f32)
    bwo[...] = pltpu.bitcast(t.astype(bf16), u32)

    def w_body(g, c):
        for slot in range(3):
            @pl.when(g % 3 == slot)
            def _():
                @pl.when(g + 2 < NP)
                def _():
                    for cpy in cp_w(g + 2, (slot + 2) % 3):
                        cpy.start()

                @pl.when(g + 2 == NP)
                def _():
                    cp_wo().start()
                for j, cpy in enumerate(cp_w(g, slot)):
                    cpy.wait()
                    wqkv[g, :, j * PW:(j + 1) * PW] = pltpu.bitcast(wst[slot, j].T, u32)
        return c
    jax.lax.fori_loop(0, NP, w_body, 0)
    cp_wo().wait()

    lane = jax.lax.broadcasted_iota(jnp.int32, (LL, 128), 1)
    row = jax.lax.broadcasted_iota(jnp.int32, (LL, 128), 0)
    a_scale = DH ** -0.5 * LOG2E
    b_scale = BDH ** -0.5 * LOG2E

    def a_tick(tau):
        seg = tau & (nseg - 1)
        rows = pl.ds(pl.multiple_of(seg * SEG, SEG), SEG)
        lo = lane < 64
        first = lane < LL
        key = jnp.where(first, lane, lane - LL)
        valid = (lane < 2 * LL) & ((row < MEM) | (row >= key))
        m0 = valid & first
        m1 = valid & jnp.logical_not(first)
        z40 = jnp.zeros((LL, 128), f32)
        z48 = jnp.zeros((128 - 2 * LL, 128), f32)

        def proj(g, j):
            h = jnp.concatenate([mem[...], hx[rows, :]], axis=0)
            w = pltpu.bitcast(wqkv[g, :, j * PW:(j + 1) * PW], bf16)
            return jnp.dot(h, w, preferred_element_type=f32)

        def blk(t):
            ta, tb, tc = t[:, 0:128], t[:, 128:256], t[:, 256:384]
            a = jnp.concatenate([ta, z40, z48], 0)
            b = jnp.concatenate([jnp.where(lo, tb, 0.), jnp.where(lo, 0., tb), z48], 0)
            c = jnp.concatenate([z40, tc, z48], 0)
            return jnp.concatenate([a, b, c], 1).astype(bf16)

        def softmax(sc):
            sc = sc * a_scale
            mx0 = jnp.max(jnp.where(m0, sc, NEG), axis=1, keepdims=True)
            mx1 = jnp.max(jnp.where(m1, sc, NEG), axis=1, keepdims=True)
            p = jnp.where(valid, jnp.exp2(sc - jnp.where(first, mx0, mx1)), 0.)
            l0 = jnp.sum(jnp.where(first, p, 0.), axis=1, keepdims=True)
            l1 = jnp.sum(jnp.where(first, 0., p), axis=1, keepdims=True)
            return p * pl.reciprocal(jnp.where(first, l0, l1), approx=True)

        def pv(g, p, vmat):
            obuf[:, g * PW:(g + 1) * PW] = jnp.dot(p, vmat, preferred_element_type=f32)

        def oproj(g0, g1):
            return jnp.dot(obuf[:, g0 * PW:g1 * PW], wo[g0 * PW:g1 * PW, :], preferred_element_type=f32)

        scs, vms, ps = {}, {}, {}
        for g in range(NP):
            kmat = blk(proj(g, 1))
            q = proj(g, 0)
            vms[g] = blk(proj(g, 2))
            if g >= 1:
                ps[g - 1] = softmax(scs.pop(g - 1))
            scs[g] = jax.lax.dot_general(q, kmat, (((1,), (1,)), ((), ())), preferred_element_type=f32)
            if g >= 1:
                pv(g - 1, ps.pop(g - 1), vms.pop(g - 1))
        ps[NP - 1] = softmax(scs.pop(NP - 1))
        r1 = oproj(0, NP // 2)
        pv(NP - 1, ps.pop(NP - 1), vms.pop(NP - 1))
        res = r1 + oproj(NP // 2, NP)
        mem[...] = jnp.where(seg == nseg - 1, mem0_ref[...].astype(f32), res[0:MEM])
        xres[rows, :] = xres[rows, :] + res[MEM:LL]

    def b_tick(tau):
        j = jnp.where(tau == 0, nseg, (tau - 1) & (nseg - 1))
        rows = pl.ds(pl.multiple_of(j * SEG, SEG), SEG)
        x1 = xres[rows, :]
        hb = _ln(x1)
        qkv = jnp.dot(hb, pltpu.bitcast(bw[...], bf16), preferred_element_type=f32)
        q = qkv[:, 0:DM] * b_scale
        for c in range(5):
            kbuf[c, 0:16, :] = kbuf[c, SEG:SEG + 16, :]
            vbuf[c, 0:16, :] = vbuf[c, SEG:SEG + 16, :]
            kbuf[c, 16:16 + SEG, :] = qkv[:, DM + c * 128:DM + (c + 1) * 128]
            vbuf[c, 16:16 + SEG, :] = qkv[:, 2 * DM + c * 128:2 * DM + (c + 1) * 128]
        pos = jax.lax.broadcasted_iota(jnp.int32, (SEG, 128), 0) + (j & (nseg - 1)) * SEG
        lgs = []
        for w in range(BW):
            off = 16 - w * BDIL
            acc = q[:, 0:128] * kbuf[0, off:off + SEG, :]
            for c in range(1, 5):
                acc = acc + q[:, c * 128:(c + 1) * 128] * kbuf[c, off:off + SEG, :]
            acc = acc + pltpu.roll(acc, 64, 1)
            acc = acc + pltpu.roll(acc, 32, 1)
            if w > 0:
                acc = jnp.where(pos >= w * BDIL, acc, NEG)
            lgs.append(acc)
        mx = functools.reduce(jnp.maximum, lgs)
        es = [jnp.exp2(l - mx) for l in lgs]
        inv = pl.reciprocal(functools.reduce(jnp.add, es), approx=True)
        es = [e * inv for e in es]
        outs = []
        for c in range(5):
            acc = None
            for w in range(BW):
                off = 16 - w * BDIL
                t = es[w] * vbuf[c, off:off + SEG, :]
                acc = t if acc is None else acc + t
            outs.append(acc)
        o = jnp.concatenate(outs, axis=1)
        x2 = x1 + jnp.dot(o, pltpu.bitcast(bwo[...], bf16), preferred_element_type=f32)
        xres[rows, :] = x2
        hx[rows, :] = _ln(x2)
        outv[pl.ds(pl.multiple_of((j & (nseg - 1)) * SEG, SEG), SEG), :] = x2.astype(bf16)

    def body(tau, c):
        b_tick(tau)
        a_tick(tau)
        return c
    jax.lax.fori_loop(0, 2 * nseg, body, 0)
    b_tick(2 * nseg)
    cp = pltpu.make_async_copy(outv, out_hbm, out_sem)
    cp.start()
    cp.wait()


@functools.partial(jax.jit, static_argnames=("A_seg_len",))
def pallas_interleave_layers__memory_aug_recurrent_mem_tr__sliding_local_dilated__prompt_kernel(
    A_x, A_mem0, A_Wq, A_Wk, A_Wv, A_Wo, A_seg_len, B_x, B_wqkv, B_wo,
):
    del B_x
    B, S, Dm = A_x.shape
    assert B == 1 and Dm == DM and A_seg_len == SEG and S % SEG == 0
    nseg = S // SEG
    x = A_x.reshape(S, DM)
    mem0 = A_mem0.reshape(MEM, DM)
    wt = lambda w: jnp.transpose(w, (1, 2, 0)).reshape(NH * DH, DM)
    any_spec = pl.BlockSpec(memory_space=pl.ANY)
    out = pl.pallas_call(
        functools.partial(_kernel, nseg=nseg),
        out_shape=jax.ShapeDtypeStruct((S, DM), A_x.dtype),
        in_specs=[any_spec, pl.BlockSpec(memory_space=pltpu.VMEM)] + [any_spec] * 6,
        out_specs=any_spec,
        scratch_shapes=[
            pltpu.VMEM((S, DM), bf16),
            pltpu.VMEM((3, 3, PW, DM), bf16),
            pltpu.VMEM((DM, 3 * DM), bf16),
            pltpu.VMEM((DM, DM), bf16),
            pltpu.VMEM((NP, DM // 2, 3 * PW), u32),
            pltpu.VMEM((NH * DH, DM), bf16),
            pltpu.VMEM((DM // 2, 3 * DM), u32),
            pltpu.VMEM((DM // 2, DM), u32),
            pltpu.VMEM((S + SEG, DM), f32),
            pltpu.VMEM((S + SEG, DM), f32),
            pltpu.VMEM((MEM, DM), f32),
            pltpu.VMEM((LL, NH * DH), f32),
            pltpu.VMEM((5, 16 + SEG, 128), f32),
            pltpu.VMEM((5, 16 + SEG, 128), f32),
            pltpu.VMEM((S, DM), bf16),
            pltpu.SemaphoreType.DMA((13,)),
            pltpu.SemaphoreType.DMA(()),
        ],
        compiler_params=pltpu.CompilerParams(vmem_limit_bytes=100 * 1024 * 1024),
    )(x, mem0, wt(A_Wq), wt(A_Wk), wt(A_Wv), A_Wo.reshape(NH * DH, DM), B_wqkv, B_wo)
    return out.reshape(B, S, DM)
```

```python
import functools

import jax
import jax.numpy as jnp
import jax.experimental.pallas as pl
import jax.experimental.pallas.tpu as pltpu

f32 = jnp.float32
bf16 = jnp.bfloat16
u32 = jnp.uint32

DM = 640
NH = 32
DH = 192
NP = NH // 2
PW = 2 * DH
MEM = 8
SEG = 32
LL = MEM + SEG
BDH = DM // NH
BW, BDIL = 8, 2
LOG2E = 1.4426950408889634
EPS = 1e-5
NEG = -1e30


def _ln(x):
    m = jnp.mean(x, axis=-1, keepdims=True)
    d = x - m
    v = jnp.mean(d * d, axis=-1, keepdims=True)
    return d * jax.lax.rsqrt(v + EPS)


def _kernel(x_hbm, mem0_ref, wq_hbm, wk_hbm, wv_hbm, wo_hbm, bqkv_hbm, bwo_hbm,
            out_hbm,
            xst, wst, bst, bwo_st,
            wqkv, wo, bw, bwo, xres, hx, mem, obuf, kbuf, vbuf, hb, qb, lg, outv,
            sems, out_sem, *, nseg):
    def cp_x():
        return pltpu.make_async_copy(x_hbm, xst, sems.at[0])

    def cp_b():
        return pltpu.make_async_copy(bqkv_hbm, bst, sems.at[1])

    def cp_bo():
        return pltpu.make_async_copy(bwo_hbm, bwo_st, sems.at[2])

    def cp_w(g, slot):
        return [pltpu.make_async_copy(w.at[pl.ds(g * PW, PW), :], wst.at[slot, j], sems.at[3 + slot * 3 + j])
                for j, w in enumerate((wq_hbm, wk_hbm, wv_hbm))]

    def cp_wo():
        return [pltpu.make_async_copy(wo_hbm.at[:, pl.ds(c * 128, 128)], wo.at[c], sems.at[12 + c])
                for c in range(5)]

    cp_x().start()
    cp_b().start()
    cp_bo().start()
    for c in cp_w(0, 0):
        c.start()
    for c in cp_w(1, 1):
        c.start()

    cp_x().wait()

    def ln_body(i, c):
        r = pl.ds(pl.multiple_of(i * 64, 64), 64)
        xv = xst[r, :].astype(f32)
        xres[r, :] = xv
        hx[r, :] = _ln(xv)
        return c
    jax.lax.fori_loop(0, nseg * SEG // 64, ln_body, 0)
    zseg = jnp.zeros((SEG, DM), f32)
    xres[pl.ds(nseg * SEG, SEG), :] = zseg
    mem[0:MEM, :] = mem0_ref[...].astype(f32)
    kbuf[...] = jnp.zeros(kbuf.shape, f32)
    vbuf[...] = jnp.zeros(vbuf.shape, f32)

    cp_b().wait()
    cp_bo().wait()
    r_i = jax.lax.broadcasted_iota(jnp.int32, (DM, DM), 0)
    c_i = jax.lax.broadcasted_iota(jnp.int32, (DM, DM), 1)
    perm = (r_i == BDH * (c_i & (NH - 1)) + (c_i >> 5)).astype(bf16)
    perm_t = (c_i == BDH * (r_i & (NH - 1)) + (r_i >> 5)).astype(bf16)
    for j in range(3):
        t = jnp.dot(bst[:, j * DM:(j + 1) * DM], perm, preferred_element_type=f32)
        bw[:, j * DM:(j + 1) * DM] = pltpu.bitcast(t.astype(bf16), u32)
    t = jnp.dot(perm_t, bwo_st[...], preferred_element_type=f32)
    bwo[...] = pltpu.bitcast(t.astype(bf16), u32)

    def w_body(g, c):
        for slot in range(3):
            @pl.when(g % 3 == slot)
            def _():
                @pl.when(g + 2 < NP)
                def _():
                    for cpy in cp_w(g + 2, (slot + 2) % 3):
                        cpy.start()

                @pl.when(g + 2 == NP)
                def _():
                    for cpy in cp_wo():
                        cpy.start()
                for j, cpy in enumerate(cp_w(g, slot)):
                    cpy.wait()
                    wqkv[g, :, j * PW:(j + 1) * PW] = pltpu.bitcast(wst[slot, j].T, u32)
        return c
    jax.lax.fori_loop(0, NP, w_body, 0)
    for cpy in cp_wo():
        cpy.wait()

    lane = jax.lax.broadcasted_iota(jnp.int32, (LL, 128), 1)
    row = jax.lax.broadcasted_iota(jnp.int32, (LL, 128), 0)
    a_scale = DH ** -0.5 * LOG2E
    b_scale = BDH ** -0.5 * LOG2E

    def a_steps(tau):
        seg = tau & (nseg - 1)
        rows = pl.ds(pl.multiple_of(seg * SEG, SEG), SEG)
        lo = lane < 64
        first = lane < LL
        key = jnp.where(first, lane, lane - LL)
        valid = (lane < 2 * LL) & ((row < MEM) | (row >= key))
        m0 = valid & first
        m1 = valid & jnp.logical_not(first)
        z40 = jnp.zeros((LL, 128), f32)
        z48 = jnp.zeros((128 - 2 * LL, 128), f32)

        mem[MEM:LL, :] = hx[rows, :]

        def proj(g, j):
            h = mem[...]
            w = pltpu.bitcast(wqkv[g, :, j * PW:(j + 1) * PW], bf16)
            return jnp.dot(h, w, preferred_element_type=f32)

        def blk(t):
            ta, tb, tc = t[:, 0:128], t[:, 128:256], t[:, 256:384]
            a = jnp.concatenate([ta, z40, z48], 0)
            b = jnp.concatenate([jnp.where(lo, tb, 0.), jnp.where(lo, 0., tb), z48], 0)
            c = jnp.concatenate([z40, tc, z48], 0)
            return jnp.concatenate([a, b, c], 1).astype(bf16)

        def softmax(sc):
            sc = sc * a_scale
            mx0 = jnp.max(jnp.where(m0, sc, NEG), axis=1, keepdims=True)
            mx1 = jnp.max(jnp.where(m1, sc, NEG), axis=1, keepdims=True)
            p = jnp.where(valid, jnp.exp2(sc - jnp.where(first, mx0, mx1)), 0.)
            l0 = jnp.sum(jnp.where(first, p, 0.), axis=1, keepdims=True)
            l1 = jnp.sum(jnp.where(first, 0., p), axis=1, keepdims=True)
            return p * pl.reciprocal(jnp.where(first, l0, l1), approx=True)

        def pv(g, p, vmat):
            obuf[:, g * PW:(g + 1) * PW] = jnp.dot(p, vmat, preferred_element_type=f32)

        def oproj(g0, g1):
            return jnp.concatenate(
                [jnp.dot(obuf[:, g0 * PW:g1 * PW], wo[c, g0 * PW:g1 * PW, :], preferred_element_type=f32)
                 for c in range(5)], axis=1)

        scs, vms, ps = {}, {}, {}
        for g in range(NP):
            kmat = blk(proj(g, 1))
            q = proj(g, 0)
            vms[g] = blk(proj(g, 2))
            if g >= 1:
                ps[g - 1] = softmax(scs.pop(g - 1))
            scs[g] = jax.lax.dot_general(q, kmat, (((1,), (1,)), ((), ())), preferred_element_type=f32)
            if g >= 1:
                pv(g - 1, ps.pop(g - 1), vms.pop(g - 1))
            yield
        ps[NP - 1] = softmax(scs.pop(NP - 1))
        r1 = oproj(0, NP // 2)
        pv(NP - 1, ps.pop(NP - 1), vms.pop(NP - 1))
        res = r1 + oproj(NP // 2, NP)
        mem[0:MEM, :] = jnp.where(seg == nseg - 1, mem0_ref[...].astype(f32), res[0:MEM])
        xres[rows, :] = xres[rows, :] + res[MEM:LL]

    def b_steps(tau):
        j = jnp.where(tau == 0, nseg, (tau - 1) & (nseg - 1))
        rows = pl.ds(pl.multiple_of(j * SEG, SEG), SEG)

        def bproj(t):
            return jnp.dot(hb[...], pltpu.bitcast(bw[:, t * DM:(t + 1) * DM], bf16),
                           preferred_element_type=f32)

        hb[...] = _ln(xres[rows, :])
        for c in range(5):
            kbuf[c, 0:16, :] = kbuf[c, SEG:SEG + 16, :]
            vbuf[c, 0:16, :] = vbuf[c, SEG:SEG + 16, :]
        yield
        qb[...] = bproj(0) * b_scale
        yield
        k = bproj(1)
        for c in range(5):
            kbuf[c, 16:16 + SEG, :] = k[:, c * 128:(c + 1) * 128]
        yield
        v = bproj(2)
        for c in range(5):
            vbuf[c, 16:16 + SEG, :] = v[:, c * 128:(c + 1) * 128]
        yield
        pos = jax.lax.broadcasted_iota(jnp.int32, (SEG, 128), 0) + (j & (nseg - 1)) * SEG
        for w in range(BW):
            off = 16 - w * BDIL
            acc = qb[:, 0:128] * kbuf[0, off:off + SEG, :]
            for c in range(1, 5):
                acc = acc + qb[:, c * 128:(c + 1) * 128] * kbuf[c, off:off + SEG, :]
            acc = acc + pltpu.roll(acc, 64, 1)
            acc = acc + pltpu.roll(acc, 32, 1)
            if w > 0:
                acc = jnp.where(pos >= w * BDIL, acc, NEG)
            lg[w] = acc
            if w % 2 == 1:
                yield
        lgs = [lg[w] for w in range(BW)]
        mx = functools.reduce(jnp.maximum, lgs)
        es = [jnp.exp2(l - mx) for l in lgs]
        inv = pl.reciprocal(functools.reduce(jnp.add, es), approx=True)
        for w in range(BW):
            lg[w] = es[w] * inv
        yield
        for c in range(5):
            acc = None
            for w in range(BW):
                off = 16 - w * BDIL
                t = lg[w] * vbuf[c, off:off + SEG, :]
                acc = t if acc is None else acc + t
            qb[:, c * 128:(c + 1) * 128] = acc
            if c in (1, 3):
                yield
        yield
        x2 = xres[rows, :] + jnp.dot(qb[...], pltpu.bitcast(bwo[...], bf16), preferred_element_type=f32)
        xres[rows, :] = x2
        hx[rows, :] = _ln(x2)
        outv[pl.ds(pl.multiple_of((j & (nseg - 1)) * SEG, SEG), SEG), :] = x2.astype(bf16)

    def body(tau, c):
        ga, gb = a_steps(tau), b_steps(tau)
        live = [gb, ga]
        while live:
            for gen in list(live):
                try:
                    next(gen)
                except StopIteration:
                    live.remove(gen)
        return c
    jax.lax.fori_loop(0, 2 * nseg, body, 0)
    for _ in b_steps(2 * nseg):
        pass
    cp = pltpu.make_async_copy(outv, out_hbm, out_sem)
    cp.start()
    cp.wait()


@functools.partial(jax.jit, static_argnames=("A_seg_len",))
def pallas_interleave_layers__memory_aug_recurrent_mem_tr__sliding_local_dilated__prompt_kernel(
    A_x, A_mem0, A_Wq, A_Wk, A_Wv, A_Wo, A_seg_len, B_x, B_wqkv, B_wo,
):
    del B_x
    B, S, Dm = A_x.shape
    assert B == 1 and Dm == DM and A_seg_len == SEG and S % SEG == 0
    nseg = S // SEG
    x = A_x.reshape(S, DM)
    mem0 = A_mem0.reshape(MEM, DM)
    wt = lambda w: jnp.transpose(w, (1, 2, 0)).reshape(NH * DH, DM)
    any_spec = pl.BlockSpec(memory_space=pl.ANY)
    out = pl.pallas_call(
        functools.partial(_kernel, nseg=nseg),
        out_shape=jax.ShapeDtypeStruct((S, DM), A_x.dtype),
        in_specs=[any_spec, pl.BlockSpec(memory_space=pltpu.VMEM)] + [any_spec] * 6,
        out_specs=any_spec,
        scratch_shapes=[
            pltpu.VMEM((S, DM), bf16),
            pltpu.VMEM((3, 3, PW, DM), bf16),
            pltpu.VMEM((DM, 3 * DM), bf16),
            pltpu.VMEM((DM, DM), bf16),
            pltpu.VMEM((NP, DM // 2, 3 * PW), u32),
            pltpu.VMEM((5, NH * DH, 128), bf16),
            pltpu.VMEM((DM // 2, 3 * DM), u32),
            pltpu.VMEM((DM // 2, DM), u32),
            pltpu.VMEM((S + SEG, DM), f32),
            pltpu.VMEM((S + SEG, DM), f32),
            pltpu.VMEM((LL, DM), f32),
            pltpu.VMEM((LL, NH * DH), f32),
            pltpu.VMEM((5, 16 + SEG, 128), f32),
            pltpu.VMEM((5, 16 + SEG, 128), f32),
            pltpu.VMEM((SEG, DM), f32),
            pltpu.VMEM((SEG, DM), f32),
            pltpu.VMEM((BW, SEG, 128), f32),
            pltpu.VMEM((S, DM), bf16),
            pltpu.SemaphoreType.DMA((17,)),
            pltpu.SemaphoreType.DMA(()),
        ],
        compiler_params=pltpu.CompilerParams(vmem_limit_bytes=100 * 1024 * 1024),
    )(x, mem0, wt(A_Wq), wt(A_Wk), wt(A_Wv), A_Wo.reshape(NH * DH, DM), B_wqkv, B_wo)
    return out.reshape(B, S, DM)
```

```python
import functools

import jax
import jax.numpy as jnp
import jax.experimental.pallas as pl
import jax.experimental.pallas.tpu as pltpu

f32 = jnp.float32
bf16 = jnp.bfloat16
u32 = jnp.uint32

DM = 640
NH = 32
DH = 192
NP = NH // 2
PW = 2 * DH
MEM = 8
SEG = 32
LL = MEM + SEG
BDH = DM // NH
BW, BDIL = 8, 2
LOG2E = 1.4426950408889634
EPS = 1e-5
NEG = -1e30


def _ln(x):
    m = jnp.mean(x, axis=-1, keepdims=True)
    d = x - m
    v = jnp.mean(d * d, axis=-1, keepdims=True)
    return d * jax.lax.rsqrt(v + EPS)


def _kernel(x_hbm, mem0_ref, wq_hbm, wk_hbm, wv_hbm, wo_hbm, bqkv_hbm, bwo_hbm,
            out_hbm,
            xst, wst, bst, bwo_st,
            wqkv, wo, bw, bwo, xres, hx, mem, obuf, kbuf, vbuf, hb, qb, lg, outv,
            sems, out_sem, *, nseg):
    def cp_x():
        return pltpu.make_async_copy(x_hbm, xst, sems.at[0])

    def cp_b():
        return pltpu.make_async_copy(bqkv_hbm, bst, sems.at[1])

    def cp_bo():
        return pltpu.make_async_copy(bwo_hbm, bwo_st, sems.at[2])

    def cp_w(g):
        return [pltpu.make_async_copy(w.at[pl.ds(g * PW, PW), :], wst.at[g, j], sems.at[8 + g * 3 + j])
                for j, w in enumerate((wq_hbm, wk_hbm, wv_hbm))]

    def cp_wo():
        return [pltpu.make_async_copy(wo_hbm.at[:, pl.ds(c * 128, 128)], wo.at[c], sems.at[3 + c])
                for c in range(5)]

    for cpy in [cp_x(), cp_b(), cp_bo()] + [c for g in range(NP) for c in cp_w(g)] + cp_wo():
        cpy.start()

    cp_x().wait()

    def ln_body(i, c):
        r = pl.ds(pl.multiple_of(i * 64, 64), 64)
        xv = xst[r, :].astype(f32)
        xres[r, :] = xv
        hx[r, :] = _ln(xv)
        return c
    jax.lax.fori_loop(0, nseg * SEG // 64, ln_body, 0)
    zseg = jnp.zeros((SEG, DM), f32)
    xres[pl.ds(nseg * SEG, SEG), :] = zseg
    mem[0:MEM, :] = mem0_ref[...].astype(f32)
    kbuf[...] = jnp.zeros(kbuf.shape, f32)
    vbuf[...] = jnp.zeros(vbuf.shape, f32)

    cp_b().wait()
    cp_bo().wait()
    r_i = jax.lax.broadcasted_iota(jnp.int32, (DM, DM), 0)
    c_i = jax.lax.broadcasted_iota(jnp.int32, (DM, DM), 1)
    perm = (r_i == BDH * (c_i & (NH - 1)) + (c_i >> 5)).astype(bf16)
    perm_t = (c_i == BDH * (r_i & (NH - 1)) + (r_i >> 5)).astype(bf16)
    for j in range(3):
        t = jnp.dot(bst[:, j * DM:(j + 1) * DM], perm, preferred_element_type=f32)
        bw[:, j * DM:(j + 1) * DM] = pltpu.bitcast(t.astype(bf16), u32)
    t = jnp.dot(perm_t, bwo_st[...], preferred_element_type=f32)
    bwo[...] = pltpu.bitcast(t.astype(bf16), u32)

    def w_body(g, c):
        for j, w in enumerate((wq_hbm, wk_hbm, wv_hbm)):
            pltpu.make_async_copy(w.at[pl.ds(g * PW, PW), :], wst.at[g, j], sems.at[8 + g * 3 + j]).wait()
            wqkv[g, :, j * PW:(j + 1) * PW] = pltpu.bitcast(wst[g, j].T, u32)
        return c
    jax.lax.fori_loop(0, NP, w_body, 0)
    for cpy in cp_wo():
        cpy.wait()

    lane = jax.lax.broadcasted_iota(jnp.int32, (LL, 128), 1)
    row = jax.lax.broadcasted_iota(jnp.int32, (LL, 128), 0)
    a_scale = DH ** -0.5 * LOG2E
    b_scale = BDH ** -0.5 * LOG2E

    def a_steps(tau):
        seg = tau & (nseg - 1)
        rows = pl.ds(pl.multiple_of(seg * SEG, SEG), SEG)
        lo = lane < 64
        first = lane < LL
        key = jnp.where(first, lane, lane - LL)
        valid = (lane < 2 * LL) & ((row < MEM) | (row >= key))
        m0 = valid & first
        m1 = valid & jnp.logical_not(first)
        z40 = jnp.zeros((LL, 128), f32)
        z48 = jnp.zeros((128 - 2 * LL, 128), f32)

        mem[MEM:LL, :] = hx[rows, :]

        def proj(g, j):
            h = mem[...]
            w = pltpu.bitcast(wqkv[g, :, j * PW:(j + 1) * PW], bf16)
            return jnp.dot(h, w, preferred_element_type=f32)

        def blk(t):
            ta, tb, tc = t[:, 0:128], t[:, 128:256], t[:, 256:384]
            a = jnp.concatenate([ta, z40, z48], 0)
            b = jnp.concatenate([jnp.where(lo, tb, 0.), jnp.where(lo, 0., tb), z48], 0)
            c = jnp.concatenate([z40, tc, z48], 0)
            return jnp.concatenate([a, b, c], 1).astype(bf16)

        def softmax(sc):
            sc = sc * a_scale
            mx0 = jnp.max(jnp.where(m0, sc, NEG), axis=1, keepdims=True)
            mx1 = jnp.max(jnp.where(m1, sc, NEG), axis=1, keepdims=True)
            p = jnp.where(valid, jnp.exp2(sc - jnp.where(first, mx0, mx1)), 0.)
            l0 = jnp.sum(jnp.where(first, p, 0.), axis=1, keepdims=True)
            l1 = jnp.sum(jnp.where(first, 0., p), axis=1, keepdims=True)
            return p * pl.reciprocal(jnp.where(first, l0, l1), approx=True)

        def pv(g, p, vmat):
            obuf[:, g * PW:(g + 1) * PW] = jnp.dot(p, vmat, preferred_element_type=f32)

        def oproj(g0, g1):
            return jnp.concatenate(
                [jnp.dot(obuf[:, g0 * PW:g1 * PW], wo[c, g0 * PW:g1 * PW, :], preferred_element_type=f32)
                 for c in range(5)], axis=1)

        scs, vms, ps = {}, {}, {}
        for g in range(NP):
            kmat = blk(proj(g, 1))
            q = proj(g, 0)
            vms[g] = blk(proj(g, 2))
            if g >= 1:
                ps[g - 1] = softmax(scs.pop(g - 1))
            scs[g] = jax.lax.dot_general(q, kmat, (((1,), (1,)), ((), ())), preferred_element_type=f32)
            if g >= 1:
                pv(g - 1, ps.pop(g - 1), vms.pop(g - 1))
            yield
        ps[NP - 1] = softmax(scs.pop(NP - 1))
        r1 = oproj(0, NP // 2)
        pv(NP - 1, ps.pop(NP - 1), vms.pop(NP - 1))
        res = r1 + oproj(NP // 2, NP)
        mem[0:MEM, :] = jnp.where(seg == nseg - 1, mem0_ref[...].astype(f32), res[0:MEM])
        xres[rows, :] = xres[rows, :] + res[MEM:LL]

    def b_steps(tau):
        j = jnp.where(tau == 0, nseg, (tau - 1) & (nseg - 1))
        rows = pl.ds(pl.multiple_of(j * SEG, SEG), SEG)

        def bproj(t):
            return jnp.dot(hb[...], pltpu.bitcast(bw[:, t * DM:(t + 1) * DM], bf16),
                           preferred_element_type=f32)

        hb[...] = _ln(xres[rows, :])
        for c in range(5):
            kbuf[c, 0:16, :] = kbuf[c, SEG:SEG + 16, :]
            vbuf[c, 0:16, :] = vbuf[c, SEG:SEG + 16, :]
        yield
        qb[...] = bproj(0) * b_scale
        yield
        k = bproj(1)
        for c in range(5):
            kbuf[c, 16:16 + SEG, :] = k[:, c * 128:(c + 1) * 128]
        yield
        v = bproj(2)
        for c in range(5):
            vbuf[c, 16:16 + SEG, :] = v[:, c * 128:(c + 1) * 128]
        yield
        pos = jax.lax.broadcasted_iota(jnp.int32, (SEG, 128), 0) + (j & (nseg - 1)) * SEG
        for w in range(BW):
            off = 16 - w * BDIL
            acc = qb[:, 0:128] * kbuf[0, off:off + SEG, :]
            for c in range(1, 5):
                acc = acc + qb[:, c * 128:(c + 1) * 128] * kbuf[c, off:off + SEG, :]
            acc = acc + pltpu.roll(acc, 64, 1)
            acc = acc + pltpu.roll(acc, 32, 1)
            if w > 0:
                acc = jnp.where(pos >= w * BDIL, acc, NEG)
            lg[w] = acc
            if w % 2 == 1:
                yield
        lgs = [lg[w] for w in range(BW)]
        mx = functools.reduce(jnp.maximum, lgs)
        es = [jnp.exp2(l - mx) for l in lgs]
        inv = pl.reciprocal(functools.reduce(jnp.add, es), approx=True)
        for w in range(BW):
            lg[w] = es[w] * inv
        yield
        for c in range(5):
            acc = None
            for w in range(BW):
                off = 16 - w * BDIL
                t = lg[w] * vbuf[c, off:off + SEG, :]
                acc = t if acc is None else acc + t
            qb[:, c * 128:(c + 1) * 128] = acc
            if c in (1, 3):
                yield
        yield
        x2 = xres[rows, :] + jnp.dot(qb[...], pltpu.bitcast(bwo[...], bf16), preferred_element_type=f32)
        xres[rows, :] = x2
        hx[rows, :] = _ln(x2)
        outv[pl.ds(pl.multiple_of((j & (nseg - 1)) * SEG, SEG), SEG), :] = x2.astype(bf16)

    def out_copy(j):
        r = pl.ds(pl.multiple_of(j * SEG, SEG), SEG)
        return pltpu.make_async_copy(outv.at[r, :], out_hbm.at[r, :], out_sem)

    def body(tau, c):
        ga, gb = a_steps(tau), b_steps(tau)
        live = [gb, ga]
        while live:
            for gen in list(live):
                try:
                    next(gen)
                except StopIteration:
                    live.remove(gen)

        @pl.when(tau > nseg)
        def _():
            out_copy(tau - 1 - nseg).start()
        return c
    jax.lax.fori_loop(0, 2 * nseg, body, 0)
    for _ in b_steps(2 * nseg):
        pass
    out_copy(nseg - 1).start()
    pltpu.make_async_copy(outv, out_hbm, out_sem).wait()


@functools.partial(jax.jit, static_argnames=("A_seg_len",))
def pallas_interleave_layers__memory_aug_recurrent_mem_tr__sliding_local_dilated__prompt_kernel(
    A_x, A_mem0, A_Wq, A_Wk, A_Wv, A_Wo, A_seg_len, B_x, B_wqkv, B_wo,
):
    del B_x
    B, S, Dm = A_x.shape
    assert B == 1 and Dm == DM and A_seg_len == SEG and S % SEG == 0
    nseg = S // SEG
    x = A_x.reshape(S, DM)
    mem0 = A_mem0.reshape(MEM, DM)
    wt = lambda w: jnp.transpose(w, (1, 2, 0)).reshape(NH * DH, DM)
    any_spec = pl.BlockSpec(memory_space=pl.ANY)
    out = pl.pallas_call(
        functools.partial(_kernel, nseg=nseg),
        out_shape=jax.ShapeDtypeStruct((S, DM), A_x.dtype),
        in_specs=[any_spec, pl.BlockSpec(memory_space=pltpu.VMEM)] + [any_spec] * 6,
        out_specs=any_spec,
        scratch_shapes=[
            pltpu.VMEM((S, DM), bf16),
            pltpu.VMEM((NP, 3, PW, DM), bf16),
            pltpu.VMEM((DM, 3 * DM), bf16),
            pltpu.VMEM((DM, DM), bf16),
            pltpu.VMEM((NP, DM // 2, 3 * PW), u32),
            pltpu.VMEM((5, NH * DH, 128), bf16),
            pltpu.VMEM((DM // 2, 3 * DM), u32),
            pltpu.VMEM((DM // 2, DM), u32),
            pltpu.VMEM((S + SEG, DM), f32),
            pltpu.VMEM((S + SEG, DM), f32),
            pltpu.VMEM((LL, DM), f32),
            pltpu.VMEM((LL, NH * DH), f32),
            pltpu.VMEM((5, 16 + SEG, 128), f32),
            pltpu.VMEM((5, 16 + SEG, 128), f32),
            pltpu.VMEM((SEG, DM), f32),
            pltpu.VMEM((SEG, DM), f32),
            pltpu.VMEM((BW, SEG, 128), f32),
            pltpu.VMEM((S, DM), bf16),
            pltpu.SemaphoreType.DMA((8 + 3 * NP,)),
            pltpu.SemaphoreType.DMA(()),
        ],
        compiler_params=pltpu.CompilerParams(vmem_limit_bytes=100 * 1024 * 1024),
    )(x, mem0, wt(A_Wq), wt(A_Wk), wt(A_Wv), A_Wo.reshape(NH * DH, DM), B_wqkv, B_wo)
    return out.reshape(B, S, DM)
```

```python
import functools

import jax
import jax.numpy as jnp
import jax.experimental.pallas as pl
import jax.experimental.pallas.tpu as pltpu

f32 = jnp.float32
bf16 = jnp.bfloat16
u32 = jnp.uint32

DM = 640
NH = 32
DH = 192
NP = NH // 2
PW = 2 * DH
MEM = 8
SEG = 32
LL = MEM + SEG
BDH = DM // NH
BW, BDIL = 8, 2
LOG2E = 1.4426950408889634
EPS = 1e-5
NEG = -1e30
NLEAD = 35


def _ln(x):
    m = jnp.mean(x, axis=-1, keepdims=True)
    d = x - m
    v = jnp.mean(d * d, axis=-1, keepdims=True)
    return d * jax.lax.rsqrt(v + EPS)


def _kernel(x_hbm, mem0_ref, wq_hbm, wk_hbm, wv_hbm, wo_hbm, bqkv_hbm, bwo_hbm,
            out_hbm,
            xst, wst, bst, bwo_st, tq, to, wping, wpong,
            wqkv, wo, bw, bwo, xres, mem, h0, pre, obuf, kbuf, vbuf, hb, qb, lg, outv,
            sems, out_sem, *, nseg, nlead):
    def cp_x():
        return pltpu.make_async_copy(x_hbm, xst, sems.at[0])

    def cp_b():
        return pltpu.make_async_copy(bqkv_hbm, bst, sems.at[1])

    def cp_bo():
        return pltpu.make_async_copy(bwo_hbm, bwo_st, sems.at[2])

    def cp_w(g, j):
        w = (wq_hbm, wk_hbm, wv_hbm)[j]
        return pltpu.make_async_copy(w.at[pl.ds(g * PW, PW), :], wst.at[g, j], sems.at[8 + g])

    def cp_wo():
        return [pltpu.make_async_copy(wo_hbm.at[:, pl.ds(c * 128, 128)], wo.at[c], sems.at[3 + c])
                for c in range(5)]

    for cpy in ([cp_x()] + [cp_w(g, j) for g in range(NP) for j in (1, 0, 2)]
                + [cp_b(), cp_bo()] + cp_wo()):
        cpy.start()

    kbuf[...] = jnp.zeros(kbuf.shape, f32)
    vbuf[...] = jnp.zeros(vbuf.shape, f32)
    pre[NP - 1, 0:LL, :] = jnp.zeros((LL, 3 * PW), f32)
    h0[0:MEM, :] = mem0_ref[...].astype(f32)
    cp_x().wait()
    h0[MEM:LL, :] = _ln(xst[0:SEG, :].astype(f32))
    for s in range(nlead):
        xs = xst[SEG * (s + 1):SEG * (s + 1) + 16, :].astype(f32)
        h0[LL + 8 * s:LL + 8 * s + 8, :] = _ln(xs[0:8])

    def x_body(i, c):
        r = pl.ds(pl.multiple_of(i * 128, 128), 128)
        xres[r, :] = xst[r, :].astype(f32)
        return c
    jax.lax.fori_loop(0, nseg * SEG // 128, x_body, 0)

    lane = jax.lax.broadcasted_iota(jnp.int32, (LL, 128), 1)
    row = jax.lax.broadcasted_iota(jnp.int32, (LL, 128), 0)
    a_scale = DH ** -0.5 * LOG2E
    b_scale = BDH ** -0.5 * LOG2E
    lo = lane < 64
    first = lane < LL
    key = jnp.where(first, lane, lane - LL)
    valid = (lane < 2 * LL) & ((row < MEM) | (row >= key))
    m0 = valid & first
    m1 = valid & jnp.logical_not(first)

    def blk(t):
        z40 = jnp.zeros((LL, 128), f32)
        z48 = jnp.zeros((128 - 2 * LL, 128), f32)
        ta, tb, tc = t[:, 0:128], t[:, 128:256], t[:, 256:384]
        a = jnp.concatenate([ta, z40, z48], 0)
        b = jnp.concatenate([jnp.where(lo, tb, 0.), jnp.where(lo, 0., tb), z48], 0)
        c = jnp.concatenate([z40, tc, z48], 0)
        return jnp.concatenate([a, b, c], 1).astype(bf16)

    def scores(q, kmat):
        return jax.lax.dot_general(q, kmat, (((1,), (1,)), ((), ())), preferred_element_type=f32)

    def softmax(sc):
        sc = sc * a_scale
        mx0 = jnp.max(jnp.where(m0, sc, NEG), axis=1, keepdims=True)
        mx1 = jnp.max(jnp.where(m1, sc, NEG), axis=1, keepdims=True)
        p = jnp.where(valid, jnp.exp2(sc - jnp.where(first, mx0, mx1)), 0.)
        l0 = jnp.sum(jnp.where(first, p, 0.), axis=1, keepdims=True)
        l1 = jnp.sum(jnp.where(first, 0., p), axis=1, keepdims=True)
        return p * pl.reciprocal(jnp.where(first, l0, l1), approx=True)

    def pv(g, p, vmat):
        obuf[g] = jnp.dot(p, vmat, preferred_element_type=f32)

    def oproj(g0, g1):
        o = jnp.concatenate([obuf[g] for g in range(g0, g1)], axis=1)
        return jnp.concatenate(
            [jnp.dot(o, wo[c, g0 * PW:g1 * PW, :], preferred_element_type=f32) for c in range(5)], axis=1)

    def a_finish(tau, p_last, vm_last, next_mode, mid=None):
        seg = tau & (nseg - 1)
        rows = pl.ds(pl.multiple_of(seg * SEG, SEG), SEG)
        nxt = (tau + 1) & (nseg - 1)
        if next_mode == "short":
            mem[MEM:SEG, :] = _ln(xres[pl.ds(pl.multiple_of(nxt * SEG + 8, 8), SEG - 8), :])
        else:
            mem[MEM:LL, :] = _ln(xres[pl.ds(pl.multiple_of(nxt * SEG, SEG), SEG), :])
        r1 = oproj(0, NP // 2)
        if mid is not None:
            mid()
        pv(NP - 1, p_last, vm_last)
        res = r1 + oproj(NP // 2, NP)
        mem[0:MEM, :] = jnp.where(seg == nseg - 1, mem0_ref[...].astype(f32), res[0:MEM])
        xres[rows, :] = xres[rows, :] + res[MEM:LL]

    def a_steps(tau, mode, next_mode):
        if mode == "short":
            prow = pl.ds(pl.multiple_of(LL + (tau - 1) * 8, 8), 8)

        def proj(g, j):
            cols = slice(j * PW, (j + 1) * PW)
            w = pltpu.bitcast(wqkv[g, :, cols], bf16)
            if mode == "short":
                y = jnp.dot(mem[0:SEG, :], w, preferred_element_type=f32)
                return jnp.concatenate([y[0:MEM], pre[g, prow, cols], y[MEM:SEG]], axis=0)
            return jnp.dot(mem[...], w, preferred_element_type=f32)

        scs, vms, ps = {}, {}, {}
        for g in range(NP):
            kmat = blk(proj(g, 1))
            q = proj(g, 0)
            vms[g] = blk(proj(g, 2))
            if g >= 1:
                ps[g - 1] = softmax(scs.pop(g - 1))
            scs[g] = scores(q, kmat)
            if g >= 1:
                pv(g - 1, ps.pop(g - 1), vms.pop(g - 1))
            yield
        a_finish(tau, softmax(scs.pop(NP - 1)), vms.pop(NP - 1), next_mode)

    def b_steps(tau):
        j = (tau - 1) & (nseg - 1)
        rows = pl.ds(pl.multiple_of(j * SEG, SEG), SEG)

        def bproj(t):
            return jnp.dot(hb[...], pltpu.bitcast(bw[:, t * DM:(t + 1) * DM], bf16),
                           preferred_element_type=f32)

        hb[...] = _ln(xres[rows, :])
        for c in range(5):
            kbuf[c, 0:16, :] = kbuf[c, SEG:SEG + 16, :]
            vbuf[c, 0:16, :] = vbuf[c, SEG:SEG + 16, :]
        yield
        qb[...] = bproj(0) * b_scale
        yield
        k = bproj(1)
        for c in range(5):
            kbuf[c, 16:16 + SEG, :] = k[:, c * 128:(c + 1) * 128]
        yield
        v = bproj(2)
        for c in range(5):
            vbuf[c, 16:16 + SEG, :] = v[:, c * 128:(c + 1) * 128]
        yield
        pos = jax.lax.broadcasted_iota(jnp.int32, (SEG, 128), 0) + j * SEG
        for w in range(BW):
            off = 16 - w * BDIL
            acc = qb[:, 0:128] * kbuf[0, off:off + SEG, :]
            for c in range(1, 5):
                acc = acc + qb[:, c * 128:(c + 1) * 128] * kbuf[c, off:off + SEG, :]
            acc = acc + pltpu.roll(acc, 64, 1)
            acc = acc + pltpu.roll(acc, 32, 1)
            if w > 0:
                acc = jnp.where(pos >= w * BDIL, acc, NEG)
            lg[w] = acc
            if w % 2 == 1:
                yield
        lgs = [lg[w] for w in range(BW)]
        mx = functools.reduce(jnp.maximum, lgs)
        es = [jnp.exp2(l - mx) for l in lgs]
        inv = pl.reciprocal(functools.reduce(jnp.add, es), approx=True)
        for w in range(BW):
            lg[w] = es[w] * inv
        yield
        for c in range(5):
            acc = None
            for w in range(BW):
                off = 16 - w * BDIL
                t = lg[w] * vbuf[c, off:off + SEG, :]
                acc = t if acc is None else acc + t
            qb[:, c * 128:(c + 1) * 128] = acc
            if c in (1, 3):
                yield
        yield
        x2 = xres[rows, :] + jnp.dot(qb[...], pltpu.bitcast(bwo[...], bf16), preferred_element_type=f32)
        xres[rows, :] = x2
        outv[rows, :] = x2.astype(bf16)

    def out_copy(j, n):
        r = pl.ds(pl.multiple_of(j * SEG, SEG), n * SEG)
        return pltpu.make_async_copy(outv.at[r, :], out_hbm.at[r, :], out_sem)

    def tick(tau, mode, next_mode):
        live = [b_steps(tau), a_steps(tau, mode, next_mode)]
        while live:
            for gen in list(live):
                try:
                    next(gen)
                except StopIteration:
                    live.remove(gen)

    def w_wait(g):
        pltpu.make_async_copy(wst.at[g], wst.at[g], sems.at[8 + g]).wait()

    def stage(g, dst):
        for j in range(3):
            dst[:, j * PW:(j + 1) * PW] = pltpu.bitcast(wst[g, j].T, u32)

    def first_att(g):
        q, k, v = (pre[g, 0:LL, j * PW:(j + 1) * PW] for j in range(3))
        return softmax(scores(q, blk(k))), blk(v)

    def first_pair(g, cur, nxt):
        p, vm = first_att((g + NP - 1) & (NP - 1))
        pv((g + NP - 1) & (NP - 1), p, vm)
        stage(jnp.minimum(g + 1, NP - 1), nxt)
        for j in (1, 0, 2):
            cols = slice(j * PW, (j + 1) * PW)
            w = cur[:, cols]
            wqkv[g, :, cols] = w
            pre[g, :, cols] = jnp.dot(h0[...], pltpu.bitcast(w, bf16), preferred_element_type=f32)

    w_wait(0)
    stage(0, wping)

    def first_body(i, c):
        w_wait(2 * i + 1)
        first_pair(2 * i, wping, wpong)

        @pl.when(2 * i + 2 < NP)
        def _():
            w_wait(2 * i + 2)
        first_pair(2 * i + 1, wpong, wping)
        return c
    jax.lax.fori_loop(0, NP // 2, first_body, 0)
    p_last, vm_last = first_att(NP - 1)

    def b_weights():
        for ft in range(3 * DM // 128):
            w = pltpu.bitcast(bst[:, ft * 128:(ft + 1) * 128], u32)
            for kc in range(3):
                t = w[kc * 128:(kc + 1) * 128, :]
                if kc == 2:
                    t = jnp.concatenate([t, jnp.zeros((64, 128), u32)], 0)
                tq[kc, ft * 128:(ft + 1) * 128, :] = t.T
        for j in range(3):
            for t in range(5):
                for kc in range(3):
                    rows = [tq[kc, pl.ds(j * DM + 4 * t + dd, NH, stride=BDH), :] for dd in range(4)]
                    gt = jnp.concatenate(rows, 0).T
                    n = 128 if kc < 2 else 64
                    bw[kc * 128:kc * 128 + n, j * DM + t * 128:j * DM + (t + 1) * 128] = gt[0:n]
        for c5 in range(5):
            to[c5] = bwo_st[:, c5 * 128:(c5 + 1) * 128].astype(f32)
        for c5 in range(5):
            for t in range(5):
                rows = [to[c5, pl.ds(4 * t + dd, NH, stride=BDH), :] for dd in range(4)]
                gt = jnp.concatenate(rows, 0).astype(bf16)
                bwo[t * 64:(t + 1) * 64, c5 * 128:(c5 + 1) * 128] = pltpu.bitcast(gt, u32)

    cp_b().wait()
    cp_bo().wait()
    for cpy in cp_wo():
        cpy.wait()
    a_finish(0, p_last, vm_last, "short", mid=b_weights)

    def short_body(tau, c):
        tick(tau, "short", "short")
        return c
    jax.lax.fori_loop(1, nlead, short_body, 0)
    tick(nlead, "short", "normal")

    def body(t2, c):
        tau = nlead + 1 + 2 * t2
        tick(tau, "normal", "normal")
        tick(tau + 1, "normal", "normal")

        @pl.when(tau > nseg)
        def _():
            out_copy(tau - nseg - 2, 2).start()
        return c
    assert (2 * nseg - nlead - 1) % 2 == 0 and 0 < nlead < nseg
    jax.lax.fori_loop(0, (2 * nseg - nlead - 1) // 2, body, 0)
    for _ in b_steps(2 * nseg):
        pass
    out_copy(nseg - 2, 2).start()
    pltpu.make_async_copy(outv, out_hbm, out_sem).wait()


@functools.partial(jax.jit, static_argnames=("A_seg_len",))
def pallas_interleave_layers__memory_aug_recurrent_mem_tr__sliding_local_dilated__prompt_kernel(
    A_x, A_mem0, A_Wq, A_Wk, A_Wv, A_Wo, A_seg_len, B_x, B_wqkv, B_wo,
):
    del B_x
    B, S, Dm = A_x.shape
    assert B == 1 and Dm == DM and A_seg_len == SEG and S % SEG == 0
    nseg = S // SEG
    x = A_x.reshape(S, DM)
    mem0 = A_mem0.reshape(MEM, DM)
    wt = lambda w: jnp.transpose(w, (1, 2, 0)).reshape(NH * DH, DM)
    any_spec = pl.BlockSpec(memory_space=pl.ANY)
    out = pl.pallas_call(
        functools.partial(_kernel, nseg=nseg, nlead=NLEAD),
        out_shape=jax.ShapeDtypeStruct((S, DM), A_x.dtype),
        in_specs=[any_spec, pl.BlockSpec(memory_space=pltpu.VMEM)] + [any_spec] * 6,
        out_specs=any_spec,
        scratch_shapes=[
            pltpu.VMEM((S, DM), bf16),
            pltpu.VMEM((NP, 3, PW, DM), bf16),
            pltpu.VMEM((DM, 3 * DM), bf16),
            pltpu.VMEM((DM, DM), bf16),
            pltpu.VMEM((3, 3 * DM, 128), u32),
            pltpu.VMEM((5, DM, 128), f32),
            pltpu.VMEM((DM // 2, 3 * PW), u32),
            pltpu.VMEM((DM // 2, 3 * PW), u32),
            pltpu.VMEM((NP, DM // 2, 3 * PW), u32),
            pltpu.VMEM((5, NH * DH, 128), bf16),
            pltpu.VMEM((DM // 2, 3 * DM), u32),
            pltpu.VMEM((DM // 2, DM), u32),
            pltpu.VMEM((S, DM), f32),
            pltpu.VMEM((LL, DM), f32),
            pltpu.VMEM((LL + 8 * NLEAD, DM), f32),
            pltpu.VMEM((NP, LL + 8 * NLEAD, 3 * PW), f32),
            pltpu.VMEM((NP, LL, PW), f32),
            pltpu.VMEM((5, 16 + SEG, 128), f32),
            pltpu.VMEM((5, 16 + SEG, 128), f32),
            pltpu.VMEM((SEG, DM), f32),
            pltpu.VMEM((SEG, DM), f32),
            pltpu.VMEM((BW, SEG, 128), f32),
            pltpu.VMEM((S, DM), bf16),
            pltpu.SemaphoreType.DMA((8 + NP,)),
            pltpu.SemaphoreType.DMA(()),
        ],
        compiler_params=pltpu.CompilerParams(vmem_limit_bytes=116 * 1024 * 1024),
    )(x, mem0, wt(A_Wq), wt(A_Wk), wt(A_Wv), A_Wo.reshape(NH * DH, DM), B_wqkv, B_wo)
    return out.reshape(B, S, DM)
```

```python
import functools

import jax
import jax.numpy as jnp
import jax.experimental.pallas as pl
import jax.experimental.pallas.tpu as pltpu

f32 = jnp.float32
bf16 = jnp.bfloat16
u32 = jnp.uint32

DM = 640
NH = 32
DH = 192
NP = NH // 2
PW = 2 * DH
MEM = 8
SEG = 32
LL = MEM + SEG
BDH = DM // NH
BW, BDIL = 8, 2
LOG2E = 1.4426950408889634
EPS = 1e-5
NEG = -1e30
NLEAD = 35


def _ln(x):
    m = jnp.mean(x, axis=-1, keepdims=True)
    d = x - m
    v = jnp.mean(d * d, axis=-1, keepdims=True)
    return d * jax.lax.rsqrt(v + EPS)


def _kernel(x_hbm, mem0_ref, wq_hbm, wk_hbm, wv_hbm, wo_hbm, bqkv_hbm, bwo_hbm,
            out_hbm,
            xst, wst, bst, bwo_st, tq, to, wping, wpong,
            wqkv, wo, bw, bwo, xres, mem, h0, pre, obuf, kbuf, vbuf, hb, qb, lg, outv,
            sems, out_sem, *, nseg, nlead):
    def cp_x():
        return pltpu.make_async_copy(x_hbm, xst, sems.at[0])

    def cp_b():
        return pltpu.make_async_copy(bqkv_hbm, bst, sems.at[1])

    def cp_bo():
        return pltpu.make_async_copy(bwo_hbm, bwo_st, sems.at[2])

    def cp_w(g, j):
        w = (wq_hbm, wk_hbm, wv_hbm)[j]
        return pltpu.make_async_copy(w.at[pl.ds(g * PW, PW), :], wst.at[g, j], sems.at[8 + g])

    def cp_wo():
        return [pltpu.make_async_copy(wo_hbm.at[:, pl.ds(c * 128, 128)], wo.at[c], sems.at[3 + c])
                for c in range(5)]

    for cpy in ([cp_x()] + [cp_w(g, j) for g in range(NP) for j in (1, 0, 2)]
                + [cp_b(), cp_bo()] + cp_wo()):
        cpy.start()

    kbuf[...] = jnp.zeros(kbuf.shape, f32)
    vbuf[...] = jnp.zeros(vbuf.shape, f32)
    pre[NP - 1, 0:LL, :] = jnp.zeros((LL, 3 * PW), f32)
    h0[0:MEM, :] = mem0_ref[...].astype(f32)
    cp_x().wait()
    h0[MEM:LL, :] = _ln(xst[0:SEG, :].astype(f32))
    for s in range(nlead):
        xs = xst[SEG * (s + 1):SEG * (s + 1) + 16, :].astype(f32)
        h0[LL + 8 * s:LL + 8 * s + 8, :] = _ln(xs[0:8])

    def x_body(i, c):
        r = pl.ds(pl.multiple_of(i * 128, 128), 128)
        xres[r, :] = xst[r, :].astype(f32)
        return c
    jax.lax.fori_loop(0, nseg * SEG // 128, x_body, 0)

    lane = jax.lax.broadcasted_iota(jnp.int32, (LL, 128), 1)
    row = jax.lax.broadcasted_iota(jnp.int32, (LL, 128), 0)
    a_scale = DH ** -0.5 * LOG2E
    b_scale = BDH ** -0.5 * LOG2E
    lo = lane < 64
    first = lane < LL
    key = jnp.where(first, lane, lane - LL)
    valid = (lane < 2 * LL) & ((row < MEM) | (row >= key))
    m0 = valid & first
    m1 = valid & jnp.logical_not(first)

    def blk(t):
        z40 = jnp.zeros((LL, 128), f32)
        z48 = jnp.zeros((128 - 2 * LL, 128), f32)
        ta, tb, tc = t[:, 0:128], t[:, 128:256], t[:, 256:384]
        a = jnp.concatenate([ta, z40, z48], 0)
        b = jnp.concatenate([jnp.where(lo, tb, 0.), jnp.where(lo, 0., tb), z48], 0)
        c = jnp.concatenate([z40, tc, z48], 0)
        return jnp.concatenate([a, b, c], 1).astype(bf16)

    def scores(q, kmat):
        return jax.lax.dot_general(q, kmat, (((1,), (1,)), ((), ())), preferred_element_type=f32)

    def softmax(sc):
        sc = sc * a_scale
        mx0 = jnp.max(jnp.where(m0, sc, NEG), axis=1, keepdims=True)
        mx1 = jnp.max(jnp.where(m1, sc, NEG), axis=1, keepdims=True)
        p = jnp.where(valid, jnp.exp2(sc - jnp.where(first, mx0, mx1)), 0.)
        l0 = jnp.sum(jnp.where(first, p, 0.), axis=1, keepdims=True)
        l1 = jnp.sum(jnp.where(first, 0., p), axis=1, keepdims=True)
        return p * pl.reciprocal(jnp.where(first, l0, l1), approx=True)

    def pv(g, p, vmat):
        obuf[g] = jnp.dot(p, vmat, preferred_element_type=f32)

    def oproj(g0, g1):
        o = jnp.concatenate([obuf[g] for g in range(g0, g1)], axis=1)
        return jnp.concatenate(
            [jnp.dot(o, wo[c, g0 * PW:g1 * PW, :], preferred_element_type=f32) for c in range(5)], axis=1)

    def a_finish(tau, p_last, vm_last, next_mode, mid=None):
        seg = tau & (nseg - 1)
        rows = pl.ds(pl.multiple_of(seg * SEG, SEG), SEG)
        nxt = (tau + 1) & (nseg - 1)
        if next_mode == "short":
            mem[MEM:SEG, :] = _ln(xres[pl.ds(pl.multiple_of(nxt * SEG + 8, 8), SEG - 8), :])
        else:
            mem[MEM:LL, :] = _ln(xres[pl.ds(pl.multiple_of(nxt * SEG, SEG), SEG), :])
        r1 = oproj(0, NP // 2)
        if mid is not None:
            mid()
        pv(NP - 1, p_last, vm_last)
        res = r1 + oproj(NP // 2, NP)
        mem[0:MEM, :] = jnp.where(seg == nseg - 1, mem0_ref[...].astype(f32), res[0:MEM])
        xres[rows, :] = xres[rows, :] + res[MEM:LL]

    def a_steps(tau, mode, next_mode):
        if mode == "short":
            prow = pl.ds(pl.multiple_of(LL + (tau - 1) * 8, 8), 8)

        def proj(g, j):
            cols = slice(j * PW, (j + 1) * PW)
            w = pltpu.bitcast(wqkv[g, :, cols], bf16)
            if mode == "short":
                y = jnp.dot(mem[0:SEG, :], w, preferred_element_type=f32)
                return jnp.concatenate([y[0:MEM], pre[g, prow, cols], y[MEM:SEG]], axis=0)
            return jnp.dot(mem[...], w, preferred_element_type=f32)

        scs, vms, ps = {}, {}, {}
        for g in range(NP):
            kmat = blk(proj(g, 1))
            q = proj(g, 0)
            vms[g] = blk(proj(g, 2))
            if g >= 1:
                ps[g - 1] = softmax(scs.pop(g - 1))
            scs[g] = scores(q, kmat)
            if g >= 1:
                pv(g - 1, ps.pop(g - 1), vms.pop(g - 1))
            yield
        a_finish(tau, softmax(scs.pop(NP - 1)), vms.pop(NP - 1), next_mode)

    def b_steps(tau):
        j = (tau - 1) & (nseg - 1)
        rows = pl.ds(pl.multiple_of(j * SEG, SEG), SEG)

        def bproj(t):
            return jnp.dot(hb[...], pltpu.bitcast(bw[:, t * DM:(t + 1) * DM], bf16),
                           preferred_element_type=f32)

        hb[...] = _ln(xres[rows, :])
        for c in range(5):
            kbuf[c, 0:16, :] = kbuf[c, SEG:SEG + 16, :]
            vbuf[c, 0:16, :] = vbuf[c, SEG:SEG + 16, :]
        yield
        qb[...] = bproj(0) * b_scale
        yield
        k = bproj(1)
        for c in range(5):
            kbuf[c, 16:16 + SEG, :] = k[:, c * 128:(c + 1) * 128]
        yield
        v = bproj(2)
        for c in range(5):
            vbuf[c, 16:16 + SEG, :] = v[:, c * 128:(c + 1) * 128]
        yield
        pos = jax.lax.broadcasted_iota(jnp.int32, (SEG, 128), 0) + j * SEG
        for w in range(BW):
            off = 16 - w * BDIL
            acc = qb[:, 0:128] * kbuf[0, off:off + SEG, :]
            for c in range(1, 5):
                acc = acc + qb[:, c * 128:(c + 1) * 128] * kbuf[c, off:off + SEG, :]
            acc = acc + pltpu.roll(acc, 64, 1)
            acc = acc + pltpu.roll(acc, 32, 1)
            if w > 0:
                acc = jnp.where(pos >= w * BDIL, acc, NEG)
            lg[w] = acc
            if w % 2 == 1:
                yield
        lgs = [lg[w] for w in range(BW)]
        mx = functools.reduce(jnp.maximum, lgs)
        es = [jnp.exp2(l - mx) for l in lgs]
        inv = pl.reciprocal(functools.reduce(jnp.add, es), approx=True)
        for w in range(BW):
            lg[w] = es[w] * inv
        yield
        for c in range(5):
            acc = None
            for w in range(BW):
                off = 16 - w * BDIL
                t = lg[w] * vbuf[c, off:off + SEG, :]
                acc = t if acc is None else acc + t
            qb[:, c * 128:(c + 1) * 128] = acc
            if c in (1, 3):
                yield
        yield
        x2 = xres[rows, :] + jnp.dot(qb[...], pltpu.bitcast(bwo[...], bf16), preferred_element_type=f32)
        xres[rows, :] = x2
        outv[rows, :] = x2.astype(bf16)

    def out_copy(j, n):
        r = pl.ds(pl.multiple_of(j * SEG, SEG), n * SEG)
        return pltpu.make_async_copy(outv.at[r, :], out_hbm.at[r, :], out_sem)

    def tick(tau, mode, next_mode):
        live = [b_steps(tau), a_steps(tau, mode, next_mode)]
        while live:
            for gen in list(live):
                try:
                    next(gen)
                except StopIteration:
                    live.remove(gen)

    def w_wait(g):
        pltpu.make_async_copy(wst.at[g], wst.at[g], sems.at[8 + g]).wait()

    def stage(g, dst, t):
        j, r = divmod(t, 3)
        dst[:, t * 128:(t + 1) * 128] = pltpu.bitcast(wst[g, j, r * 128:(r + 1) * 128, :].T, u32)

    def first_att(g):
        q, k, v = (pre[g, 0:LL, j * PW:(j + 1) * PW] for j in range(3))
        return softmax(scores(q, blk(k))), blk(v)

    def first_pair(g, cur, nxt):
        gp = (g + NP - 1) & (NP - 1)
        gn = jnp.minimum(g + 1, NP - 1)
        for t in range(9):
            if t == 0:
                sc = scores(pre[gp, 0:LL, 0:PW], blk(pre[gp, 0:LL, PW:2 * PW]))
            cols = slice(t * 128, (t + 1) * 128)
            w = cur[:, cols]
            wqkv[g, :, cols] = w
            pre[g, :, cols] = jnp.dot(h0[...], pltpu.bitcast(w, bf16), preferred_element_type=f32)
            stage(gn, nxt, t)
            if t == 2:
                p = softmax(sc)
            if t == 4:
                pv(gp, p, blk(pre[gp, 0:LL, 2 * PW:3 * PW]))

    w_wait(0)
    for t in range(9):
        stage(0, wping, t)

    def first_body(i, c):
        w_wait(2 * i + 1)
        first_pair(2 * i, wping, wpong)

        @pl.when(2 * i + 2 < NP)
        def _():
            w_wait(2 * i + 2)
        first_pair(2 * i + 1, wpong, wping)
        return c
    jax.lax.fori_loop(0, NP // 2, first_body, 0)
    p_last, vm_last = first_att(NP - 1)

    def b_weights():
        for ft in range(3 * DM // 128):
            w = pltpu.bitcast(bst[:, ft * 128:(ft + 1) * 128], u32)
            for kc in range(3):
                t = w[kc * 128:(kc + 1) * 128, :]
                if kc == 2:
                    t = jnp.concatenate([t, jnp.zeros((64, 128), u32)], 0)
                tq[kc, ft * 128:(ft + 1) * 128, :] = t.T
        for j in range(3):
            for t in range(5):
                for kc in range(3):
                    rows = [tq[kc, pl.ds(j * DM + 4 * t + dd, NH, stride=BDH), :] for dd in range(4)]
                    gt = jnp.concatenate(rows, 0).T
                    n = 128 if kc < 2 else 64
                    bw[kc * 128:kc * 128 + n, j * DM + t * 128:j * DM + (t + 1) * 128] = gt[0:n]
        for c5 in range(5):
            to[c5] = bwo_st[:, c5 * 128:(c5 + 1) * 128].astype(f32)
        for c5 in range(5):
            for t in range(5):
                rows = [to[c5, pl.ds(4 * t + dd, NH, stride=BDH), :] for dd in range(4)]
                gt = jnp.concatenate(rows, 0).astype(bf16)
                bwo[t * 64:(t + 1) * 64, c5 * 128:(c5 + 1) * 128] = pltpu.bitcast(gt, u32)

    cp_b().wait()
    cp_bo().wait()
    for cpy in cp_wo():
        cpy.wait()
    a_finish(0, p_last, vm_last, "short", mid=b_weights)

    def short_body(tau, c):
        tick(tau, "short", "short")
        return c
    jax.lax.fori_loop(1, nlead, short_body, 0)
    tick(nlead, "short", "normal")

    def body(t2, c):
        tau = nlead + 1 + 2 * t2
        tick(tau, "normal", "normal")
        tick(tau + 1, "normal", "normal")

        @pl.when(tau > nseg)
        def _():
            out_copy(tau - nseg - 2, 2).start()
        return c
    assert (2 * nseg - nlead - 1) % 2 == 0 and 0 < nlead < nseg
    jax.lax.fori_loop(0, (2 * nseg - nlead - 1) // 2, body, 0)
    for _ in b_steps(2 * nseg):
        pass
    out_copy(nseg - 2, 2).start()
    pltpu.make_async_copy(outv, out_hbm, out_sem).wait()


@functools.partial(jax.jit, static_argnames=("A_seg_len",))
def pallas_interleave_layers__memory_aug_recurrent_mem_tr__sliding_local_dilated__prompt_kernel(
    A_x, A_mem0, A_Wq, A_Wk, A_Wv, A_Wo, A_seg_len, B_x, B_wqkv, B_wo,
):
    del B_x
    B, S, Dm = A_x.shape
    assert B == 1 and Dm == DM and A_seg_len == SEG and S % SEG == 0
    nseg = S // SEG
    x = A_x.reshape(S, DM)
    mem0 = A_mem0.reshape(MEM, DM)
    wt = lambda w: jnp.transpose(w, (1, 2, 0)).reshape(NH * DH, DM)
    any_spec = pl.BlockSpec(memory_space=pl.ANY)
    out = pl.pallas_call(
        functools.partial(_kernel, nseg=nseg, nlead=NLEAD),
        out_shape=jax.ShapeDtypeStruct((S, DM), A_x.dtype),
        in_specs=[any_spec, pl.BlockSpec(memory_space=pltpu.VMEM)] + [any_spec] * 6,
        out_specs=any_spec,
        scratch_shapes=[
            pltpu.VMEM((S, DM), bf16),
            pltpu.VMEM((NP, 3, PW, DM), bf16),
            pltpu.VMEM((DM, 3 * DM), bf16),
            pltpu.VMEM((DM, DM), bf16),
            pltpu.VMEM((3, 3 * DM, 128), u32),
            pltpu.VMEM((5, DM, 128), f32),
            pltpu.VMEM((DM // 2, 3 * PW), u32),
            pltpu.VMEM((DM // 2, 3 * PW), u32),
            pltpu.VMEM((NP, DM // 2, 3 * PW), u32),
            pltpu.VMEM((5, NH * DH, 128), bf16),
            pltpu.VMEM((DM // 2, 3 * DM), u32),
            pltpu.VMEM((DM // 2, DM), u32),
            pltpu.VMEM((S, DM), f32),
            pltpu.VMEM((LL, DM), f32),
            pltpu.VMEM((LL + 8 * NLEAD, DM), f32),
            pltpu.VMEM((NP, LL + 8 * NLEAD, 3 * PW), f32),
            pltpu.VMEM((NP, LL, PW), f32),
            pltpu.VMEM((5, 16 + SEG, 128), f32),
            pltpu.VMEM((5, 16 + SEG, 128), f32),
            pltpu.VMEM((SEG, DM), f32),
            pltpu.VMEM((SEG, DM), f32),
            pltpu.VMEM((BW, SEG, 128), f32),
            pltpu.VMEM((S, DM), bf16),
            pltpu.SemaphoreType.DMA((8 + NP,)),
            pltpu.SemaphoreType.DMA(()),
        ],
        compiler_params=pltpu.CompilerParams(vmem_limit_bytes=116 * 1024 * 1024),
    )(x, mem0, wt(A_Wq), wt(A_Wk), wt(A_Wv), A_Wo.reshape(NH * DH, DM), B_wqkv, B_wo)
    return out.reshape(B, S, DM)
```

```python
import functools

import jax
import jax.numpy as jnp
import jax.experimental.pallas as pl
import jax.experimental.pallas.tpu as pltpu

f32 = jnp.float32
bf16 = jnp.bfloat16
u32 = jnp.uint32

DM = 640
NH = 32
DH = 192
NP = NH // 2
PW = 2 * DH
MEM = 8
SEG = 32
LL = MEM + SEG
BDH = DM // NH
BW, BDIL = 8, 2
LOG2E = 1.4426950408889634
EPS = 1e-5
NEG = -1e30
NLEAD = 35


def _ln(x):
    m = jnp.mean(x, axis=-1, keepdims=True)
    d = x - m
    v = jnp.mean(d * d, axis=-1, keepdims=True)
    return d * jax.lax.rsqrt(v + EPS)


def _kernel(x_hbm, mem0_hbm, wq_hbm, wk_hbm, wv_hbm, wo_hbm, bqkv_hbm, bwo_hbm,
            out_hbm,
            xst, mem0_ref, wst, bst, bwo_st, tq, to, wping, wpong,
            wqkv, wo, bw, bwo, xres, mem, h0, pre, obuf, kbuf, vbuf, hb, qb, lg, outv,
            sems, out_sem, *, nseg, nlead):
    nx = (nlead + 1) * SEG

    def cp_mem0():
        return pltpu.make_async_copy(mem0_hbm, mem0_ref, sems.at[0])

    def cp_x(part):
        r = pl.ds(0, nx) if part == 0 else pl.ds(nx, nseg * SEG - nx)
        return pltpu.make_async_copy(x_hbm.at[r, :], xst.at[r, :], sems.at[8 + NP + part])

    def cp_b():
        return pltpu.make_async_copy(bqkv_hbm, bst, sems.at[1])

    def cp_bo():
        return pltpu.make_async_copy(bwo_hbm, bwo_st, sems.at[2])

    def cp_w(g, j):
        w = (wq_hbm, wk_hbm, wv_hbm)[j]
        return pltpu.make_async_copy(w.at[pl.ds(g * PW, PW), :], wst.at[g, j], sems.at[8 + g])

    def cp_wo():
        return [pltpu.make_async_copy(wo_hbm.at[:, pl.ds(c * 128, 128)], wo.at[c], sems.at[3 + c])
                for c in range(5)]

    for cpy in ([cp_x(0), cp_mem0()] + [cp_w(g, j) for g in range(NP) for j in (1, 0, 2)]
                + [cp_b(), cp_bo()] + cp_wo() + [cp_x(1)]):
        cpy.start()

    kbuf[...] = jnp.zeros(kbuf.shape, f32)
    vbuf[...] = jnp.zeros(vbuf.shape, f32)
    pre[NP - 1, 0:LL, :] = jnp.zeros((LL, 3 * PW), f32)
    cp_x(0).wait()
    cp_mem0().wait()
    h0[0:MEM, :] = mem0_ref[...].astype(f32)
    h0[MEM:LL, :] = _ln(xst[0:SEG, :].astype(f32))
    for s in range(nlead):
        xs = xst[SEG * (s + 1):SEG * (s + 1) + 16, :].astype(f32)
        h0[LL + 8 * s:LL + 8 * s + 8, :] = _ln(xs[0:8])

    def x_init(s):
        r = pl.ds(pl.multiple_of(s * SEG, SEG), SEG)
        xres[r, :] = xst[r, :].astype(f32)

    def x_body(i, c):
        for u in range(4):
            x_init(4 * i + u)
        return c
    assert (nlead + 1) % 4 == 0
    jax.lax.fori_loop(0, (nlead + 1) // 4, x_body, 0)

    lane = jax.lax.broadcasted_iota(jnp.int32, (LL, 128), 1)
    row = jax.lax.broadcasted_iota(jnp.int32, (LL, 128), 0)
    a_scale = DH ** -0.5 * LOG2E
    b_scale = BDH ** -0.5 * LOG2E
    lo = lane < 64
    first = lane < LL
    key = jnp.where(first, lane, lane - LL)
    valid = (lane < 2 * LL) & ((row < MEM) | (row >= key))
    m0 = valid & first
    m1 = valid & jnp.logical_not(first)

    def blk(t):
        z40 = jnp.zeros((LL, 128), f32)
        z48 = jnp.zeros((128 - 2 * LL, 128), f32)
        ta, tb, tc = t[:, 0:128], t[:, 128:256], t[:, 256:384]
        a = jnp.concatenate([ta, z40, z48], 0)
        b = jnp.concatenate([jnp.where(lo, tb, 0.), jnp.where(lo, 0., tb), z48], 0)
        c = jnp.concatenate([z40, tc, z48], 0)
        return jnp.concatenate([a, b, c], 1).astype(bf16)

    def scores(q, kmat):
        return jax.lax.dot_general(q, kmat, (((1,), (1,)), ((), ())), preferred_element_type=f32)

    def softmax(sc):
        sc = sc * a_scale
        mx0 = jnp.max(jnp.where(m0, sc, NEG), axis=1, keepdims=True)
        mx1 = jnp.max(jnp.where(m1, sc, NEG), axis=1, keepdims=True)
        p = jnp.where(valid, jnp.exp2(sc - jnp.where(first, mx0, mx1)), 0.)
        l0 = jnp.sum(jnp.where(first, p, 0.), axis=1, keepdims=True)
        l1 = jnp.sum(jnp.where(first, 0., p), axis=1, keepdims=True)
        return p * pl.reciprocal(jnp.where(first, l0, l1), approx=True)

    def pv(g, p, vmat):
        obuf[g] = jnp.dot(p, vmat, preferred_element_type=f32)

    def oproj(g0, g1):
        o = jnp.concatenate([obuf[g] for g in range(g0, g1)], axis=1)
        return jnp.concatenate(
            [jnp.dot(o, wo[c, g0 * PW:g1 * PW, :], preferred_element_type=f32) for c in range(5)], axis=1)

    def a_finish(tau, p_last, vm_last, next_mode, mid=None):
        seg = tau & (nseg - 1)
        rows = pl.ds(pl.multiple_of(seg * SEG, SEG), SEG)
        nxt = (tau + 1) & (nseg - 1)
        if next_mode == "short":
            mem[MEM:SEG, :] = _ln(xres[pl.ds(pl.multiple_of(nxt * SEG + 8, 8), SEG - 8), :])
        else:
            mem[MEM:LL, :] = _ln(xres[pl.ds(pl.multiple_of(nxt * SEG, SEG), SEG), :])
        r1 = oproj(0, NP // 2)
        if mid is not None:
            mid()
        pv(NP - 1, p_last, vm_last)
        res = r1 + oproj(NP // 2, NP)
        mem[0:MEM, :] = jnp.where(seg == nseg - 1, mem0_ref[...].astype(f32), res[0:MEM])
        xres[rows, :] = xres[rows, :] + res[MEM:LL]

    def a_steps(tau, mode, next_mode):
        if mode == "short":
            prow = pl.ds(pl.multiple_of(LL + (tau - 1) * 8, 8), 8)

        def proj(g, j):
            cols = slice(j * PW, (j + 1) * PW)
            w = pltpu.bitcast(wqkv[g, :, cols], bf16)
            if mode == "short":
                y = jnp.dot(mem[0:SEG, :], w, preferred_element_type=f32)
                return jnp.concatenate([y[0:MEM], pre[g, prow, cols], y[MEM:SEG]], axis=0)
            return jnp.dot(mem[...], w, preferred_element_type=f32)

        scs, vms, ps = {}, {}, {}
        for g in range(NP):
            kmat = blk(proj(g, 1))
            q = proj(g, 0)
            vms[g] = blk(proj(g, 2))
            if g >= 1:
                ps[g - 1] = softmax(scs.pop(g - 1))
            scs[g] = scores(q, kmat)
            if g >= 1:
                pv(g - 1, ps.pop(g - 1), vms.pop(g - 1))
            yield
        a_finish(tau, softmax(scs.pop(NP - 1)), vms.pop(NP - 1), next_mode)

    def b_steps(tau):
        j = (tau - 1) & (nseg - 1)
        rows = pl.ds(pl.multiple_of(j * SEG, SEG), SEG)

        def bproj(t):
            return jnp.dot(hb[...], pltpu.bitcast(bw[:, t * DM:(t + 1) * DM], bf16),
                           preferred_element_type=f32)

        hb[...] = _ln(xres[rows, :])
        for c in range(5):
            kbuf[c, 0:16, :] = kbuf[c, SEG:SEG + 16, :]
            vbuf[c, 0:16, :] = vbuf[c, SEG:SEG + 16, :]
        yield
        qb[...] = bproj(0) * b_scale
        yield
        k = bproj(1)
        for c in range(5):
            kbuf[c, 16:16 + SEG, :] = k[:, c * 128:(c + 1) * 128]
        yield
        v = bproj(2)
        for c in range(5):
            vbuf[c, 16:16 + SEG, :] = v[:, c * 128:(c + 1) * 128]
        yield
        pos = jax.lax.broadcasted_iota(jnp.int32, (SEG, 128), 0) + j * SEG
        for w in range(BW):
            off = 16 - w * BDIL
            acc = qb[:, 0:128] * kbuf[0, off:off + SEG, :]
            for c in range(1, 5):
                acc = acc + qb[:, c * 128:(c + 1) * 128] * kbuf[c, off:off + SEG, :]
            acc = acc + pltpu.roll(acc, 64, 1)
            acc = acc + pltpu.roll(acc, 32, 1)
            if w > 0:
                acc = jnp.where(pos >= w * BDIL, acc, NEG)
            lg[w] = acc
            if w % 2 == 1:
                yield
        lgs = [lg[w] for w in range(BW)]
        mx = functools.reduce(jnp.maximum, lgs)
        es = [jnp.exp2(l - mx) for l in lgs]
        inv = pl.reciprocal(functools.reduce(jnp.add, es), approx=True)
        for w in range(BW):
            lg[w] = es[w] * inv
        yield
        for c in range(5):
            acc = None
            for w in range(BW):
                off = 16 - w * BDIL
                t = lg[w] * vbuf[c, off:off + SEG, :]
                acc = t if acc is None else acc + t
            qb[:, c * 128:(c + 1) * 128] = acc
            if c in (1, 3):
                yield
        yield
        x2 = xres[rows, :] + jnp.dot(qb[...], pltpu.bitcast(bwo[...], bf16), preferred_element_type=f32)
        xres[rows, :] = x2
        outv[rows, :] = x2.astype(bf16)

    def out_copy(j, n):
        r = pl.ds(pl.multiple_of(j * SEG, SEG), n * SEG)
        return pltpu.make_async_copy(outv.at[r, :], out_hbm.at[r, :], out_sem)

    def tick(tau, mode, next_mode):
        live = [b_steps(tau), a_steps(tau, mode, next_mode)]
        while live:
            for gen in list(live):
                try:
                    next(gen)
                except StopIteration:
                    live.remove(gen)

    def w_wait(g):
        pltpu.make_async_copy(wst.at[g], wst.at[g], sems.at[8 + g]).wait()

    def stage(g, dst, t):
        j, r = divmod(t, 3)
        dst[:, t * 128:(t + 1) * 128] = pltpu.bitcast(wst[g, j, r * 128:(r + 1) * 128, :].T, u32)

    def first_att(g):
        q, k, v = (pre[g, 0:LL, j * PW:(j + 1) * PW] for j in range(3))
        return softmax(scores(q, blk(k))), blk(v)

    def first_pair(g, cur, nxt):
        gp = (g + NP - 1) & (NP - 1)
        gn = jnp.minimum(g + 1, NP - 1)
        for t in range(9):
            if t == 0:
                sc = scores(pre[gp, 0:LL, 0:PW], blk(pre[gp, 0:LL, PW:2 * PW]))
            cols = slice(t * 128, (t + 1) * 128)
            w = cur[:, cols]
            wqkv[g, :, cols] = w
            pre[g, :, cols] = jnp.dot(h0[...], pltpu.bitcast(w, bf16), preferred_element_type=f32)
            stage(gn, nxt, t)
            if t == 2:
                p = softmax(sc)
            if t == 4:
                pv(gp, p, blk(pre[gp, 0:LL, 2 * PW:3 * PW]))

    w_wait(0)
    for t in range(9):
        stage(0, wping, t)

    def first_body(i, c):
        w_wait(2 * i + 1)
        first_pair(2 * i, wping, wpong)

        @pl.when(2 * i + 2 < NP)
        def _():
            w_wait(2 * i + 2)
        first_pair(2 * i + 1, wpong, wping)
        return c
    jax.lax.fori_loop(0, NP // 2, first_body, 0)
    p_last, vm_last = first_att(NP - 1)

    def b_weights():
        for ft in range(3 * DM // 128):
            w = pltpu.bitcast(bst[:, ft * 128:(ft + 1) * 128], u32)
            for kc in range(3):
                t = w[kc * 128:(kc + 1) * 128, :]
                if kc == 2:
                    t = jnp.concatenate([t, jnp.zeros((64, 128), u32)], 0)
                tq[kc, ft * 128:(ft + 1) * 128, :] = t.T
        for j in range(3):
            for t in range(5):
                for kc in range(3):
                    rows = [tq[kc, pl.ds(j * DM + 4 * t + dd, NH, stride=BDH), :] for dd in range(4)]
                    gt = jnp.concatenate(rows, 0).T
                    n = 128 if kc < 2 else 64
                    bw[kc * 128:kc * 128 + n, j * DM + t * 128:j * DM + (t + 1) * 128] = gt[0:n]
        for c5 in range(5):
            to[c5] = bwo_st[:, c5 * 128:(c5 + 1) * 128].astype(f32)
        for c5 in range(5):
            for t in range(5):
                rows = [to[c5, pl.ds(4 * t + dd, NH, stride=BDH), :] for dd in range(4)]
                gt = jnp.concatenate(rows, 0).astype(bf16)
                bwo[t * 64:(t + 1) * 64, c5 * 128:(c5 + 1) * 128] = pltpu.bitcast(gt, u32)

    cp_b().wait()
    cp_bo().wait()
    for cpy in cp_wo():
        cpy.wait()
    a_finish(0, p_last, vm_last, "short", mid=b_weights)

    cp_x(1).wait()

    def short_body(tau, c):
        x_init(jnp.minimum(nlead + tau, nseg - 1))
        tick(tau, "short", "short")
        return c
    jax.lax.fori_loop(1, nlead, short_body, 0)
    tick(nlead, "short", "normal")

    def body(t2, c):
        tau = nlead + 1 + 2 * t2
        tick(tau, "normal", "normal")
        tick(tau + 1, "normal", "normal")

        @pl.when(tau > nseg)
        def _():
            out_copy(tau - nseg - 2, 2).start()
        return c
    assert (2 * nseg - nlead - 1) % 2 == 0 and nseg // 2 <= nlead < nseg
    jax.lax.fori_loop(0, (2 * nseg - nlead - 1) // 2, body, 0)
    for _ in b_steps(2 * nseg):
        pass
    out_copy(nseg - 2, 2).start()
    pltpu.make_async_copy(outv, out_hbm, out_sem).wait()


@functools.partial(jax.jit, static_argnames=("A_seg_len",))
def pallas_interleave_layers__memory_aug_recurrent_mem_tr__sliding_local_dilated__prompt_kernel(
    A_x, A_mem0, A_Wq, A_Wk, A_Wv, A_Wo, A_seg_len, B_x, B_wqkv, B_wo,
):
    del B_x
    B, S, Dm = A_x.shape
    assert B == 1 and Dm == DM and A_seg_len == SEG and S % SEG == 0
    nseg = S // SEG
    x = A_x.reshape(S, DM)
    mem0 = A_mem0.reshape(MEM, DM)
    wt = lambda w: jnp.transpose(w, (1, 2, 0)).reshape(NH * DH, DM)
    any_spec = pl.BlockSpec(memory_space=pl.ANY)
    out = pl.pallas_call(
        functools.partial(_kernel, nseg=nseg, nlead=NLEAD),
        out_shape=jax.ShapeDtypeStruct((S, DM), A_x.dtype),
        in_specs=[any_spec] * 8,
        out_specs=any_spec,
        scratch_shapes=[
            pltpu.VMEM((S, DM), bf16),
            pltpu.VMEM((MEM, DM), bf16),
            pltpu.VMEM((NP, 3, PW, DM), bf16),
            pltpu.VMEM((DM, 3 * DM), bf16),
            pltpu.VMEM((DM, DM), bf16),
            pltpu.VMEM((3, 3 * DM, 128), u32),
            pltpu.VMEM((5, DM, 128), f32),
            pltpu.VMEM((DM // 2, 3 * PW), u32),
            pltpu.VMEM((DM // 2, 3 * PW), u32),
            pltpu.VMEM((NP, DM // 2, 3 * PW), u32),
            pltpu.VMEM((5, NH * DH, 128), bf16),
            pltpu.VMEM((DM // 2, 3 * DM), u32),
            pltpu.VMEM((DM // 2, DM), u32),
            pltpu.VMEM((S, DM), f32),
            pltpu.VMEM((LL, DM), f32),
            pltpu.VMEM((LL + 8 * NLEAD, DM), f32),
            pltpu.VMEM((NP, LL + 8 * NLEAD, 3 * PW), f32),
            pltpu.VMEM((NP, LL, PW), f32),
            pltpu.VMEM((5, 16 + SEG, 128), f32),
            pltpu.VMEM((5, 16 + SEG, 128), f32),
            pltpu.VMEM((SEG, DM), f32),
            pltpu.VMEM((SEG, DM), f32),
            pltpu.VMEM((BW, SEG, 128), f32),
            pltpu.VMEM((S, DM), bf16),
            pltpu.SemaphoreType.DMA((10 + NP,)),
            pltpu.SemaphoreType.DMA(()),
        ],
        compiler_params=pltpu.CompilerParams(vmem_limit_bytes=116 * 1024 * 1024),
    )(x, mem0, wt(A_Wq), wt(A_Wk), wt(A_Wv), A_Wo.reshape(NH * DH, DM), B_wqkv, B_wo)
    return out.reshape(B, S, DM)
```

```python
import functools

import jax
import jax.numpy as jnp
import jax.experimental.pallas as pl
import jax.experimental.pallas.tpu as pltpu

f32 = jnp.float32
bf16 = jnp.bfloat16
u32 = jnp.uint32

DM = 640
NH = 32
DH = 192
NP = NH // 2
PW = 2 * DH
MEM = 8
SEG = 32
LL = MEM + SEG
BDH = DM // NH
BW, BDIL = 8, 2
LOG2E = 1.4426950408889634
EPS = 1e-5
NEG = -1e30
import os
PAD0 = int(os.environ.get('PAD0', '1'))
T_S, T_P, T_O = [int(v) for v in os.environ.get('TSPO', '0,2,4').split(',')]
OPT = os.environ.get('OPT', '')
OSPLIT = int(os.environ.get('OSPLIT', '8'))
import os
UNROLL = int(os.environ.get('UNROLL', '2'))
NLEAD = int(os.environ.get('NLEAD', '35'))


def _ln(x):
    m = jnp.mean(x, axis=-1, keepdims=True)
    d = x - m
    v = jnp.mean(d * d, axis=-1, keepdims=True)
    return d * jax.lax.rsqrt(v + EPS)


def _kernel(x_hbm, mem0_hbm, wq_hbm, wk_hbm, wv_hbm, wo_hbm, bqkv_hbm, bwo_hbm,
            out_hbm,
            pad0, xst, mem0_ref, wst, wo_st, bst, bwo_st, tq, to,
            wq_even, wq_odd, wo, bw, bwo, xres, mem, mem0f, hn, h0, pre, obuf, kbuf, vbuf, hb, qb, lg, outv,
            sems, out_sem, *, nseg, nlead):
    nx = (nlead + 1) * SEG

    def cp_mem0():
        return pltpu.make_async_copy(mem0_hbm, mem0_ref, sems.at[0])

    def cp_x(part):
        r = pl.ds(0, nx) if part == 0 else pl.ds(nx, nseg * SEG - nx)
        return pltpu.make_async_copy(x_hbm.at[r, :], xst.at[r, :], sems.at[8 + NP + part])

    def cp_b():
        return pltpu.make_async_copy(bqkv_hbm, bst, sems.at[1])

    def cp_bo():
        return pltpu.make_async_copy(bwo_hbm, bwo_st, sems.at[2])

    def cp_w(g, j):
        w = (wq_hbm, wk_hbm, wv_hbm)[j]
        return pltpu.make_async_copy(w.at[pl.ds(g * PW, PW), :], wst.at[g, j], sems.at[8 + g])

    def cp_wo():
        return [pltpu.make_async_copy(wo_hbm.at[:, pl.ds(c * 128, 128)], wo_st.at[c], sems.at[3 + c])
                for c in range(5)]

    for cpy in ([cp_x(0), cp_mem0()] + [cp_w(g, j) for g in range(NP) for j in (1, 0, 2)]
                + [cp_b(), cp_bo()] + cp_wo() + [cp_x(1)]):
        cpy.start()

    kbuf[...] = jnp.zeros(kbuf.shape, f32)
    vbuf[...] = jnp.zeros(vbuf.shape, f32)
    pre[NP - 1, 0:LL, :] = jnp.zeros((LL, 3 * PW), f32)
    for i in range(PAD0):
        pad0[8 * i:8 * i + 8, :] = jnp.full((8, 128), float(i), f32)
    cp_x(0).wait()
    cp_mem0().wait()
    h0[0:MEM, :] = mem0_ref[...].astype(f32)
    mem0f[...] = mem0_ref[...].astype(f32)
    h0[MEM:LL, :] = _ln(xst[0:SEG, :].astype(f32))
    for s in range(nlead):
        xs = xst[SEG * (s + 1):SEG * (s + 1) + 16, :].astype(f32)
        h0[LL + 8 * s:LL + 8 * s + 8, :] = _ln(xs[0:8])

    def x_init(s):
        r = pl.ds(pl.multiple_of(s * SEG, SEG), SEG)
        xres[r, :] = xst[r, :].astype(f32)

    def x_body(i, c):
        for u in range(4):
            x_init(4 * i + u)
        return c
    jax.lax.fori_loop(0, (nlead + 1) // 4, x_body, 0)
    for s in range((nlead + 1) // 4 * 4, nlead + 1):
        x_init(s)

    lane = jax.lax.broadcasted_iota(jnp.int32, (LL, 128), 1)
    row = jax.lax.broadcasted_iota(jnp.int32, (LL, 128), 0)
    a_scale = DH ** -0.5 * LOG2E
    b_scale = BDH ** -0.5 * LOG2E
    lo = lane < 64
    first = lane < LL
    key = jnp.where(first, lane, lane - LL)
    valid = (lane < 2 * LL) & ((row < MEM) | (row >= key))
    m0 = valid & first
    m1 = valid & jnp.logical_not(first)

    def blk(t):
        z40 = jnp.zeros((LL, 128), f32)
        z48 = jnp.zeros((128 - 2 * LL, 128), f32)
        ta, tb, tc = t[:, 0:128], t[:, 128:256], t[:, 256:384]
        a = jnp.concatenate([ta, z40, z48], 0)
        b = jnp.concatenate([jnp.where(lo, tb, 0.), jnp.where(lo, 0., tb), z48], 0)
        c = jnp.concatenate([z40, tc, z48], 0)
        return jnp.concatenate([a, b, c], 1).astype(bf16)

    def scores(q, kmat):
        return jax.lax.dot_general(q, kmat, (((1,), (1,)), ((), ())), preferred_element_type=f32)

    def softmax(sc):
        sc = sc * a_scale
        mx0 = jnp.max(jnp.where(m0, sc, NEG), axis=1, keepdims=True)
        mx1 = jnp.max(jnp.where(m1, sc, NEG), axis=1, keepdims=True)
        p = jnp.where(valid, jnp.exp2(sc - jnp.where(first, mx0, mx1)), 0.)
        l0 = jnp.sum(jnp.where(first, p, 0.), axis=1, keepdims=True)
        l1 = jnp.sum(jnp.where(first, 0., p), axis=1, keepdims=True)
        return p * pl.reciprocal(jnp.where(first, l0, l1), approx=True)

    def pv(g, p, vmat):
        obuf[g] = jnp.dot(p, vmat, preferred_element_type=f32)

    def oproj(g0, g1, first=False):
        o = jnp.concatenate([obuf[g] for g in range(g0, g1)], axis=1)
        outs = []
        for c in range(5):
            if first:
                w = wo_st[c, g0 * PW:g1 * PW, :]
                wo[c, g0 * DH:g1 * DH, :] = pltpu.bitcast(w, u32)
            else:
                w = pltpu.bitcast(wo[c, g0 * DH:g1 * DH, :], bf16)
            outs.append(jnp.dot(o, w, preferred_element_type=f32))
        return jnp.concatenate(outs, axis=1)

    def a_finish(tau, p_last, vm_last, first):
        seg = tau & (nseg - 1)
        rows = pl.ds(pl.multiple_of(seg * SEG, SEG), SEG)
        nxt = (tau + 1) & (nseg - 1)
        if 'lnlate' not in OPT:
            hn[...] = _ln(xres[pl.ds(pl.multiple_of(nxt * SEG, SEG), SEG), :])
        r1 = oproj(0, OSPLIT, first)
        if 'lnlate' in OPT:
            hn[...] = _ln(xres[pl.ds(pl.multiple_of(nxt * SEG, SEG), SEG), :])
        if first:
            b_weights()
        pv(NP - 1, p_last, vm_last)
        res = r1 + oproj(OSPLIT, NP, first)
        if 'm0f' in OPT:
            mem[...] = jnp.where(seg == nseg - 1, mem0f[...], res[0:MEM])
        else:
            mem[...] = jnp.where(seg == nseg - 1, mem0_ref[...].astype(f32), res[0:MEM])
        xres[rows, :] = xres[rows, :] + res[MEM:LL]

    def a_steps(tau, mode):
        if mode == "short":
            prow = pl.ds(pl.multiple_of(LL + (tau - 1) * 8, 8), 8)

        def proj(g, j):
            cols = slice(j * PW, (j + 1) * PW)
            w = pltpu.bitcast((wq_even, wq_odd)[g % 2][g // 2, :, cols], bf16)
            if mode == "short":
                h = jnp.concatenate([mem[...], hn[8:SEG, :]], axis=0)
                y = jnp.dot(h, w, preferred_element_type=f32)
                return jnp.concatenate([y[0:MEM], pre[g, prow, cols], y[MEM:SEG]], axis=0)
            h = jnp.concatenate([mem[...], hn[...]], axis=0)
            return jnp.dot(h, w, preferred_element_type=f32)

        scs, vms, ps = {}, {}, {}
        for g in range(NP):
            kmat = blk(proj(g, 1))
            q = proj(g, 0)
            vms[g] = blk(proj(g, 2))
            if g >= 1:
                ps[g - 1] = softmax(scs.pop(g - 1))
            scs[g] = scores(q, kmat)
            if g >= 1:
                pv(g - 1, ps.pop(g - 1), vms.pop(g - 1))
            yield
        a_finish(tau, softmax(scs.pop(NP - 1)), vms.pop(NP - 1), False)

    def b_steps(tau):
        j = (tau - 1) & (nseg - 1)
        rows = pl.ds(pl.multiple_of(j * SEG, SEG), SEG)

        def bproj(t):
            return jnp.dot(hb[...], pltpu.bitcast(bw[:, t * DM:(t + 1) * DM], bf16),
                           preferred_element_type=f32)

        hb[...] = _ln(xres[rows, :])
        for c in range(5):
            kbuf[c, 0:16, :] = kbuf[c, SEG:SEG + 16, :]
            vbuf[c, 0:16, :] = vbuf[c, SEG:SEG + 16, :]
        yield
        qb[...] = bproj(0) * b_scale
        yield
        k = bproj(1)
        for c in range(5):
            kbuf[c, 16:16 + SEG, :] = k[:, c * 128:(c + 1) * 128]
        yield
        v = bproj(2)
        for c in range(5):
            vbuf[c, 16:16 + SEG, :] = v[:, c * 128:(c + 1) * 128]
        yield
        pos = jax.lax.broadcasted_iota(jnp.int32, (SEG, 128), 0) + j * SEG
        for w in range(BW):
            off = 16 - w * BDIL
            acc = qb[:, 0:128] * kbuf[0, off:off + SEG, :]
            for c in range(1, 5):
                acc = acc + qb[:, c * 128:(c + 1) * 128] * kbuf[c, off:off + SEG, :]
            acc = acc + pltpu.roll(acc, 64, 1)
            acc = acc + pltpu.roll(acc, 32, 1)
            if w > 0:
                acc = jnp.where(pos >= w * BDIL, acc, NEG)
            lg[w] = acc
            if w % 2 == 1:
                yield
        lgs = [lg[w] for w in range(BW)]
        mx = functools.reduce(jnp.maximum, lgs)
        es = [jnp.exp2(l - mx) for l in lgs]
        inv = pl.reciprocal(functools.reduce(jnp.add, es), approx=True)
        for w in range(BW):
            lg[w] = es[w] * inv
        yield
        for c in range(5):
            acc = None
            for w in range(BW):
                off = 16 - w * BDIL
                t = lg[w] * vbuf[c, off:off + SEG, :]
                acc = t if acc is None else acc + t
            qb[:, c * 128:(c + 1) * 128] = acc
            if c in (1, 3):
                yield
        yield
        x2 = xres[rows, :] + jnp.dot(qb[...], pltpu.bitcast(bwo[...], bf16), preferred_element_type=f32)
        xres[rows, :] = x2
        outv[rows, :] = x2.astype(bf16)

    def out_copy(j, n):
        r = pl.ds(pl.multiple_of(j * SEG, SEG), n * SEG)
        return pltpu.make_async_copy(outv.at[r, :], out_hbm.at[r, :], out_sem)

    def tick(tau, mode):
        live = [b_steps(tau), a_steps(tau, mode)]
        if 'ab' in OPT:
            live = live[::-1]
        if 'b1' in OPT:
            next(live[1] if 'ab' not in OPT else live[0])
        if 'b2' in OPT:
            next(live[1] if 'ab' not in OPT else live[0])
            next(live[1] if 'ab' not in OPT else live[0])
        while live:
            for gen in list(live):
                try:
                    next(gen)
                except StopIteration:
                    live.remove(gen)

    def w_wait(g):
        pltpu.make_async_copy(wst.at[g], wst.at[g], sems.at[8 + g]).wait()

    def stage(g, dst, slot, t):
        j, r = divmod(t, 3)
        dst[slot, :, t * 128:(t + 1) * 128] = pltpu.bitcast(wst[g, j, r * 128:(r + 1) * 128, :].T, u32)

    def first_att(g):
        q, k, v = (pre[g, 0:LL, j * PW:(j + 1) * PW] for j in range(3))
        return softmax(scores(q, blk(k))), blk(v)

    def first_pair(g, cur, cur_slot, nxt, nxt_slot):
        gp = (g + NP - 1) & (NP - 1)
        gn = jnp.minimum(g + 1, NP - 1)
        for t in range(9):
            if t == T_S:
                sc = scores(pre[gp, 0:LL, 0:PW], blk(pre[gp, 0:LL, PW:2 * PW]))
            cols = slice(t * 128, (t + 1) * 128)
            w = pltpu.bitcast(cur[cur_slot, :, cols], bf16)
            pre[g, :, cols] = jnp.dot(h0[...], w, preferred_element_type=f32)
            stage(gn, nxt, nxt_slot, t)
            if t == T_P:
                p = softmax(sc)
            if t == T_O:
                pv(gp, p, blk(pre[gp, 0:LL, 2 * PW:3 * PW]))

    w_wait(0)
    for t in range(9):
        stage(0, wq_even, 0, t)

    def first_body(i, c):
        w_wait(2 * i + 1)
        first_pair(2 * i, wq_even, i, wq_odd, i)

        @pl.when(2 * i + 2 < NP)
        def _():
            w_wait(2 * i + 2)
        first_pair(2 * i + 1, wq_odd, i, wq_even, i + 1)
        return c
    jax.lax.fori_loop(0, NP // 2, first_body, 0)
    p_last, vm_last = first_att(NP - 1)

    def b_weights():
        for ft in range(3 * DM // 128):
            w = pltpu.bitcast(bst[:, ft * 128:(ft + 1) * 128], u32)
            for kc in range(3):
                t = w[kc * 128:(kc + 1) * 128, :]
                if kc == 2:
                    t = jnp.concatenate([t, jnp.zeros((64, 128), u32)], 0)
                tq[kc, ft * 128:(ft + 1) * 128, :] = t.T
        for j in range(3):
            for t in range(5):
                for kc in range(3):
                    rows = [tq[kc, pl.ds(j * DM + 4 * t + dd, NH, stride=BDH), :] for dd in range(4)]
                    gt = jnp.concatenate(rows, 0).T
                    n = 128 if kc < 2 else 64
                    bw[kc * 128:kc * 128 + n, j * DM + t * 128:j * DM + (t + 1) * 128] = gt[0:n]
        for c5 in range(5):
            to[c5] = bwo_st[:, c5 * 128:(c5 + 1) * 128].astype(f32)
        for c5 in range(5):
            for t in range(5):
                rows = [to[c5, pl.ds(4 * t + dd, NH, stride=BDH), :] for dd in range(4)]
                gt = jnp.concatenate(rows, 0).astype(bf16)
                bwo[t * 64:(t + 1) * 64, c5 * 128:(c5 + 1) * 128] = pltpu.bitcast(gt, u32)

    cp_b().wait()
    cp_bo().wait()
    for cpy in cp_wo():
        cpy.wait()
    a_finish(0, p_last, vm_last, True)

    cp_x(1).wait()

    def short_body(tau, c):
        tick(tau, "short")
        x_init(jnp.minimum(nlead + tau, nseg - 1))
        return c
    jax.lax.fori_loop(1, nlead + 1, short_body, 0)

    un = UNROLL

    def body(it, c):
        tau = nlead + 1 + un * it
        for u in range(un):
            tick(tau + u, "normal")

        @pl.when(tau >= nseg + un)
        def _():
            out_copy(tau - nseg - un, un).start()
        return c
    assert (2 * nseg - nlead - 1) % un == 0 and nseg // 2 <= nlead < nseg
    jax.lax.fori_loop(0, (2 * nseg - nlead - 1) // un, body, 0)
    for _ in b_steps(2 * nseg):
        pass
    t0 = nlead + 1 + un * (-(-(nseg + un - nlead - 1) // un))
    if t0 - nseg - un > 0:
        pltpu.make_async_copy(outv.at[0:(t0 - nseg - un) * SEG, :], out_hbm.at[0:(t0 - nseg - un) * SEG, :], out_sem).start()
    out_copy(nseg - un, un).start()
    pltpu.make_async_copy(outv, out_hbm, out_sem).wait()


@functools.partial(jax.jit, static_argnames=("A_seg_len",))
def pallas_interleave_layers__memory_aug_recurrent_mem_tr__sliding_local_dilated__prompt_kernel(
    A_x, A_mem0, A_Wq, A_Wk, A_Wv, A_Wo, A_seg_len, B_x, B_wqkv, B_wo,
):
    del B_x
    B, S, Dm = A_x.shape
    assert B == 1 and Dm == DM and A_seg_len == SEG and S % SEG == 0
    nseg = S // SEG
    x = A_x.reshape(S, DM)
    mem0 = A_mem0.reshape(MEM, DM)
    wt = lambda w: jnp.transpose(w, (1, 2, 0)).reshape(NH * DH, DM)
    any_spec = pl.BlockSpec(memory_space=pl.ANY)
    out = pl.pallas_call(
        functools.partial(_kernel, nseg=nseg, nlead=NLEAD),
        out_shape=jax.ShapeDtypeStruct((S, DM), A_x.dtype),
        in_specs=[any_spec] * 8,
        out_specs=any_spec,
        scratch_shapes=[
            pltpu.VMEM((PAD0 * 8, 128), f32),
            pltpu.VMEM((S, DM), bf16),
            pltpu.VMEM((MEM, DM), bf16),
            pltpu.VMEM((NP, 3, PW, DM), bf16),
            pltpu.VMEM((5, NH * DH, 128), bf16),
            pltpu.VMEM((DM, 3 * DM), bf16),
            pltpu.VMEM((DM, DM), bf16),
            pltpu.VMEM((3, 3 * DM, 128), u32),
            pltpu.VMEM((5, DM, 128), f32),
            pltpu.VMEM((NP // 2 + 1, DM // 2, 3 * PW), u32),
            pltpu.VMEM((NP // 2, DM // 2, 3 * PW), u32),
            pltpu.VMEM((5, NH * DH // 2, 128), u32),
            pltpu.VMEM((DM // 2, 3 * DM), u32),
            pltpu.VMEM((DM // 2, DM), u32),
            pltpu.VMEM((S, DM), f32),
            pltpu.VMEM((MEM, DM), f32),
            pltpu.VMEM((MEM, DM), f32),
            pltpu.VMEM((SEG, DM), f32),
            pltpu.VMEM((LL + 8 * NLEAD, DM), f32),
            pltpu.VMEM((NP, LL + 8 * NLEAD, 3 * PW), f32),
            pltpu.VMEM((NP, LL, PW), f32),
            pltpu.VMEM((5, 16 + SEG, 128), f32),
            pltpu.VMEM((5, 16 + SEG, 128), f32),
            pltpu.VMEM((SEG, DM), f32),
            pltpu.VMEM((SEG, DM), f32),
            pltpu.VMEM((BW, SEG, 128), f32),
            pltpu.VMEM((S, DM), bf16),
            pltpu.SemaphoreType.DMA((10 + NP,)),
            pltpu.SemaphoreType.DMA(()),
        ],
        compiler_params=pltpu.CompilerParams(vmem_limit_bytes=124 * 1024 * 1024),
    )(x, mem0, wt(A_Wq), wt(A_Wk), wt(A_Wv), A_Wo.reshape(NH * DH, DM), B_wqkv, B_wo)
    return out.reshape(B, S, DM)
```

```python
import functools

import jax
import jax.numpy as jnp
import jax.experimental.pallas as pl
import jax.experimental.pallas.tpu as pltpu

f32 = jnp.float32
bf16 = jnp.bfloat16
u32 = jnp.uint32

DM = 640
NH = 32
DH = 192
NP = NH // 2
PW = 2 * DH
MEM = 8
SEG = 32
LL = MEM + SEG
BDH = DM // NH
BW, BDIL = 8, 2
LOG2E = 1.4426950408889634
EPS = 1e-5
NEG = -1e30
import os
PAD0 = int(os.environ.get('PAD0', '1'))
T_S, T_P, T_O = [int(v) for v in os.environ.get('TSPO', '0,2,4').split(',')]
OPT = os.environ.get('OPT', '')
OSPLIT = int(os.environ.get('OSPLIT', '8'))
import os
UNROLL = int(os.environ.get('UNROLL', '2'))
NLEAD = int(os.environ.get('NLEAD', '35'))


def _ln(x):
    m = jnp.mean(x, axis=-1, keepdims=True)
    d = x - m
    v = jnp.mean(d * d, axis=-1, keepdims=True)
    return d * jax.lax.rsqrt(v + EPS)


def _kernel(x_hbm, mem0_hbm, wq_hbm, wk_hbm, wv_hbm, wo_hbm, bqkv_hbm, bwo_hbm,
            out_hbm,
            pad0, xst, mem0_ref, wst, wo_st, bst, bwo_st, tq, to,
            wq_even, wq_odd, wo, bw, bwo, xres, mem, mem0f, hn, h0, pre, obuf, kbuf, vbuf, hb, qb, lg, outv,
            sems, out_sem, *, nseg, nlead):
    nx = (nlead + 1) * SEG

    def cp_mem0():
        return pltpu.make_async_copy(mem0_hbm, mem0_ref, sems.at[0])

    def cp_x(part):
        r = pl.ds(0, nx) if part == 0 else pl.ds(nx, nseg * SEG - nx)
        return pltpu.make_async_copy(x_hbm.at[r, :], xst.at[r, :], sems.at[8 + NP + part])

    def cp_b():
        return pltpu.make_async_copy(bqkv_hbm, bst, sems.at[1])

    def cp_bo():
        return pltpu.make_async_copy(bwo_hbm, bwo_st, sems.at[2])

    def cp_w(g, j):
        w = (wq_hbm, wk_hbm, wv_hbm)[j]
        return pltpu.make_async_copy(w.at[pl.ds(g * PW, PW), :], wst.at[g, j], sems.at[8 + g])

    def cp_wo():
        return [pltpu.make_async_copy(wo_hbm.at[:, pl.ds(c * 128, 128)], wo_st.at[c], sems.at[3 + c])
                for c in range(5)]

    for cpy in ([cp_x(0), cp_mem0()] + [cp_w(g, j) for g in range(NP) for j in (1, 0, 2)]
                + [cp_b(), cp_bo()] + cp_wo() + [cp_x(1)]):
        cpy.start()

    kbuf[...] = jnp.zeros(kbuf.shape, f32)
    vbuf[...] = jnp.zeros(vbuf.shape, f32)
    for i in range(PAD0):
        pad0[8 * i:8 * i + 8, :] = jnp.full((8, 128), float(i), f32)
    cp_x(0).wait()
    cp_mem0().wait()
    h0[0:MEM, :] = mem0_ref[...].astype(f32)
    mem0f[...] = mem0_ref[...].astype(f32)
    h0[MEM:LL, :] = _ln(xst[0:SEG, :].astype(f32))
    for s in range(nlead):
        xs = xst[SEG * (s + 1):SEG * (s + 1) + 16, :].astype(f32)
        h0[LL + 8 * s:LL + 8 * s + 8, :] = _ln(xs[0:8])

    def x_init(s):
        r = pl.ds(pl.multiple_of(s * SEG, SEG), SEG)
        xres[r, :] = xst[r, :].astype(f32)

    def x_body(i, c):
        for u in range(4):
            x_init(4 * i + u)
        return c
    jax.lax.fori_loop(0, (nlead + 1) // 4, x_body, 0)
    for s in range((nlead + 1) // 4 * 4, nlead + 1):
        x_init(s)

    lane = jax.lax.broadcasted_iota(jnp.int32, (LL, 128), 1)
    row = jax.lax.broadcasted_iota(jnp.int32, (LL, 128), 0)
    a_scale = DH ** -0.5 * LOG2E
    b_scale = BDH ** -0.5 * LOG2E
    lo = lane < 64
    first = lane < LL
    key = jnp.where(first, lane, lane - LL)
    valid = (lane < 2 * LL) & ((row < MEM) | (row >= key))
    m0 = valid & first
    m1 = valid & jnp.logical_not(first)

    def blk(t):
        z40 = jnp.zeros((LL, 128), f32)
        z48 = jnp.zeros((128 - 2 * LL, 128), f32)
        ta, tb, tc = t[:, 0:128], t[:, 128:256], t[:, 256:384]
        a = jnp.concatenate([ta, z40, z48], 0)
        b = jnp.concatenate([jnp.where(lo, tb, 0.), jnp.where(lo, 0., tb), z48], 0)
        c = jnp.concatenate([z40, tc, z48], 0)
        return jnp.concatenate([a, b, c], 1).astype(bf16)

    def scores(q, kmat):
        return jax.lax.dot_general(q, kmat, (((1,), (1,)), ((), ())), preferred_element_type=f32)

    def softmax(sc):
        sc = sc * a_scale
        mx0 = jnp.max(jnp.where(m0, sc, NEG), axis=1, keepdims=True)
        mx1 = jnp.max(jnp.where(m1, sc, NEG), axis=1, keepdims=True)
        p = jnp.where(valid, jnp.exp2(sc - jnp.where(first, mx0, mx1)), 0.)
        l0 = jnp.sum(jnp.where(first, p, 0.), axis=1, keepdims=True)
        l1 = jnp.sum(jnp.where(first, 0., p), axis=1, keepdims=True)
        return p * pl.reciprocal(jnp.where(first, l0, l1), approx=True)

    def pv(g, p, vmat):
        obuf[g] = jnp.dot(p, vmat, preferred_element_type=f32)

    def oproj(g0, g1, first=False):
        o = jnp.concatenate([obuf[g] for g in range(g0, g1)], axis=1)
        outs = []
        for c in range(5):
            if first:
                w = wo_st[c, g0 * PW:g1 * PW, :]
                wo[c, g0 * DH:g1 * DH, :] = pltpu.bitcast(w, u32)
            else:
                w = pltpu.bitcast(wo[c, g0 * DH:g1 * DH, :], bf16)
            outs.append(jnp.dot(o, w, preferred_element_type=f32))
        return jnp.concatenate(outs, axis=1)

    def a_finish(tau, p_last, vm_last, first):
        seg = tau & (nseg - 1)
        rows = pl.ds(pl.multiple_of(seg * SEG, SEG), SEG)
        nxt = (tau + 1) & (nseg - 1)
        if 'lnlate' not in OPT:
            hn[...] = _ln(xres[pl.ds(pl.multiple_of(nxt * SEG, SEG), SEG), :])
        r1 = oproj(0, OSPLIT, first)
        if 'lnlate' in OPT:
            hn[...] = _ln(xres[pl.ds(pl.multiple_of(nxt * SEG, SEG), SEG), :])
        if first:
            b_weights()
        pv(NP - 1, p_last, vm_last)
        res = r1 + oproj(OSPLIT, NP, first)
        if 'm0f' in OPT:
            mem[...] = jnp.where(seg == nseg - 1, mem0f[...], res[0:MEM])
        else:
            mem[...] = jnp.where(seg == nseg - 1, mem0_ref[...].astype(f32), res[0:MEM])
        xres[rows, :] = xres[rows, :] + res[MEM:LL]

    def a_steps(tau, mode):
        if mode == "short":
            prow = pl.ds(pl.multiple_of((tau - 1) * 8, 8), 8)

        def proj(g, j):
            cols = slice(j * PW, (j + 1) * PW)
            w = pltpu.bitcast((wq_even, wq_odd)[g % 2][g // 2, :, cols], bf16)
            if mode == "short":
                h = jnp.concatenate([mem[...], hn[8:SEG, :]], axis=0)
                y = jnp.dot(h, w, preferred_element_type=f32)
                return jnp.concatenate([y[0:MEM], pre[g, prow, cols], y[MEM:SEG]], axis=0)
            h = jnp.concatenate([mem[...], hn[...]], axis=0)
            return jnp.dot(h, w, preferred_element_type=f32)

        scs, vms, ps = {}, {}, {}
        for g in range(NP):
            kmat = blk(proj(g, 1))
            q = proj(g, 0)
            vms[g] = blk(proj(g, 2))
            if g >= 1:
                ps[g - 1] = softmax(scs.pop(g - 1))
            scs[g] = scores(q, kmat)
            if g >= 1:
                pv(g - 1, ps.pop(g - 1), vms.pop(g - 1))
            yield
        a_finish(tau, softmax(scs.pop(NP - 1)), vms.pop(NP - 1), False)

    def b_steps(tau):
        j = (tau - 1) & (nseg - 1)
        rows = pl.ds(pl.multiple_of(j * SEG, SEG), SEG)

        def bproj(t):
            return jnp.dot(hb[...], pltpu.bitcast(bw[:, t * DM:(t + 1) * DM], bf16),
                           preferred_element_type=f32)

        hb[...] = _ln(xres[rows, :])
        for c in range(5):
            kbuf[c, 0:16, :] = kbuf[c, SEG:SEG + 16, :]
            vbuf[c, 0:16, :] = vbuf[c, SEG:SEG + 16, :]
        yield
        qb[...] = bproj(0) * b_scale
        yield
        k = bproj(1)
        for c in range(5):
            kbuf[c, 16:16 + SEG, :] = k[:, c * 128:(c + 1) * 128]
        yield
        v = bproj(2)
        for c in range(5):
            vbuf[c, 16:16 + SEG, :] = v[:, c * 128:(c + 1) * 128]
        yield
        pos = jax.lax.broadcasted_iota(jnp.int32, (SEG, 128), 0) + j * SEG
        for w in range(BW):
            off = 16 - w * BDIL
            acc = qb[:, 0:128] * kbuf[0, off:off + SEG, :]
            for c in range(1, 5):
                acc = acc + qb[:, c * 128:(c + 1) * 128] * kbuf[c, off:off + SEG, :]
            acc = acc + pltpu.roll(acc, 64, 1)
            acc = acc + pltpu.roll(acc, 32, 1)
            if w > 0:
                acc = jnp.where(pos >= w * BDIL, acc, NEG)
            lg[w] = acc
            if w % 2 == 1:
                yield
        lgs = [lg[w] for w in range(BW)]
        mx = functools.reduce(jnp.maximum, lgs)
        es = [jnp.exp2(l - mx) for l in lgs]
        inv = pl.reciprocal(functools.reduce(jnp.add, es), approx=True)
        for w in range(BW):
            lg[w] = es[w] * inv
        yield
        for c in range(5):
            acc = None
            for w in range(BW):
                off = 16 - w * BDIL
                t = lg[w] * vbuf[c, off:off + SEG, :]
                acc = t if acc is None else acc + t
            qb[:, c * 128:(c + 1) * 128] = acc
            if c in (1, 3):
                yield
        yield
        x2 = xres[rows, :] + jnp.dot(qb[...], pltpu.bitcast(bwo[...], bf16), preferred_element_type=f32)
        xres[rows, :] = x2
        outv[rows, :] = x2.astype(bf16)

    def out_copy(j, n):
        r = pl.ds(pl.multiple_of(j * SEG, SEG), n * SEG)
        return pltpu.make_async_copy(outv.at[r, :], out_hbm.at[r, :], out_sem)

    def tick(tau, mode):
        live = [b_steps(tau), a_steps(tau, mode)]
        if 'ab' in OPT:
            live = live[::-1]
        if 'b1' in OPT:
            next(live[1] if 'ab' not in OPT else live[0])
        if 'b2' in OPT:
            next(live[1] if 'ab' not in OPT else live[0])
            next(live[1] if 'ab' not in OPT else live[0])
        while live:
            for gen in list(live):
                try:
                    next(gen)
                except StopIteration:
                    live.remove(gen)

    def w_wait(g):
        pltpu.make_async_copy(wst.at[g], wst.at[g], sems.at[8 + g]).wait()

    def stage(g, dst, slot, t):
        j, r = divmod(t, 3)
        dst[slot, :, t * 128:(t + 1) * 128] = pltpu.bitcast(wst[g, j, r * 128:(r + 1) * 128, :].T, u32)

    def first_pair(g, cur, cur_slot, nxt, nxt_slot, sc_prev, vm_prev):
        gp = (g + NP - 1) & (NP - 1)
        gn = jnp.minimum(g + 1, NP - 1)

        def proj(j):
            tiles = []
            for r in range(3):
                t = 3 * j + r
                cols = slice(t * 128, (t + 1) * 128)
                w = pltpu.bitcast(cur[cur_slot, :, cols], bf16)
                y = jnp.dot(h0[...], w, preferred_element_type=f32)
                pre[g, :, cols] = y[LL:]
                tiles.append(y[0:LL])
                stage(gn, nxt, nxt_slot, (3 * ((j + 2) % 3) + r))
            return jnp.concatenate(tiles, axis=1)

        kmat = blk(proj(1))
        p = softmax(sc_prev)
        q = proj(0)
        sc = scores(q, kmat)
        pv(gp, p, vm_prev)
        vm = blk(proj(2))
        return sc, vm

    w_wait(0)
    for t in range(9):
        stage(0, wq_even, 0, t)

    def first_body(i, carry):
        w_wait(2 * i + 1)
        carry = first_pair(2 * i, wq_even, i, wq_odd, i, *carry)

        @pl.when(2 * i + 2 < NP)
        def _():
            w_wait(2 * i + 2)
        return first_pair(2 * i + 1, wq_odd, i, wq_even, i + 1, *carry)
    sc_last, vm_last = jax.lax.fori_loop(
        0, NP // 2, first_body, (jnp.zeros((LL, 128), f32), jnp.zeros((128, PW), bf16)))
    p_last = softmax(sc_last)

    def b_weights():
        for ft in range(3 * DM // 128):
            w = pltpu.bitcast(bst[:, ft * 128:(ft + 1) * 128], u32)
            for kc in range(3):
                t = w[kc * 128:(kc + 1) * 128, :]
                if kc == 2:
                    t = jnp.concatenate([t, jnp.zeros((64, 128), u32)], 0)
                tq[kc, ft * 128:(ft + 1) * 128, :] = t.T
        for j in range(3):
            for t in range(5):
                for kc in range(3):
                    rows = [tq[kc, pl.ds(j * DM + 4 * t + dd, NH, stride=BDH), :] for dd in range(4)]
                    gt = jnp.concatenate(rows, 0).T
                    n = 128 if kc < 2 else 64
                    bw[kc * 128:kc * 128 + n, j * DM + t * 128:j * DM + (t + 1) * 128] = gt[0:n]
        for c5 in range(5):
            to[c5] = bwo_st[:, c5 * 128:(c5 + 1) * 128].astype(f32)
        for c5 in range(5):
            for t in range(5):
                rows = [to[c5, pl.ds(4 * t + dd, NH, stride=BDH), :] for dd in range(4)]
                gt = jnp.concatenate(rows, 0).astype(bf16)
                bwo[t * 64:(t + 1) * 64, c5 * 128:(c5 + 1) * 128] = pltpu.bitcast(gt, u32)

    cp_b().wait()
    cp_bo().wait()
    for cpy in cp_wo():
        cpy.wait()
    a_finish(0, p_last, vm_last, True)

    cp_x(1).wait()

    def short_body(tau, c):
        tick(tau, "short")
        x_init(jnp.minimum(nlead + tau, nseg - 1))
        return c
    jax.lax.fori_loop(1, nlead + 1, short_body, 0)

    un = UNROLL

    def body(it, c):
        tau = nlead + 1 + un * it
        for u in range(un):
            tick(tau + u, "normal")

        @pl.when(tau >= nseg + un)
        def _():
            out_copy(tau - nseg - un, un).start()
        return c
    assert (2 * nseg - nlead - 1) % un == 0 and nseg // 2 <= nlead < nseg
    jax.lax.fori_loop(0, (2 * nseg - nlead - 1) // un, body, 0)
    for _ in b_steps(2 * nseg):
        pass
    t0 = nlead + 1 + un * (-(-(nseg + un - nlead - 1) // un))
    if t0 - nseg - un > 0:
        pltpu.make_async_copy(outv.at[0:(t0 - nseg - un) * SEG, :], out_hbm.at[0:(t0 - nseg - un) * SEG, :], out_sem).start()
    out_copy(nseg - un, un).start()
    pltpu.make_async_copy(outv, out_hbm, out_sem).wait()


@functools.partial(jax.jit, static_argnames=("A_seg_len",))
def pallas_interleave_layers__memory_aug_recurrent_mem_tr__sliding_local_dilated__prompt_kernel(
    A_x, A_mem0, A_Wq, A_Wk, A_Wv, A_Wo, A_seg_len, B_x, B_wqkv, B_wo,
):
    del B_x
    B, S, Dm = A_x.shape
    assert B == 1 and Dm == DM and A_seg_len == SEG and S % SEG == 0
    nseg = S // SEG
    x = A_x.reshape(S, DM)
    mem0 = A_mem0.reshape(MEM, DM)
    wt = lambda w: jnp.transpose(w, (1, 2, 0)).reshape(NH * DH, DM)
    any_spec = pl.BlockSpec(memory_space=pl.ANY)
    out = pl.pallas_call(
        functools.partial(_kernel, nseg=nseg, nlead=NLEAD),
        out_shape=jax.ShapeDtypeStruct((S, DM), A_x.dtype),
        in_specs=[any_spec] * 8,
        out_specs=any_spec,
        scratch_shapes=[
            pltpu.VMEM((PAD0 * 8, 128), f32),
            pltpu.VMEM((S, DM), bf16),
            pltpu.VMEM((MEM, DM), bf16),
            pltpu.VMEM((NP, 3, PW, DM), bf16),
            pltpu.VMEM((5, NH * DH, 128), bf16),
            pltpu.VMEM((DM, 3 * DM), bf16),
            pltpu.VMEM((DM, DM), bf16),
            pltpu.VMEM((3, 3 * DM, 128), u32),
            pltpu.VMEM((5, DM, 128), f32),
            pltpu.VMEM((NP // 2 + 1, DM // 2, 3 * PW), u32),
            pltpu.VMEM((NP // 2, DM // 2, 3 * PW), u32),
            pltpu.VMEM((5, NH * DH // 2, 128), u32),
            pltpu.VMEM((DM // 2, 3 * DM), u32),
            pltpu.VMEM((DM // 2, DM), u32),
            pltpu.VMEM((S, DM), f32),
            pltpu.VMEM((MEM, DM), f32),
            pltpu.VMEM((MEM, DM), f32),
            pltpu.VMEM((SEG, DM), f32),
            pltpu.VMEM((LL + 8 * NLEAD, DM), f32),
            pltpu.VMEM((NP, 8 * NLEAD, 3 * PW), f32),
            pltpu.VMEM((NP, LL, PW), f32),
            pltpu.VMEM((5, 16 + SEG, 128), f32),
            pltpu.VMEM((5, 16 + SEG, 128), f32),
            pltpu.VMEM((SEG, DM), f32),
            pltpu.VMEM((SEG, DM), f32),
            pltpu.VMEM((BW, SEG, 128), f32),
            pltpu.VMEM((S, DM), bf16),
            pltpu.SemaphoreType.DMA((10 + NP,)),
            pltpu.SemaphoreType.DMA(()),
        ],
        compiler_params=pltpu.CompilerParams(vmem_limit_bytes=124 * 1024 * 1024),
    )(x, mem0, wt(A_Wq), wt(A_Wk), wt(A_Wv), A_Wo.reshape(NH * DH, DM), B_wqkv, B_wo)
    return out.reshape(B, S, DM)
```

```python
import functools

import jax
import jax.numpy as jnp
import jax.experimental.pallas as pl
import jax.experimental.pallas.tpu as pltpu

f32 = jnp.float32
bf16 = jnp.bfloat16
u32 = jnp.uint32

DM = 640
NH = 32
DH = 192
NP = NH // 2
PW = 2 * DH
MEM = 8
SEG = 32
LL = MEM + SEG
BDH = DM // NH
BW, BDIL = 8, 2
LOG2E = 1.4426950408889634
EPS = 1e-5
NEG = -1e30
import os
PAD0 = int(os.environ.get('PAD0', '1'))
T_S, T_P, T_O = [int(v) for v in os.environ.get('TSPO', '0,2,4').split(',')]
OPT = os.environ.get('OPT', '')
OSPLIT = int(os.environ.get('OSPLIT', '8'))
import os
UNROLL = int(os.environ.get('UNROLL', '2'))
NLEAD = int(os.environ.get('NLEAD', '35'))


def _ln(x):
    m = jnp.mean(x, axis=-1, keepdims=True)
    d = x - m
    v = jnp.mean(d * d, axis=-1, keepdims=True)
    return d * jax.lax.rsqrt(v + EPS)


def _kernel(x_hbm, mem0_hbm, wq_hbm, wk_hbm, wv_hbm, wo_hbm, bqkv_hbm, bwo_hbm,
            out_hbm,
            pad0, xst, mem0_ref, wst, wo_st, bst, bwo_st, tq, to,
            wq_even, wq_odd, wo, bw, bwo, xres, mem, mem0f, hn, h0, pre, obuf, kbuf, vbuf, hb, qb, lg, outv,
            sems, out_sem, *, nseg, nlead):
    nx = (nlead + 1) * SEG

    def cp_mem0():
        return pltpu.make_async_copy(mem0_hbm, mem0_ref, sems.at[0])

    def cp_x(part):
        r = pl.ds(0, nx) if part == 0 else pl.ds(nx, nseg * SEG - nx)
        return pltpu.make_async_copy(x_hbm.at[r, :], xst.at[r, :], sems.at[8 + NP + part])

    def cp_b():
        return pltpu.make_async_copy(bqkv_hbm, bst, sems.at[1])

    def cp_bo():
        return pltpu.make_async_copy(bwo_hbm, bwo_st, sems.at[2])

    def cp_w(g, j):
        w = (wq_hbm, wk_hbm, wv_hbm)[j]
        return pltpu.make_async_copy(w.at[pl.ds(g * PW, PW), :], wst.at[g, j], sems.at[8 + g])

    def cp_wo():
        return [pltpu.make_async_copy(wo_hbm.at[:, pl.ds(c * 128, 128)], wo_st.at[c], sems.at[3 + c])
                for c in range(5)]

    for cpy in ([cp_x(0), cp_mem0()] + [cp_w(g, j) for g in range(NP) for j in (1, 0, 2)]
                + [cp_b(), cp_bo()] + cp_wo() + [cp_x(1)]):
        cpy.start()

    kbuf[...] = jnp.zeros(kbuf.shape, f32)
    vbuf[...] = jnp.zeros(vbuf.shape, f32)
    for i in range(PAD0):
        pad0[8 * i:8 * i + 8, :] = jnp.full((8, 128), float(i), f32)
    cp_x(0).wait()
    cp_mem0().wait()
    h0[0:MEM, :] = mem0_ref[...].astype(f32)
    mem0f[...] = mem0_ref[...].astype(f32)
    h0[MEM:LL, :] = _ln(xst[0:SEG, :].astype(f32))
    for s in range(nlead):
        xs = xst[SEG * (s + 1):SEG * (s + 1) + 16, :].astype(f32)
        h0[LL + 8 * s:LL + 8 * s + 8, :] = _ln(xs[0:8])

    def x_init(s):
        r = pl.ds(pl.multiple_of(s * SEG, SEG), SEG)
        xres[r, :] = xst[r, :].astype(f32)

    def x_body(i, c):
        for u in range(4):
            x_init(4 * i + u)
        return c
    jax.lax.fori_loop(0, (nlead + 1) // 4, x_body, 0)
    for s in range((nlead + 1) // 4 * 4, nlead + 1):
        x_init(s)

    lane = jax.lax.broadcasted_iota(jnp.int32, (LL, 128), 1)
    row = jax.lax.broadcasted_iota(jnp.int32, (LL, 128), 0)
    a_scale = DH ** -0.5 * LOG2E
    b_scale = BDH ** -0.5 * LOG2E
    lo = lane < 64
    first = lane < LL
    key = jnp.where(first, lane, lane - LL)
    valid = (lane < 2 * LL) & ((row < MEM) | (row >= key))
    m0 = valid & first
    m1 = valid & jnp.logical_not(first)

    def blk(t):
        z40 = jnp.zeros((LL, 128), f32)
        z48 = jnp.zeros((128 - 2 * LL, 128), f32)
        ta, tb, tc = t[:, 0:128], t[:, 128:256], t[:, 256:384]
        a = jnp.concatenate([ta, z40, z48], 0)
        b = jnp.concatenate([jnp.where(lo, tb, 0.), jnp.where(lo, 0., tb), z48], 0)
        c = jnp.concatenate([z40, tc, z48], 0)
        return jnp.concatenate([a, b, c], 1).astype(bf16)

    def scores(q, kmat):
        return jax.lax.dot_general(q, kmat, (((1,), (1,)), ((), ())), preferred_element_type=f32)

    def softmax(sc):
        sc = sc * a_scale
        mx0 = jnp.max(jnp.where(m0, sc, NEG), axis=1, keepdims=True)
        mx1 = jnp.max(jnp.where(m1, sc, NEG), axis=1, keepdims=True)
        p = jnp.where(valid, jnp.exp2(sc - jnp.where(first, mx0, mx1)), 0.)
        l0 = jnp.sum(jnp.where(first, p, 0.), axis=1, keepdims=True)
        l1 = jnp.sum(jnp.where(first, 0., p), axis=1, keepdims=True)
        return p * pl.reciprocal(jnp.where(first, l0, l1), approx=True)

    def pv(g, p, vmat):
        obuf[g] = jnp.dot(p, vmat, preferred_element_type=f32)

    def oproj(g0, g1, first=False):
        o = jnp.concatenate([obuf[g] for g in range(g0, g1)], axis=1)
        outs = []
        for c in range(5):
            if first:
                w = wo_st[c, g0 * PW:g1 * PW, :]
                wo[c, g0 * DH:g1 * DH, :] = pltpu.bitcast(w, u32)
            else:
                w = pltpu.bitcast(wo[c, g0 * DH:g1 * DH, :], bf16)
            outs.append(jnp.dot(o, w, preferred_element_type=f32))
        return jnp.concatenate(outs, axis=1)

    def a_finish(tau, p_last, vm_last, first):
        seg = tau & (nseg - 1)
        rows = pl.ds(pl.multiple_of(seg * SEG, SEG), SEG)
        nxt = (tau + 1) & (nseg - 1)
        if 'lnlate' not in OPT:
            hn[...] = _ln(xres[pl.ds(pl.multiple_of(nxt * SEG, SEG), SEG), :])
        r1 = oproj(0, OSPLIT, first)
        if 'lnlate' in OPT:
            hn[...] = _ln(xres[pl.ds(pl.multiple_of(nxt * SEG, SEG), SEG), :])
        if first:
            b_weights()
        pv(NP - 1, p_last, vm_last)
        res = r1 + oproj(OSPLIT, NP, first)
        if 'm0f' in OPT:
            mem[...] = jnp.where(seg == nseg - 1, mem0f[...], res[0:MEM])
        else:
            mem[...] = jnp.where(seg == nseg - 1, mem0_ref[...].astype(f32), res[0:MEM])
        xres[rows, :] = xres[rows, :] + res[MEM:LL]

    def a_steps(tau, mode):
        if mode == "short":
            prow = pl.ds(pl.multiple_of((tau - 1) * 8, 8), 8)

        def proj(g, j):
            cols = slice(j * PW, (j + 1) * PW)
            w = pltpu.bitcast((wq_even, wq_odd)[g % 2][g // 2, :, cols], bf16)
            if mode == "short":
                h = jnp.concatenate([mem[...], hn[8:SEG, :]], axis=0)
                y = jnp.dot(h, w, preferred_element_type=f32)
                return jnp.concatenate([y[0:MEM], pre[g, prow, cols], y[MEM:SEG]], axis=0)
            h = jnp.concatenate([mem[...], hn[...]], axis=0)
            return jnp.dot(h, w, preferred_element_type=f32)

        scs, vms, ps = {}, {}, {}
        for g in range(NP):
            kmat = blk(proj(g, 1))
            q = proj(g, 0)
            vms[g] = blk(proj(g, 2))
            if g >= 1:
                ps[g - 1] = softmax(scs.pop(g - 1))
            scs[g] = scores(q, kmat)
            if g >= 1:
                pv(g - 1, ps.pop(g - 1), vms.pop(g - 1))
            yield
        a_finish(tau, softmax(scs.pop(NP - 1)), vms.pop(NP - 1), False)

    def b_steps(tau):
        j = (tau - 1) & (nseg - 1)
        rows = pl.ds(pl.multiple_of(j * SEG, SEG), SEG)

        def bproj(t):
            return jnp.dot(hb[...], pltpu.bitcast(bw[:, t * DM:(t + 1) * DM], bf16),
                           preferred_element_type=f32)

        hb[...] = _ln(xres[rows, :])
        for c in range(5):
            kbuf[c, 0:16, :] = kbuf[c, SEG:SEG + 16, :]
            vbuf[c, 0:16, :] = vbuf[c, SEG:SEG + 16, :]
        yield
        qb[...] = bproj(0) * b_scale
        yield
        k = bproj(1)
        for c in range(5):
            kbuf[c, 16:16 + SEG, :] = k[:, c * 128:(c + 1) * 128]
        yield
        v = bproj(2)
        for c in range(5):
            vbuf[c, 16:16 + SEG, :] = v[:, c * 128:(c + 1) * 128]
        yield
        pos = jax.lax.broadcasted_iota(jnp.int32, (SEG, 128), 0) + j * SEG
        for w in range(BW):
            off = 16 - w * BDIL
            acc = qb[:, 0:128] * kbuf[0, off:off + SEG, :]
            for c in range(1, 5):
                acc = acc + qb[:, c * 128:(c + 1) * 128] * kbuf[c, off:off + SEG, :]
            acc = acc + pltpu.roll(acc, 64, 1)
            acc = acc + pltpu.roll(acc, 32, 1)
            if w > 0:
                acc = jnp.where(pos >= w * BDIL, acc, NEG)
            lg[w] = acc
            if w % 2 == 1:
                yield
        lgs = [lg[w] for w in range(BW)]
        mx = functools.reduce(jnp.maximum, lgs)
        es = [jnp.exp2(l - mx) for l in lgs]
        inv = pl.reciprocal(functools.reduce(jnp.add, es), approx=True)
        for w in range(BW):
            lg[w] = es[w] * inv
        yield
        for c in range(5):
            acc = None
            for w in range(BW):
                off = 16 - w * BDIL
                t = lg[w] * vbuf[c, off:off + SEG, :]
                acc = t if acc is None else acc + t
            qb[:, c * 128:(c + 1) * 128] = acc
            if c in (1, 3):
                yield
        yield
        x2 = xres[rows, :] + jnp.dot(qb[...], pltpu.bitcast(bwo[...], bf16), preferred_element_type=f32)
        xres[rows, :] = x2
        outv[rows, :] = x2.astype(bf16)

    def out_copy(j, n):
        r = pl.ds(pl.multiple_of(j * SEG, SEG), n * SEG)
        return pltpu.make_async_copy(outv.at[r, :], out_hbm.at[r, :], out_sem)

    def tick(tau, mode):
        live = [b_steps(tau), a_steps(tau, mode)]
        if 'ab' in OPT:
            live = live[::-1]
        if 'b1' in OPT:
            next(live[1] if 'ab' not in OPT else live[0])
        if 'b2' in OPT:
            next(live[1] if 'ab' not in OPT else live[0])
            next(live[1] if 'ab' not in OPT else live[0])
        while live:
            for gen in list(live):
                try:
                    next(gen)
                except StopIteration:
                    live.remove(gen)

    def w_wait(g):
        pltpu.make_async_copy(wst.at[g], wst.at[g], sems.at[8 + g]).wait()

    def stage(g, dst, slot, t):
        j, r = divmod(t, 3)
        dst[slot, :, t * 128:(t + 1) * 128] = pltpu.bitcast(wst[g, j, r * 128:(r + 1) * 128, :].T, u32)

    def first_pair(g, cur, cur_slot, nxt, nxt_slot, sc_prev, vm_prev):
        gp = (g + NP - 1) & (NP - 1)
        gn = jnp.minimum(g + 1, NP - 1)

        m0 = h0.shape[0]

        def proj(t, nsplit=1):
            cols = slice(t * 128, (t + 1) * 128)
            w = pltpu.bitcast(cur[cur_slot, :, cols], bf16)
            cuts = [8 * ((m0 // 8 * i) // nsplit) for i in range(nsplit + 1)]
            assert cuts[1] >= LL
            head = None
            for r0, r1 in zip(cuts[:-1], cuts[1:]):
                y = jnp.dot(h0[r0:r1, :], w, preferred_element_type=f32)
                if r0 == 0:
                    head, y, r0 = y[0:LL], y[LL:], LL
                pre[g, r0 - LL:r1 - LL, cols] = y
            return head

        def step(t, nsplit=1):
            y = proj(t, nsplit)
            stage(gn, nxt, nxt_slot, (t + 6) % 9)
            return y

        kmat = blk(jnp.concatenate([step(t) for t in (3, 4, 5)], axis=1))
        p = softmax(sc_prev)
        q = jnp.concatenate([step(t) for t in (0, 1, 2)], axis=1)
        v01 = [step(6), step(7)]
        sc = scores(q, kmat)
        pv(gp, p, vm_prev)
        vm = blk(jnp.concatenate(v01 + [step(8, 4)], axis=1))
        return sc, vm

    w_wait(0)
    for t in range(9):
        stage(0, wq_even, 0, t)

    def first_body(i, carry):
        w_wait(2 * i + 1)
        carry = first_pair(2 * i, wq_even, i, wq_odd, i, *carry)

        @pl.when(2 * i + 2 < NP)
        def _():
            w_wait(2 * i + 2)
        return first_pair(2 * i + 1, wq_odd, i, wq_even, i + 1, *carry)
    sc_last, vm_last = jax.lax.fori_loop(
        0, NP // 2, first_body, (jnp.zeros((LL, 128), f32), jnp.zeros((128, PW), bf16)))
    p_last = softmax(sc_last)

    def b_weights():
        for ft in range(3 * DM // 128):
            w = pltpu.bitcast(bst[:, ft * 128:(ft + 1) * 128], u32)
            for kc in range(3):
                t = w[kc * 128:(kc + 1) * 128, :]
                if kc == 2:
                    t = jnp.concatenate([t, jnp.zeros((64, 128), u32)], 0)
                tq[kc, ft * 128:(ft + 1) * 128, :] = t.T
        for j in range(3):
            for t in range(5):
                for kc in range(3):
                    rows = [tq[kc, pl.ds(j * DM + 4 * t + dd, NH, stride=BDH), :] for dd in range(4)]
                    gt = jnp.concatenate(rows, 0).T
                    n = 128 if kc < 2 else 64
                    bw[kc * 128:kc * 128 + n, j * DM + t * 128:j * DM + (t + 1) * 128] = gt[0:n]
        for c5 in range(5):
            to[c5] = bwo_st[:, c5 * 128:(c5 + 1) * 128].astype(f32)
        for c5 in range(5):
            for t in range(5):
                rows = [to[c5, pl.ds(4 * t + dd, NH, stride=BDH), :] for dd in range(4)]
                gt = jnp.concatenate(rows, 0).astype(bf16)
                bwo[t * 64:(t + 1) * 64, c5 * 128:(c5 + 1) * 128] = pltpu.bitcast(gt, u32)

    cp_b().wait()
    cp_bo().wait()
    for cpy in cp_wo():
        cpy.wait()
    a_finish(0, p_last, vm_last, True)

    cp_x(1).wait()

    def short_body(tau, c):
        tick(tau, "short")
        x_init(jnp.minimum(nlead + tau, nseg - 1))
        return c
    jax.lax.fori_loop(1, nlead + 1, short_body, 0)

    un = UNROLL

    def body(it, c):
        tau = nlead + 1 + un * it
        for u in range(un):
            tick(tau + u, "normal")

        @pl.when(tau >= nseg + un)
        def _():
            out_copy(tau - nseg - un, un).start()
        return c
    assert (2 * nseg - nlead - 1) % un == 0 and nseg // 2 <= nlead < nseg
    jax.lax.fori_loop(0, (2 * nseg - nlead - 1) // un, body, 0)
    for _ in b_steps(2 * nseg):
        pass
    t0 = nlead + 1 + un * (-(-(nseg + un - nlead - 1) // un))
    if t0 - nseg - un > 0:
        pltpu.make_async_copy(outv.at[0:(t0 - nseg - un) * SEG, :], out_hbm.at[0:(t0 - nseg - un) * SEG, :], out_sem).start()
    out_copy(nseg - un, un).start()
    pltpu.make_async_copy(outv, out_hbm, out_sem).wait()


@functools.partial(jax.jit, static_argnames=("A_seg_len",))
def pallas_interleave_layers__memory_aug_recurrent_mem_tr__sliding_local_dilated__prompt_kernel(
    A_x, A_mem0, A_Wq, A_Wk, A_Wv, A_Wo, A_seg_len, B_x, B_wqkv, B_wo,
):
    del B_x
    B, S, Dm = A_x.shape
    assert B == 1 and Dm == DM and A_seg_len == SEG and S % SEG == 0
    nseg = S // SEG
    x = A_x.reshape(S, DM)
    mem0 = A_mem0.reshape(MEM, DM)
    wt = lambda w: jnp.transpose(w, (1, 2, 0)).reshape(NH * DH, DM)
    any_spec = pl.BlockSpec(memory_space=pl.ANY)
    out = pl.pallas_call(
        functools.partial(_kernel, nseg=nseg, nlead=NLEAD),
        out_shape=jax.ShapeDtypeStruct((S, DM), A_x.dtype),
        in_specs=[any_spec] * 8,
        out_specs=any_spec,
        scratch_shapes=[
            pltpu.VMEM((PAD0 * 8, 128), f32),
            pltpu.VMEM((S, DM), bf16),
            pltpu.VMEM((MEM, DM), bf16),
            pltpu.VMEM((NP, 3, PW, DM), bf16),
            pltpu.VMEM((5, NH * DH, 128), bf16),
            pltpu.VMEM((DM, 3 * DM), bf16),
            pltpu.VMEM((DM, DM), bf16),
            pltpu.VMEM((3, 3 * DM, 128), u32),
            pltpu.VMEM((5, DM, 128), f32),
            pltpu.VMEM((NP // 2 + 1, DM // 2, 3 * PW), u32),
            pltpu.VMEM((NP // 2, DM // 2, 3 * PW), u32),
            pltpu.VMEM((5, NH * DH // 2, 128), u32),
            pltpu.VMEM((DM // 2, 3 * DM), u32),
            pltpu.VMEM((DM // 2, DM), u32),
            pltpu.VMEM((S, DM), f32),
            pltpu.VMEM((MEM, DM), f32),
            pltpu.VMEM((MEM, DM), f32),
            pltpu.VMEM((SEG, DM), f32),
            pltpu.VMEM((LL + 8 * NLEAD, DM), f32),
            pltpu.VMEM((NP, 8 * NLEAD, 3 * PW), f32),
            pltpu.VMEM((NP, LL, PW), f32),
            pltpu.VMEM((5, 16 + SEG, 128), f32),
            pltpu.VMEM((5, 16 + SEG, 128), f32),
            pltpu.VMEM((SEG, DM), f32),
            pltpu.VMEM((SEG, DM), f32),
            pltpu.VMEM((BW, SEG, 128), f32),
            pltpu.VMEM((S, DM), bf16),
            pltpu.SemaphoreType.DMA((10 + NP,)),
            pltpu.SemaphoreType.DMA(()),
        ],
        compiler_params=pltpu.CompilerParams(vmem_limit_bytes=124 * 1024 * 1024),
    )(x, mem0, wt(A_Wq), wt(A_Wk), wt(A_Wv), A_Wo.reshape(NH * DH, DM), B_wqkv, B_wo)
    return out.reshape(B, S, DM)
```

```python
import functools

import jax
import jax.numpy as jnp
import jax.experimental.pallas as pl
import jax.experimental.pallas.tpu as pltpu

f32 = jnp.float32
bf16 = jnp.bfloat16
u32 = jnp.uint32

DM = 640
NH = 32
DH = 192
NP = NH // 2
PW = 2 * DH
MEM = 8
SEG = 32
LL = MEM + SEG
BDH = DM // NH
BW, BDIL = 8, 2
LOG2E = 1.4426950408889634
EPS = 1e-5
NEG = -1e30
import os
PAD0 = int(os.environ.get('PAD0', '1'))
T_S, T_P, T_O = [int(v) for v in os.environ.get('TSPO', '0,2,4').split(',')]
OPT = os.environ.get('OPT', '')
OSPLIT = int(os.environ.get('OSPLIT', '8'))
import os
UNROLL = int(os.environ.get('UNROLL', '2'))
NLEAD = int(os.environ.get('NLEAD', '35'))


def _ln(x):
    m = jnp.mean(x, axis=-1, keepdims=True)
    d = x - m
    v = jnp.mean(d * d, axis=-1, keepdims=True)
    return d * jax.lax.rsqrt(v + EPS)


def _kernel(x_hbm, mem0_hbm, wq_hbm, wk_hbm, wv_hbm, wo_hbm, bqkv_hbm, bwo_hbm,
            out_hbm,
            pad0, xst, xhead, xlead, mem0_ref, wst, wo_st, bst, bwo_st, tq, to,
            wq_even, wq_odd, wo, bw, bwo, xres, mem, mem0f, hn, h0, pre, obuf, kbuf, vbuf, hb, qb, lg, outv,
            sems, out_sem, *, nseg, nlead):
    def cp_mem0():
        return pltpu.make_async_copy(mem0_hbm, mem0_ref, sems.at[0])

    def cp_xhead():
        return pltpu.make_async_copy(x_hbm.at[0:2], xhead, sems.at[8 + NP])

    def cp_xlead():
        return pltpu.make_async_copy(x_hbm.at[1:nlead + 1, 0:8, :], xlead, sems.at[9 + NP])

    def cp_x():
        return pltpu.make_async_copy(x_hbm, xst, sems.at[10 + NP])

    def cp_b():
        return pltpu.make_async_copy(bqkv_hbm, bst, sems.at[1])

    def cp_bo():
        return pltpu.make_async_copy(bwo_hbm, bwo_st, sems.at[2])

    def cp_w(g, j):
        w = (wq_hbm, wk_hbm, wv_hbm)[j]
        return pltpu.make_async_copy(w.at[pl.ds(g * PW, PW), :], wst.at[g, j], sems.at[8 + g])

    def cp_wo():
        return [pltpu.make_async_copy(wo_hbm.at[:, pl.ds(c * 128, 128)], wo_st.at[c], sems.at[3 + c])
                for c in range(5)]

    for cpy in ([cp_xlead(), cp_xhead(), cp_mem0()] + [cp_w(g, j) for g in range(NP) for j in (1, 0, 2)]
                + [cp_b(), cp_bo()] + cp_wo() + [cp_x()]):
        cpy.start()

    kbuf[...] = jnp.zeros(kbuf.shape, f32)
    vbuf[...] = jnp.zeros(vbuf.shape, f32)
    for i in range(PAD0):
        pad0[8 * i:8 * i + 8, :] = jnp.full((8, 128), float(i), f32)
    cp_xlead().wait()
    cp_xhead().wait()
    cp_mem0().wait()
    h0[0:MEM, :] = mem0_ref[...].astype(f32)
    mem0f[...] = mem0_ref[...].astype(f32)
    for s in range(2):
        xres[s * SEG:(s + 1) * SEG, :] = xhead[s].astype(f32)
    h0[MEM:LL, :] = _ln(xhead[0].astype(f32))
    for s in range(nlead):
        h0[LL + 8 * s:LL + 8 * s + 8, :] = _ln(xlead[s].astype(f32))

    def x_init(s):
        xres[pl.ds(pl.multiple_of(s * SEG, SEG), SEG), :] = xst[s].astype(f32)

    lane = jax.lax.broadcasted_iota(jnp.int32, (LL, 128), 1)
    row = jax.lax.broadcasted_iota(jnp.int32, (LL, 128), 0)
    a_scale = DH ** -0.5 * LOG2E
    b_scale = BDH ** -0.5 * LOG2E
    lo = lane < 64
    first = lane < LL
    key = jnp.where(first, lane, lane - LL)
    valid = (lane < 2 * LL) & ((row < MEM) | (row >= key))
    m0 = valid & first
    m1 = valid & jnp.logical_not(first)

    def blk(t):
        z40 = jnp.zeros((LL, 128), f32)
        z48 = jnp.zeros((128 - 2 * LL, 128), f32)
        ta, tb, tc = t[:, 0:128], t[:, 128:256], t[:, 256:384]
        a = jnp.concatenate([ta, z40, z48], 0)
        b = jnp.concatenate([jnp.where(lo, tb, 0.), jnp.where(lo, 0., tb), z48], 0)
        c = jnp.concatenate([z40, tc, z48], 0)
        return jnp.concatenate([a, b, c], 1).astype(bf16)

    def scores(q, kmat):
        return jax.lax.dot_general(q, kmat, (((1,), (1,)), ((), ())), preferred_element_type=f32)

    def softmax(sc):
        sc = sc * a_scale
        mx0 = jnp.max(jnp.where(m0, sc, NEG), axis=1, keepdims=True)
        mx1 = jnp.max(jnp.where(m1, sc, NEG), axis=1, keepdims=True)
        p = jnp.where(valid, jnp.exp2(sc - jnp.where(first, mx0, mx1)), 0.)
        l0 = jnp.sum(jnp.where(first, p, 0.), axis=1, keepdims=True)
        l1 = jnp.sum(jnp.where(first, 0., p), axis=1, keepdims=True)
        return p * pl.reciprocal(jnp.where(first, l0, l1), approx=True)

    def pv(g, p, vmat):
        obuf[g] = jnp.dot(p, vmat, preferred_element_type=f32)

    def oproj(g0, g1, first=False):
        o = jnp.concatenate([obuf[g] for g in range(g0, g1)], axis=1)
        outs = []
        for c in range(5):
            if first:
                w = wo_st[c, g0 * PW:g1 * PW, :]
                wo[c, g0 * DH:g1 * DH, :] = pltpu.bitcast(w, u32)
            else:
                w = pltpu.bitcast(wo[c, g0 * DH:g1 * DH, :], bf16)
            outs.append(jnp.dot(o, w, preferred_element_type=f32))
        return jnp.concatenate(outs, axis=1)

    def a_finish(tau, p_last, vm_last, first):
        seg = tau & (nseg - 1)
        rows = pl.ds(pl.multiple_of(seg * SEG, SEG), SEG)
        nxt = (tau + 1) & (nseg - 1)
        if 'lnlate' not in OPT:
            hn[...] = _ln(xres[pl.ds(pl.multiple_of(nxt * SEG, SEG), SEG), :])
        r1 = oproj(0, OSPLIT, first)
        if 'lnlate' in OPT:
            hn[...] = _ln(xres[pl.ds(pl.multiple_of(nxt * SEG, SEG), SEG), :])
        if first:
            b_weights()
        pv(NP - 1, p_last, vm_last)
        res = r1 + oproj(OSPLIT, NP, first)
        if 'm0f' in OPT:
            mem[...] = jnp.where(seg == nseg - 1, mem0f[...], res[0:MEM])
        else:
            mem[...] = jnp.where(seg == nseg - 1, mem0_ref[...].astype(f32), res[0:MEM])
        xres[rows, :] = xres[rows, :] + res[MEM:LL]

    def a_steps(tau, mode):
        if mode == "short":
            prow = pl.ds(pl.multiple_of((tau - 1) * 8, 8), 8)

        def proj(g, j):
            cols = slice(j * PW, (j + 1) * PW)
            w = pltpu.bitcast((wq_even, wq_odd)[g % 2][g // 2, :, cols], bf16)
            if mode == "short":
                h = jnp.concatenate([mem[...], hn[8:SEG, :]], axis=0)
                y = jnp.dot(h, w, preferred_element_type=f32)
                return jnp.concatenate([y[0:MEM], pre[g, prow, cols], y[MEM:SEG]], axis=0)
            h = jnp.concatenate([mem[...], hn[...]], axis=0)
            return jnp.dot(h, w, preferred_element_type=f32)

        scs, vms, ps = {}, {}, {}
        for g in range(NP):
            kmat = blk(proj(g, 1))
            q = proj(g, 0)
            vms[g] = blk(proj(g, 2))
            if g >= 1:
                ps[g - 1] = softmax(scs.pop(g - 1))
            scs[g] = scores(q, kmat)
            if g >= 1:
                pv(g - 1, ps.pop(g - 1), vms.pop(g - 1))
            yield
        a_finish(tau, softmax(scs.pop(NP - 1)), vms.pop(NP - 1), False)

    def b_steps(tau):
        j = (tau - 1) & (nseg - 1)
        rows = pl.ds(pl.multiple_of(j * SEG, SEG), SEG)

        def bproj(t):
            return jnp.dot(hb[...], pltpu.bitcast(bw[:, t * DM:(t + 1) * DM], bf16),
                           preferred_element_type=f32)

        hb[...] = _ln(xres[rows, :])
        for c in range(5):
            kbuf[c, 0:16, :] = kbuf[c, SEG:SEG + 16, :]
            vbuf[c, 0:16, :] = vbuf[c, SEG:SEG + 16, :]
        yield
        qb[...] = bproj(0) * b_scale
        yield
        k = bproj(1)
        for c in range(5):
            kbuf[c, 16:16 + SEG, :] = k[:, c * 128:(c + 1) * 128]
        yield
        v = bproj(2)
        for c in range(5):
            vbuf[c, 16:16 + SEG, :] = v[:, c * 128:(c + 1) * 128]
        yield
        pos = jax.lax.broadcasted_iota(jnp.int32, (SEG, 128), 0) + j * SEG
        for w in range(BW):
            off = 16 - w * BDIL
            acc = qb[:, 0:128] * kbuf[0, off:off + SEG, :]
            for c in range(1, 5):
                acc = acc + qb[:, c * 128:(c + 1) * 128] * kbuf[c, off:off + SEG, :]
            acc = acc + pltpu.roll(acc, 64, 1)
            acc = acc + pltpu.roll(acc, 32, 1)
            if w > 0:
                acc = jnp.where(pos >= w * BDIL, acc, NEG)
            lg[w] = acc
            if w % 2 == 1:
                yield
        lgs = [lg[w] for w in range(BW)]
        mx = functools.reduce(jnp.maximum, lgs)
        es = [jnp.exp2(l - mx) for l in lgs]
        inv = pl.reciprocal(functools.reduce(jnp.add, es), approx=True)
        for w in range(BW):
            lg[w] = es[w] * inv
        yield
        for c in range(5):
            acc = None
            for w in range(BW):
                off = 16 - w * BDIL
                t = lg[w] * vbuf[c, off:off + SEG, :]
                acc = t if acc is None else acc + t
            qb[:, c * 128:(c + 1) * 128] = acc
            if c in (1, 3):
                yield
        yield
        x2 = xres[rows, :] + jnp.dot(qb[...], pltpu.bitcast(bwo[...], bf16), preferred_element_type=f32)
        xres[rows, :] = x2
        outv[rows, :] = x2.astype(bf16)

    def out_copy(j, n):
        r = pl.ds(pl.multiple_of(j * SEG, SEG), n * SEG)
        return pltpu.make_async_copy(outv.at[r, :], out_hbm.at[r, :], out_sem)

    def tick(tau, mode):
        live = [b_steps(tau), a_steps(tau, mode)]
        if 'ab' in OPT:
            live = live[::-1]
        if 'b1' in OPT:
            next(live[1] if 'ab' not in OPT else live[0])
        if 'b2' in OPT:
            next(live[1] if 'ab' not in OPT else live[0])
            next(live[1] if 'ab' not in OPT else live[0])
        while live:
            for gen in list(live):
                try:
                    next(gen)
                except StopIteration:
                    live.remove(gen)

    def w_wait(g):
        pltpu.make_async_copy(wst.at[g], wst.at[g], sems.at[8 + g]).wait()

    def stage(g, dst, slot, t):
        j, r = divmod(t, 3)
        dst[slot, :, t * 128:(t + 1) * 128] = pltpu.bitcast(wst[g, j, r * 128:(r + 1) * 128, :].T, u32)

    def first_pair(g, cur, cur_slot, nxt, nxt_slot, sc_prev, vm_prev):
        gp = (g + NP - 1) & (NP - 1)
        gn = jnp.minimum(g + 1, NP - 1)

        m0 = h0.shape[0]

        def proj(t, nsplit=1):
            cols = slice(t * 128, (t + 1) * 128)
            w = pltpu.bitcast(cur[cur_slot, :, cols], bf16)
            cuts = [8 * ((m0 // 8 * i) // nsplit) for i in range(nsplit + 1)]
            assert cuts[1] >= LL
            head = None
            for r0, r1 in zip(cuts[:-1], cuts[1:]):
                y = jnp.dot(h0[r0:r1, :], w, preferred_element_type=f32)
                if r0 == 0:
                    head, y, r0 = y[0:LL], y[LL:], LL
                pre[g, r0 - LL:r1 - LL, cols] = y
            return head

        def step(t, nsplit=1):
            y = proj(t, nsplit)
            stage(gn, nxt, nxt_slot, (t + 6) % 9)
            return y

        kmat = blk(jnp.concatenate([step(t) for t in (3, 4, 5)], axis=1))
        p = softmax(sc_prev)
        q = jnp.concatenate([step(t) for t in (0, 1, 2)], axis=1)
        v01 = [step(6), step(7)]
        sc = scores(q, kmat)
        pv(gp, p, vm_prev)
        vm = blk(jnp.concatenate(v01 + [step(8, 4)], axis=1))
        return sc, vm

    w_wait(0)
    for t in range(9):
        stage(0, wq_even, 0, t)

    def first_body(i, carry):
        w_wait(2 * i + 1)
        carry = first_pair(2 * i, wq_even, i, wq_odd, i, *carry)

        @pl.when(2 * i + 2 < NP)
        def _():
            w_wait(2 * i + 2)
        return first_pair(2 * i + 1, wq_odd, i, wq_even, i + 1, *carry)
    sc_last, vm_last = jax.lax.fori_loop(
        0, NP // 2, first_body, (jnp.zeros((LL, 128), f32), jnp.zeros((128, PW), bf16)))
    p_last = softmax(sc_last)

    def b_weights():
        for ft in range(3 * DM // 128):
            w = pltpu.bitcast(bst[:, ft * 128:(ft + 1) * 128], u32)
            for kc in range(3):
                t = w[kc * 128:(kc + 1) * 128, :]
                if kc == 2:
                    t = jnp.concatenate([t, jnp.zeros((64, 128), u32)], 0)
                tq[kc, ft * 128:(ft + 1) * 128, :] = t.T
        for j in range(3):
            for t in range(5):
                for kc in range(3):
                    rows = [tq[kc, pl.ds(j * DM + 4 * t + dd, NH, stride=BDH), :] for dd in range(4)]
                    gt = jnp.concatenate(rows, 0).T
                    n = 128 if kc < 2 else 64
                    bw[kc * 128:kc * 128 + n, j * DM + t * 128:j * DM + (t + 1) * 128] = gt[0:n]
        for c5 in range(5):
            to[c5] = bwo_st[:, c5 * 128:(c5 + 1) * 128].astype(f32)
        for c5 in range(5):
            for t in range(5):
                rows = [to[c5, pl.ds(4 * t + dd, NH, stride=BDH), :] for dd in range(4)]
                gt = jnp.concatenate(rows, 0).astype(bf16)
                bwo[t * 64:(t + 1) * 64, c5 * 128:(c5 + 1) * 128] = pltpu.bitcast(gt, u32)

    cp_b().wait()
    cp_bo().wait()
    for cpy in cp_wo():
        cpy.wait()
    a_finish(0, p_last, vm_last, True)

    cp_x().wait()

    def short_body(tau, c):
        x_init(tau + 1)
        x_init(jnp.minimum(nlead + 1 + tau, nseg - 1))
        tick(tau, "short")
        return c
    jax.lax.fori_loop(1, nlead + 1, short_body, 0)

    un = UNROLL

    def body(it, c):
        tau = nlead + 1 + un * it
        for u in range(un):
            tick(tau + u, "normal")

        @pl.when(tau >= nseg + un)
        def _():
            out_copy(tau - nseg - un, un).start()
        return c
    assert (2 * nseg - nlead - 1) % un == 0 and 2 * nlead + 1 >= nseg - 1 and nlead < nseg
    jax.lax.fori_loop(0, (2 * nseg - nlead - 1) // un, body, 0)
    for _ in b_steps(2 * nseg):
        pass
    t0 = nlead + 1 + un * (-(-(nseg + un - nlead - 1) // un))
    if t0 - nseg - un > 0:
        pltpu.make_async_copy(outv.at[0:(t0 - nseg - un) * SEG, :], out_hbm.at[0:(t0 - nseg - un) * SEG, :], out_sem).start()
    out_copy(nseg - un, un).start()
    pltpu.make_async_copy(outv, out_hbm, out_sem).wait()


@functools.partial(jax.jit, static_argnames=("A_seg_len",))
def pallas_interleave_layers__memory_aug_recurrent_mem_tr__sliding_local_dilated__prompt_kernel(
    A_x, A_mem0, A_Wq, A_Wk, A_Wv, A_Wo, A_seg_len, B_x, B_wqkv, B_wo,
):
    del B_x
    B, S, Dm = A_x.shape
    assert B == 1 and Dm == DM and A_seg_len == SEG and S % SEG == 0
    nseg = S // SEG
    x = A_x.reshape(nseg, SEG, DM)
    mem0 = A_mem0.reshape(MEM, DM)
    wt = lambda w: jnp.transpose(w, (1, 2, 0)).reshape(NH * DH, DM)
    any_spec = pl.BlockSpec(memory_space=pl.ANY)
    out = pl.pallas_call(
        functools.partial(_kernel, nseg=nseg, nlead=NLEAD),
        out_shape=jax.ShapeDtypeStruct((S, DM), A_x.dtype),
        in_specs=[any_spec] * 8,
        out_specs=any_spec,
        scratch_shapes=[
            pltpu.VMEM((PAD0 * 8, 128), f32),
            pltpu.VMEM((nseg, SEG, DM), bf16),
            pltpu.VMEM((2, SEG, DM), bf16),
            pltpu.VMEM((NLEAD, 8, DM), bf16),
            pltpu.VMEM((MEM, DM), bf16),
            pltpu.VMEM((NP, 3, PW, DM), bf16),
            pltpu.VMEM((5, NH * DH, 128), bf16),
            pltpu.VMEM((DM, 3 * DM), bf16),
            pltpu.VMEM((DM, DM), bf16),
            pltpu.VMEM((3, 3 * DM, 128), u32),
            pltpu.VMEM((5, DM, 128), f32),
            pltpu.VMEM((NP // 2 + 1, DM // 2, 3 * PW), u32),
            pltpu.VMEM((NP // 2, DM // 2, 3 * PW), u32),
            pltpu.VMEM((5, NH * DH // 2, 128), u32),
            pltpu.VMEM((DM // 2, 3 * DM), u32),
            pltpu.VMEM((DM // 2, DM), u32),
            pltpu.VMEM((S, DM), f32),
            pltpu.VMEM((MEM, DM), f32),
            pltpu.VMEM((MEM, DM), f32),
            pltpu.VMEM((SEG, DM), f32),
            pltpu.VMEM((LL + 8 * NLEAD, DM), f32),
            pltpu.VMEM((NP, 8 * NLEAD, 3 * PW), f32),
            pltpu.VMEM((NP, LL, PW), f32),
            pltpu.VMEM((5, 16 + SEG, 128), f32),
            pltpu.VMEM((5, 16 + SEG, 128), f32),
            pltpu.VMEM((SEG, DM), f32),
            pltpu.VMEM((SEG, DM), f32),
            pltpu.VMEM((BW, SEG, 128), f32),
            pltpu.VMEM((S, DM), bf16),
            pltpu.SemaphoreType.DMA((11 + NP,)),
            pltpu.SemaphoreType.DMA(()),
        ],
        compiler_params=pltpu.CompilerParams(vmem_limit_bytes=124 * 1024 * 1024),
    )(x, mem0, wt(A_Wq), wt(A_Wk), wt(A_Wv), A_Wo.reshape(NH * DH, DM), B_wqkv, B_wo)
    return out.reshape(B, S, DM)
```

```python
import functools

import jax
import jax.numpy as jnp
import jax.experimental.pallas as pl
import jax.experimental.pallas.tpu as pltpu

f32 = jnp.float32
bf16 = jnp.bfloat16
u32 = jnp.uint32

DM = 640
NH = 32
DH = 192
NP = NH // 2
PW = 2 * DH
MEM = 8
SEG = 32
LL = MEM + SEG
BDH = DM // NH
BW, BDIL = 8, 2
LOG2E = 1.4426950408889634
EPS = 1e-5
NEG = -1e30
import os
PAD0 = int(os.environ.get('PAD0', '1'))
T_S, T_P, T_O = [int(v) for v in os.environ.get('TSPO', '0,2,4').split(',')]
OPT = os.environ.get('OPT', '')
OSPLIT = int(os.environ.get('OSPLIT', '8'))
FSPLIT = [int(c) for c in os.environ.get('FSPLIT', '111111114')]
FPOS = int(os.environ.get('FPOS', '2'))
import os
UNROLL = int(os.environ.get('UNROLL', '2'))
NLEAD = int(os.environ.get('NLEAD', '35'))


def _ln(x):
    m = jnp.mean(x, axis=-1, keepdims=True)
    d = x - m
    v = jnp.mean(d * d, axis=-1, keepdims=True)
    return d * jax.lax.rsqrt(v + EPS)


def _kernel(x_hbm, mem0_hbm, wq_hbm, wk_hbm, wv_hbm, wo_hbm, bqkv_hbm, bwo_hbm,
            out_hbm,
            pad0, xst, xhead, xlead, mem0_ref, wst, wo_st, bst, bwo_st, tq, to,
            wq_even, wq_odd, wo, bw, bwo, xres, mem, mem0f, hn, h0, pre, obuf, kbuf, vbuf, hb, qb, lg, outv,
            sems, out_sem, *, nseg, nlead):
    def cp_mem0():
        return pltpu.make_async_copy(mem0_hbm, mem0_ref, sems.at[0])

    def cp_xhead():
        return pltpu.make_async_copy(x_hbm.at[0:2], xhead, sems.at[8 + NP])

    def cp_xlead():
        return pltpu.make_async_copy(x_hbm.at[1:nlead + 1, 0:8, :], xlead, sems.at[9 + NP])

    def cp_x():
        return pltpu.make_async_copy(x_hbm, xst, sems.at[10 + NP])

    def cp_b():
        return pltpu.make_async_copy(bqkv_hbm, bst, sems.at[1])

    def cp_bo():
        return pltpu.make_async_copy(bwo_hbm, bwo_st, sems.at[2])

    def cp_w(g, j):
        w = (wq_hbm, wk_hbm, wv_hbm)[j]
        return pltpu.make_async_copy(w.at[pl.ds(g * PW, PW), :], wst.at[g, j], sems.at[8 + g])

    def cp_wo():
        return [pltpu.make_async_copy(wo_hbm.at[:, pl.ds(c * 128, 128)], wo_st.at[c], sems.at[3 + c])
                for c in range(5)]

    for cpy in ([cp_xlead(), cp_xhead(), cp_mem0()] + [cp_w(g, j) for g in range(NP) for j in (1, 0, 2)]
                + [cp_b(), cp_bo()] + cp_wo() + [cp_x()]):
        cpy.start()

    kbuf[...] = jnp.zeros(kbuf.shape, f32)
    vbuf[...] = jnp.zeros(vbuf.shape, f32)
    for i in range(PAD0):
        pad0[8 * i:8 * i + 8, :] = jnp.full((8, 128), float(i), f32)
    cp_xlead().wait()
    cp_xhead().wait()
    cp_mem0().wait()
    h0[0:MEM, :] = mem0_ref[...].astype(f32)
    mem0f[...] = mem0_ref[...].astype(f32)
    for s in range(2):
        xres[s * SEG:(s + 1) * SEG, :] = xhead[s].astype(f32)
    h0[MEM:LL, :] = _ln(xhead[0].astype(f32))
    for s in range(nlead):
        h0[LL + 8 * s:LL + 8 * s + 8, :] = _ln(xlead[s].astype(f32))

    def x_init(s):
        xres[pl.ds(pl.multiple_of(s * SEG, SEG), SEG), :] = xst[s].astype(f32)

    lane = jax.lax.broadcasted_iota(jnp.int32, (LL, 128), 1)
    row = jax.lax.broadcasted_iota(jnp.int32, (LL, 128), 0)
    a_scale = DH ** -0.5 * LOG2E
    b_scale = BDH ** -0.5 * LOG2E
    lo = lane < 64
    first = lane < LL
    key = jnp.where(first, lane, lane - LL)
    valid = (lane < 2 * LL) & ((row < MEM) | (row >= key))
    m0 = valid & first
    m1 = valid & jnp.logical_not(first)

    def blk(t):
        z40 = jnp.zeros((LL, 128), f32)
        z48 = jnp.zeros((128 - 2 * LL, 128), f32)
        ta, tb, tc = t[:, 0:128], t[:, 128:256], t[:, 256:384]
        a = jnp.concatenate([ta, z40, z48], 0)
        b = jnp.concatenate([jnp.where(lo, tb, 0.), jnp.where(lo, 0., tb), z48], 0)
        c = jnp.concatenate([z40, tc, z48], 0)
        return jnp.concatenate([a, b, c], 1).astype(bf16)

    def scores(q, kmat):
        return jax.lax.dot_general(q, kmat, (((1,), (1,)), ((), ())), preferred_element_type=f32)

    def softmax(sc):
        sc = sc * a_scale
        mx0 = jnp.max(jnp.where(m0, sc, NEG), axis=1, keepdims=True)
        mx1 = jnp.max(jnp.where(m1, sc, NEG), axis=1, keepdims=True)
        p = jnp.where(valid, jnp.exp2(sc - jnp.where(first, mx0, mx1)), 0.)
        l0 = jnp.sum(jnp.where(first, p, 0.), axis=1, keepdims=True)
        l1 = jnp.sum(jnp.where(first, 0., p), axis=1, keepdims=True)
        return p * pl.reciprocal(jnp.where(first, l0, l1), approx=True)

    def pv(g, p, vmat):
        obuf[g] = jnp.dot(p, vmat, preferred_element_type=f32)

    def oproj(g0, g1, first=False):
        o = jnp.concatenate([obuf[g] for g in range(g0, g1)], axis=1)
        outs = []
        for c in range(5):
            if first:
                w = wo_st[c, g0 * PW:g1 * PW, :]
                wo[c, g0 * DH:g1 * DH, :] = pltpu.bitcast(w, u32)
            else:
                w = pltpu.bitcast(wo[c, g0 * DH:g1 * DH, :], bf16)
            outs.append(jnp.dot(o, w, preferred_element_type=f32))
        return jnp.concatenate(outs, axis=1)

    def a_finish(tau, p_last, vm_last, first):
        seg = tau & (nseg - 1)
        rows = pl.ds(pl.multiple_of(seg * SEG, SEG), SEG)
        nxt = (tau + 1) & (nseg - 1)
        if 'lnlate' not in OPT:
            hn[...] = _ln(xres[pl.ds(pl.multiple_of(nxt * SEG, SEG), SEG), :])
        r1 = oproj(0, OSPLIT, first)
        if 'lnlate' in OPT:
            hn[...] = _ln(xres[pl.ds(pl.multiple_of(nxt * SEG, SEG), SEG), :])
        pv(NP - 1, p_last, vm_last)
        res = r1 + oproj(OSPLIT, NP, first)
        if 'm0f' in OPT:
            mem[...] = jnp.where(seg == nseg - 1, mem0f[...], res[0:MEM])
        else:
            mem[...] = jnp.where(seg == nseg - 1, mem0_ref[...].astype(f32), res[0:MEM])
        xres[rows, :] = xres[rows, :] + res[MEM:LL]

    def a_steps(tau, mode):
        if mode == "short":
            prow = pl.ds(pl.multiple_of((tau - 1) * 8, 8), 8)

        def proj(g, j):
            cols = slice(j * PW, (j + 1) * PW)
            w = pltpu.bitcast((wq_even, wq_odd)[g % 2][g // 2, :, cols], bf16)
            if mode == "short":
                h = jnp.concatenate([mem[...], hn[8:SEG, :]], axis=0)
                y = jnp.dot(h, w, preferred_element_type=f32)
                return jnp.concatenate([y[0:MEM], pre[g, prow, cols], y[MEM:SEG]], axis=0)
            h = jnp.concatenate([mem[...], hn[...]], axis=0)
            return jnp.dot(h, w, preferred_element_type=f32)

        scs, vms, ps = {}, {}, {}
        for g in range(NP):
            kmat = blk(proj(g, 1))
            q = proj(g, 0)
            vms[g] = blk(proj(g, 2))
            if g >= 1:
                ps[g - 1] = softmax(scs.pop(g - 1))
            scs[g] = scores(q, kmat)
            if g >= 1:
                pv(g - 1, ps.pop(g - 1), vms.pop(g - 1))
            yield
        a_finish(tau, softmax(scs.pop(NP - 1)), vms.pop(NP - 1), False)

    def b_steps(tau):
        j = (tau - 1) & (nseg - 1)
        rows = pl.ds(pl.multiple_of(j * SEG, SEG), SEG)

        def bproj(t):
            return jnp.dot(hb[...], pltpu.bitcast(bw[:, t * DM:(t + 1) * DM], bf16),
                           preferred_element_type=f32)

        hb[...] = _ln(xres[rows, :])
        for c in range(5):
            kbuf[c, 0:16, :] = kbuf[c, SEG:SEG + 16, :]
            vbuf[c, 0:16, :] = vbuf[c, SEG:SEG + 16, :]
        yield
        qb[...] = bproj(0) * b_scale
        yield
        k = bproj(1)
        for c in range(5):
            kbuf[c, 16:16 + SEG, :] = k[:, c * 128:(c + 1) * 128]
        yield
        v = bproj(2)
        for c in range(5):
            vbuf[c, 16:16 + SEG, :] = v[:, c * 128:(c + 1) * 128]
        yield
        pos = jax.lax.broadcasted_iota(jnp.int32, (SEG, 128), 0) + j * SEG
        for w in range(BW):
            off = 16 - w * BDIL
            acc = qb[:, 0:128] * kbuf[0, off:off + SEG, :]
            for c in range(1, 5):
                acc = acc + qb[:, c * 128:(c + 1) * 128] * kbuf[c, off:off + SEG, :]
            acc = acc + pltpu.roll(acc, 64, 1)
            acc = acc + pltpu.roll(acc, 32, 1)
            if w > 0:
                acc = jnp.where(pos >= w * BDIL, acc, NEG)
            lg[w] = acc
            if w % 2 == 1:
                yield
        lgs = [lg[w] for w in range(BW)]
        mx = functools.reduce(jnp.maximum, lgs)
        es = [jnp.exp2(l - mx) for l in lgs]
        inv = pl.reciprocal(functools.reduce(jnp.add, es), approx=True)
        for w in range(BW):
            lg[w] = es[w] * inv
        yield
        for c in range(5):
            acc = None
            for w in range(BW):
                off = 16 - w * BDIL
                t = lg[w] * vbuf[c, off:off + SEG, :]
                acc = t if acc is None else acc + t
            qb[:, c * 128:(c + 1) * 128] = acc
            if c in (1, 3):
                yield
        yield
        x2 = xres[rows, :] + jnp.dot(qb[...], pltpu.bitcast(bwo[...], bf16), preferred_element_type=f32)
        xres[rows, :] = x2
        outv[rows, :] = x2.astype(bf16)

    def out_copy(j, n):
        r = pl.ds(pl.multiple_of(j * SEG, SEG), n * SEG)
        return pltpu.make_async_copy(outv.at[r, :], out_hbm.at[r, :], out_sem)

    def tick(tau, mode):
        live = [b_steps(tau), a_steps(tau, mode)]
        if 'ab' in OPT:
            live = live[::-1]
        if 'b1' in OPT:
            next(live[1] if 'ab' not in OPT else live[0])
        if 'b2' in OPT:
            next(live[1] if 'ab' not in OPT else live[0])
            next(live[1] if 'ab' not in OPT else live[0])
        while live:
            for gen in list(live):
                try:
                    next(gen)
                except StopIteration:
                    live.remove(gen)

    def w_wait(g):
        pltpu.make_async_copy(wst.at[g], wst.at[g], sems.at[8 + g]).wait()

    def stage(g, dst, slot, t):
        j, r = divmod(t, 3)
        dst[slot, :, t * 128:(t + 1) * 128] = pltpu.bitcast(wst[g, j, r * 128:(r + 1) * 128, :].T, u32)

    def first_pair(g, cur, cur_slot, nxt, nxt_slot, sc_prev, vm_prev):
        gp = (g + NP - 1) & (NP - 1)
        gn = jnp.minimum(g + 1, NP - 1)

        m0 = h0.shape[0]

        def proj(t, nsplit=1):
            cols = slice(t * 128, (t + 1) * 128)
            w = pltpu.bitcast(cur[cur_slot, :, cols], bf16)
            cuts = [8 * ((m0 // 8 * i) // nsplit) for i in range(nsplit + 1)]
            assert cuts[1] >= LL
            head = None
            for r0, r1 in zip(cuts[:-1], cuts[1:]):
                y = jnp.dot(h0[r0:r1, :], w, preferred_element_type=f32)
                if r0 == 0:
                    head, y, r0 = y[0:LL], y[LL:], LL
                pre[g, r0 - LL:r1 - LL, cols] = y
            return head

        def step(t, nsplit=1):
            y = proj(t, nsplit)
            stage(gn, nxt, nxt_slot, (t + 6) % 9)
            return y

        fs = FSPLIT
        kmat = blk(jnp.concatenate([step(t, fs[t]) for t in (3, 4, 5)], axis=1))
        p = softmax(sc_prev)
        q = jnp.concatenate([step(t, fs[t]) for t in (0, 1, 2)], axis=1)
        vs = [step(t, fs[t]) for t in range(6, 6 + FPOS)]
        if 'pvfirst' in OPT:
            pv(gp, p, vm_prev)
            sc = scores(q, kmat)
        else:
            sc = scores(q, kmat)
            pv(gp, p, vm_prev)
        vm = blk(jnp.concatenate(vs + [step(t, fs[t]) for t in range(6 + FPOS, 9)], axis=1))
        return sc, vm

    w_wait(0)
    for t in range(9):
        stage(0, wq_even, 0, t)

    def first_body(i, carry):
        w_wait(2 * i + 1)
        carry = first_pair(2 * i, wq_even, i, wq_odd, i, *carry)

        @pl.when(2 * i + 2 < NP)
        def _():
            w_wait(2 * i + 2)
        return first_pair(2 * i + 1, wq_odd, i, wq_even, i + 1, *carry)
    sc_last, vm_last = jax.lax.fori_loop(
        0, NP // 2, first_body, (jnp.zeros((LL, 128), f32), jnp.zeros((128, PW), bf16)))
    p_last = softmax(sc_last)

    def b_weights():
        for ft in range(3 * DM // 128):
            w = pltpu.bitcast(bst[:, ft * 128:(ft + 1) * 128], u32)
            for kc in range(3):
                t = w[kc * 128:(kc + 1) * 128, :]
                if kc == 2:
                    t = jnp.concatenate([t, jnp.zeros((64, 128), u32)], 0)
                tq[kc, ft * 128:(ft + 1) * 128, :] = t.T
        for j in range(3):
            for t in range(5):
                for kc in range(3):
                    rows = [tq[kc, pl.ds(j * DM + 4 * t + dd, NH, stride=BDH), :] for dd in range(4)]
                    gt = jnp.concatenate(rows, 0).T
                    n = 128 if kc < 2 else 64
                    bw[kc * 128:kc * 128 + n, j * DM + t * 128:j * DM + (t + 1) * 128] = gt[0:n]
        for c5 in range(5):
            to[c5] = bwo_st[:, c5 * 128:(c5 + 1) * 128].astype(f32)
        for c5 in range(5):
            for t in range(5):
                rows = [to[c5, pl.ds(4 * t + dd, NH, stride=BDH), :] for dd in range(4)]
                gt = jnp.concatenate(rows, 0).astype(bf16)
                bwo[t * 64:(t + 1) * 64, c5 * 128:(c5 + 1) * 128] = pltpu.bitcast(gt, u32)

    cp_b().wait()
    cp_bo().wait()
    b_weights()
    for cpy in cp_wo():
        cpy.wait()
    a_finish(0, p_last, vm_last, True)

    cp_x().wait()

    def short_body(tau, c):
        x_init(tau + 1)
        x_init(jnp.minimum(nlead + 1 + tau, nseg - 1))
        tick(tau, "short")
        return c
    jax.lax.fori_loop(1, nlead + 1, short_body, 0)

    un = UNROLL

    def body(it, c):
        tau = nlead + 1 + un * it
        for u in range(un):
            tick(tau + u, "normal")

        @pl.when(tau >= nseg + un)
        def _():
            out_copy(tau - nseg - un, un).start()
        return c
    assert (2 * nseg - nlead - 1) % un == 0 and 2 * nlead + 1 >= nseg - 1 and nlead < nseg
    jax.lax.fori_loop(0, (2 * nseg - nlead - 1) // un, body, 0)
    for _ in b_steps(2 * nseg):
        pass
    t0 = nlead + 1 + un * (-(-(nseg + un - nlead - 1) // un))
    if t0 - nseg - un > 0:
        pltpu.make_async_copy(outv.at[0:(t0 - nseg - un) * SEG, :], out_hbm.at[0:(t0 - nseg - un) * SEG, :], out_sem).start()
    out_copy(nseg - un, un).start()
    pltpu.make_async_copy(outv, out_hbm, out_sem).wait()


@functools.partial(jax.jit, static_argnames=("A_seg_len",))
def pallas_interleave_layers__memory_aug_recurrent_mem_tr__sliding_local_dilated__prompt_kernel(
    A_x, A_mem0, A_Wq, A_Wk, A_Wv, A_Wo, A_seg_len, B_x, B_wqkv, B_wo,
):
    del B_x
    B, S, Dm = A_x.shape
    assert B == 1 and Dm == DM and A_seg_len == SEG and S % SEG == 0
    nseg = S // SEG
    x = A_x.reshape(nseg, SEG, DM)
    mem0 = A_mem0.reshape(MEM, DM)
    wt = lambda w: jnp.transpose(w, (1, 2, 0)).reshape(NH * DH, DM)
    any_spec = pl.BlockSpec(memory_space=pl.ANY)
    out = pl.pallas_call(
        functools.partial(_kernel, nseg=nseg, nlead=NLEAD),
        out_shape=jax.ShapeDtypeStruct((S, DM), A_x.dtype),
        in_specs=[any_spec] * 8,
        out_specs=any_spec,
        scratch_shapes=[
            pltpu.VMEM((PAD0 * 8, 128), f32),
            pltpu.VMEM((nseg, SEG, DM), bf16),
            pltpu.VMEM((2, SEG, DM), bf16),
            pltpu.VMEM((NLEAD, 8, DM), bf16),
            pltpu.VMEM((MEM, DM), bf16),
            pltpu.VMEM((NP, 3, PW, DM), bf16),
            pltpu.VMEM((5, NH * DH, 128), bf16),
            pltpu.VMEM((DM, 3 * DM), bf16),
            pltpu.VMEM((DM, DM), bf16),
            pltpu.VMEM((3, 3 * DM, 128), u32),
            pltpu.VMEM((5, DM, 128), f32),
            pltpu.VMEM((NP // 2 + 1, DM // 2, 3 * PW), u32),
            pltpu.VMEM((NP // 2, DM // 2, 3 * PW), u32),
            pltpu.VMEM((5, NH * DH // 2, 128), u32),
            pltpu.VMEM((DM // 2, 3 * DM), u32),
            pltpu.VMEM((DM // 2, DM), u32),
            pltpu.VMEM((S, DM), f32),
            pltpu.VMEM((MEM, DM), f32),
            pltpu.VMEM((MEM, DM), f32),
            pltpu.VMEM((SEG, DM), f32),
            pltpu.VMEM((LL + 8 * NLEAD, DM), f32),
            pltpu.VMEM((NP, 8 * NLEAD, 3 * PW), f32),
            pltpu.VMEM((NP, LL, PW), f32),
            pltpu.VMEM((5, 16 + SEG, 128), f32),
            pltpu.VMEM((5, 16 + SEG, 128), f32),
            pltpu.VMEM((SEG, DM), f32),
            pltpu.VMEM((SEG, DM), f32),
            pltpu.VMEM((BW, SEG, 128), f32),
            pltpu.VMEM((S, DM), bf16),
            pltpu.SemaphoreType.DMA((11 + NP,)),
            pltpu.SemaphoreType.DMA(()),
        ],
        compiler_params=pltpu.CompilerParams(vmem_limit_bytes=124 * 1024 * 1024),
    )(x, mem0, wt(A_Wq), wt(A_Wk), wt(A_Wv), A_Wo.reshape(NH * DH, DM), B_wqkv, B_wo)
    return out.reshape(B, S, DM)
```

```python
import functools

import jax
import jax.numpy as jnp
import jax.experimental.pallas as pl
import jax.experimental.pallas.tpu as pltpu

f32 = jnp.float32
bf16 = jnp.bfloat16
u32 = jnp.uint32

DM = 640
NH = 32
DH = 192
NP = NH // 2
PW = 2 * DH
MEM = 8
SEG = 32
LL = MEM + SEG
BDH = DM // NH
BW, BDIL = 8, 2
LOG2E = 1.4426950408889634
EPS = 1e-5
NEG = -1e30
import os
PAD0 = int(os.environ.get('PAD0', '1'))
T_S, T_P, T_O = [int(v) for v in os.environ.get('TSPO', '0,2,4').split(',')]
OPT = os.environ.get('OPT', '')
OSPLIT = int(os.environ.get('OSPLIT', '8'))
FSPLIT = [int(c) for c in os.environ.get('FSPLIT', '111111114')]
FPOS = int(os.environ.get('FPOS', '2'))
import os
UNROLL = int(os.environ.get('UNROLL', '2'))
NLEAD = int(os.environ.get('NLEAD', '35'))


def _ln(x):
    m = jnp.mean(x, axis=-1, keepdims=True)
    d = x - m
    v = jnp.mean(d * d, axis=-1, keepdims=True)
    return d * jax.lax.rsqrt(v + EPS)


def _kernel(x_hbm, mem0_hbm, wq_hbm, wk_hbm, wv_hbm, wo_hbm, bqkv_hbm, bwo_hbm,
            out_hbm,
            pad0, xst, xlead, mem0_ref, wst, wo_st, bst, bwo_st, tq, to,
            wq_even, wq_odd, wo, bw, bwo, xres, mem, mem0f, hn, h0, pre, obuf, kbuf, vbuf, hb, qb, lg, outv,
            sems, out_sem, *, nseg, nlead):
    def cp_mem0():
        return pltpu.make_async_copy(mem0_hbm, mem0_ref, sems.at[0])

    def cp_xhead():
        return pltpu.make_async_copy(x_hbm.at[0:3], xst.at[0:3], sems.at[8 + NP])

    def cp_xlead():
        return pltpu.make_async_copy(x_hbm.at[1:nlead + 1, 0:8, :], xlead, sems.at[9 + NP])

    def cp_x():
        return pltpu.make_async_copy(x_hbm.at[3:nseg], xst.at[3:nseg], sems.at[10 + NP])

    def cp_b():
        return pltpu.make_async_copy(bqkv_hbm, bst, sems.at[1])

    def cp_bo():
        return pltpu.make_async_copy(bwo_hbm, bwo_st, sems.at[2])

    def cp_w(g, j):
        w = (wq_hbm, wk_hbm, wv_hbm)[j]
        return pltpu.make_async_copy(w.at[pl.ds(g * PW, PW), :], wst.at[g, j], sems.at[8 + g])

    def cp_wo():
        return [pltpu.make_async_copy(wo_hbm.at[:, pl.ds(c * 128, 128)], wo_st.at[c], sems.at[3 + c])
                for c in range(5)]

    for cpy in ([cp_xlead(), cp_xhead(), cp_mem0()] + [cp_w(g, j) for g in range(NP) for j in (1, 0, 2)]
                + [cp_b(), cp_bo()] + cp_wo() + [cp_x()]):
        cpy.start()

    kbuf[...] = jnp.zeros(kbuf.shape, f32)
    vbuf[...] = jnp.zeros(vbuf.shape, f32)
    for i in range(PAD0):
        pad0[8 * i:8 * i + 8, :] = jnp.full((8, 128), float(i), f32)
    cp_xlead().wait()
    cp_xhead().wait()
    cp_mem0().wait()
    h0[0:MEM, :] = mem0_ref[...].astype(f32)
    mem0f[...] = mem0_ref[...].astype(f32)
    for s in range(2):
        xres[s * SEG:(s + 1) * SEG, :] = xst[s].astype(f32)
    h0[MEM:LL, :] = _ln(xst[0].astype(f32))
    for s in range(nlead):
        h0[LL + 8 * s:LL + 8 * s + 8, :] = _ln(xlead[s].astype(f32))

    def x_init(s):
        xres[pl.ds(pl.multiple_of(s * SEG, SEG), SEG), :] = xst[s].astype(f32)

    lane = jax.lax.broadcasted_iota(jnp.int32, (LL, 128), 1)
    row = jax.lax.broadcasted_iota(jnp.int32, (LL, 128), 0)
    a_scale = DH ** -0.5 * LOG2E
    b_scale = BDH ** -0.5 * LOG2E
    lo = lane < 64
    first = lane < LL
    key = jnp.where(first, lane, lane - LL)
    valid = (lane < 2 * LL) & ((row < MEM) | (row >= key))
    m0 = valid & first
    m1 = valid & jnp.logical_not(first)

    def blk(t):
        z40 = jnp.zeros((LL, 128), f32)
        z48 = jnp.zeros((128 - 2 * LL, 128), f32)
        ta, tb, tc = t[:, 0:128], t[:, 128:256], t[:, 256:384]
        a = jnp.concatenate([ta, z40, z48], 0)
        b = jnp.concatenate([jnp.where(lo, tb, 0.), jnp.where(lo, 0., tb), z48], 0)
        c = jnp.concatenate([z40, tc, z48], 0)
        return jnp.concatenate([a, b, c], 1).astype(bf16)

    def scores(q, kmat):
        return jax.lax.dot_general(q, kmat, (((1,), (1,)), ((), ())), preferred_element_type=f32)

    def softmax(sc):
        sc = sc * a_scale
        mx0 = jnp.max(jnp.where(m0, sc, NEG), axis=1, keepdims=True)
        mx1 = jnp.max(jnp.where(m1, sc, NEG), axis=1, keepdims=True)
        p = jnp.where(valid, jnp.exp2(sc - jnp.where(first, mx0, mx1)), 0.)
        l0 = jnp.sum(jnp.where(first, p, 0.), axis=1, keepdims=True)
        l1 = jnp.sum(jnp.where(first, 0., p), axis=1, keepdims=True)
        return p * pl.reciprocal(jnp.where(first, l0, l1), approx=True)

    def pv(g, p, vmat):
        obuf[g] = jnp.dot(p, vmat, preferred_element_type=f32)

    def oproj(g0, g1, first=False):
        o = jnp.concatenate([obuf[g] for g in range(g0, g1)], axis=1)
        outs = []
        for c in range(5):
            if first:
                w = wo_st[c, g0 * PW:g1 * PW, :]
                wo[c, g0 * DH:g1 * DH, :] = pltpu.bitcast(w, u32)
            else:
                w = pltpu.bitcast(wo[c, g0 * DH:g1 * DH, :], bf16)
            outs.append(jnp.dot(o, w, preferred_element_type=f32))
        return jnp.concatenate(outs, axis=1)

    def a_finish(tau, p_last, vm_last, first):
        seg = tau & (nseg - 1)
        rows = pl.ds(pl.multiple_of(seg * SEG, SEG), SEG)
        nxt = (tau + 1) & (nseg - 1)
        if 'lnlate' not in OPT:
            hn[...] = _ln(xres[pl.ds(pl.multiple_of(nxt * SEG, SEG), SEG), :])
        r1 = oproj(0, OSPLIT, first)
        if 'lnlate' in OPT:
            hn[...] = _ln(xres[pl.ds(pl.multiple_of(nxt * SEG, SEG), SEG), :])
        pv(NP - 1, p_last, vm_last)
        res = r1 + oproj(OSPLIT, NP, first)
        if 'm0f' in OPT:
            mem[...] = jnp.where(seg == nseg - 1, mem0f[...], res[0:MEM])
        else:
            mem[...] = jnp.where(seg == nseg - 1, mem0_ref[...].astype(f32), res[0:MEM])
        xres[rows, :] = xres[rows, :] + res[MEM:LL]

    def a_steps(tau, mode):
        if mode == "short":
            prow = pl.ds(pl.multiple_of((tau - 1) * 8, 8), 8)

        def proj(g, j):
            cols = slice(j * PW, (j + 1) * PW)
            w = pltpu.bitcast((wq_even, wq_odd)[g % 2][g // 2, :, cols], bf16)
            if mode == "short":
                h = jnp.concatenate([mem[...], hn[8:SEG, :]], axis=0)
                y = jnp.dot(h, w, preferred_element_type=f32)
                return jnp.concatenate([y[0:MEM], pre[g, prow, cols], y[MEM:SEG]], axis=0)
            h = jnp.concatenate([mem[...], hn[...]], axis=0)
            return jnp.dot(h, w, preferred_element_type=f32)

        scs, vms, ps = {}, {}, {}
        for g in range(NP):
            kmat = blk(proj(g, 1))
            q = proj(g, 0)
            vms[g] = blk(proj(g, 2))
            if g >= 1:
                ps[g - 1] = softmax(scs.pop(g - 1))
            scs[g] = scores(q, kmat)
            if g >= 1:
                pv(g - 1, ps.pop(g - 1), vms.pop(g - 1))
            yield
        a_finish(tau, softmax(scs.pop(NP - 1)), vms.pop(NP - 1), False)

    def b_steps(tau):
        j = (tau - 1) & (nseg - 1)
        rows = pl.ds(pl.multiple_of(j * SEG, SEG), SEG)

        def bproj(t):
            return jnp.dot(hb[...], pltpu.bitcast(bw[:, t * DM:(t + 1) * DM], bf16),
                           preferred_element_type=f32)

        hb[...] = _ln(xres[rows, :])
        for c in range(5):
            kbuf[c, 0:16, :] = kbuf[c, SEG:SEG + 16, :]
            vbuf[c, 0:16, :] = vbuf[c, SEG:SEG + 16, :]
        yield
        qb[...] = bproj(0) * b_scale
        yield
        k = bproj(1)
        for c in range(5):
            kbuf[c, 16:16 + SEG, :] = k[:, c * 128:(c + 1) * 128]
        yield
        v = bproj(2)
        for c in range(5):
            vbuf[c, 16:16 + SEG, :] = v[:, c * 128:(c + 1) * 128]
        yield
        pos = jax.lax.broadcasted_iota(jnp.int32, (SEG, 128), 0) + j * SEG
        for w in range(BW):
            off = 16 - w * BDIL
            acc = qb[:, 0:128] * kbuf[0, off:off + SEG, :]
            for c in range(1, 5):
                acc = acc + qb[:, c * 128:(c + 1) * 128] * kbuf[c, off:off + SEG, :]
            acc = acc + pltpu.roll(acc, 64, 1)
            acc = acc + pltpu.roll(acc, 32, 1)
            if w > 0:
                acc = jnp.where(pos >= w * BDIL, acc, NEG)
            lg[w] = acc
            if w % 2 == 1:
                yield
        lgs = [lg[w] for w in range(BW)]
        mx = functools.reduce(jnp.maximum, lgs)
        es = [jnp.exp2(l - mx) for l in lgs]
        inv = pl.reciprocal(functools.reduce(jnp.add, es), approx=True)
        for w in range(BW):
            lg[w] = es[w] * inv
        yield
        for c in range(5):
            acc = None
            for w in range(BW):
                off = 16 - w * BDIL
                t = lg[w] * vbuf[c, off:off + SEG, :]
                acc = t if acc is None else acc + t
            qb[:, c * 128:(c + 1) * 128] = acc
            if c in (1, 3):
                yield
        yield
        x2 = xres[rows, :] + jnp.dot(qb[...], pltpu.bitcast(bwo[...], bf16), preferred_element_type=f32)
        xres[rows, :] = x2
        outv[rows, :] = x2.astype(bf16)

    def out_copy(j, n):
        r = pl.ds(pl.multiple_of(j * SEG, SEG), n * SEG)
        return pltpu.make_async_copy(outv.at[r, :], out_hbm.at[r, :], out_sem)

    def tick(tau, mode):
        live = [b_steps(tau), a_steps(tau, mode)]
        if 'ab' in OPT:
            live = live[::-1]
        if 'b1' in OPT:
            next(live[1] if 'ab' not in OPT else live[0])
        if 'b2' in OPT:
            next(live[1] if 'ab' not in OPT else live[0])
            next(live[1] if 'ab' not in OPT else live[0])
        while live:
            for gen in list(live):
                try:
                    next(gen)
                except StopIteration:
                    live.remove(gen)

    def w_wait(g):
        pltpu.make_async_copy(wst.at[g], wst.at[g], sems.at[8 + g]).wait()

    def stage(g, dst, slot, t):
        j, r = divmod(t, 3)
        dst[slot, :, t * 128:(t + 1) * 128] = pltpu.bitcast(wst[g, j, r * 128:(r + 1) * 128, :].T, u32)

    def first_pair(g, cur, cur_slot, nxt, nxt_slot, sc_prev, vm_prev):
        gp = (g + NP - 1) & (NP - 1)
        gn = jnp.minimum(g + 1, NP - 1)

        m0 = h0.shape[0]

        def proj(t, nsplit=1):
            cols = slice(t * 128, (t + 1) * 128)
            w = pltpu.bitcast(cur[cur_slot, :, cols], bf16)
            cuts = [8 * ((m0 // 8 * i) // nsplit) for i in range(nsplit + 1)]
            assert cuts[1] >= LL
            head = None
            for r0, r1 in zip(cuts[:-1], cuts[1:]):
                y = jnp.dot(h0[r0:r1, :], w, preferred_element_type=f32)
                if r0 == 0:
                    head, y, r0 = y[0:LL], y[LL:], LL
                pre[g, r0 - LL:r1 - LL, cols] = y
            return head

        def step(t, nsplit=1):
            y = proj(t, nsplit)
            stage(gn, nxt, nxt_slot, (t + 6) % 9)
            return y

        fs = FSPLIT
        kmat = blk(jnp.concatenate([step(t, fs[t]) for t in (3, 4, 5)], axis=1))
        p = softmax(sc_prev)
        q = jnp.concatenate([step(t, fs[t]) for t in (0, 1, 2)], axis=1)
        vs = [step(t, fs[t]) for t in range(6, 6 + FPOS)]
        if 'pvfirst' in OPT:
            pv(gp, p, vm_prev)
            sc = scores(q, kmat)
        else:
            sc = scores(q, kmat)
            pv(gp, p, vm_prev)
        vm = blk(jnp.concatenate(vs + [step(t, fs[t]) for t in range(6 + FPOS, 9)], axis=1))
        return sc, vm

    w_wait(0)
    for t in range(9):
        stage(0, wq_even, 0, t)

    def first_body(i, carry):
        w_wait(2 * i + 1)
        carry = first_pair(2 * i, wq_even, i, wq_odd, i, *carry)

        @pl.when(2 * i + 2 < NP)
        def _():
            w_wait(2 * i + 2)
        return first_pair(2 * i + 1, wq_odd, i, wq_even, i + 1, *carry)
    sc_last, vm_last = jax.lax.fori_loop(
        0, NP // 2, first_body, (jnp.zeros((LL, 128), f32), jnp.zeros((128, PW), bf16)))
    p_last = softmax(sc_last)

    def b_weights():
        for ft in range(3 * DM // 128):
            w = pltpu.bitcast(bst[:, ft * 128:(ft + 1) * 128], u32)
            for kc in range(3):
                t = w[kc * 128:(kc + 1) * 128, :]
                if kc == 2:
                    t = jnp.concatenate([t, jnp.zeros((64, 128), u32)], 0)
                tq[kc, ft * 128:(ft + 1) * 128, :] = t.T
        for j in range(3):
            for t in range(5):
                for kc in range(3):
                    rows = [tq[kc, pl.ds(j * DM + 4 * t + dd, NH, stride=BDH), :] for dd in range(4)]
                    gt = jnp.concatenate(rows, 0).T
                    n = 128 if kc < 2 else 64
                    bw[kc * 128:kc * 128 + n, j * DM + t * 128:j * DM + (t + 1) * 128] = gt[0:n]
        for c5 in range(5):
            to[c5] = bwo_st[:, c5 * 128:(c5 + 1) * 128].astype(f32)
        for c5 in range(5):
            for t in range(5):
                rows = [to[c5, pl.ds(4 * t + dd, NH, stride=BDH), :] for dd in range(4)]
                gt = jnp.concatenate(rows, 0).astype(bf16)
                bwo[t * 64:(t + 1) * 64, c5 * 128:(c5 + 1) * 128] = pltpu.bitcast(gt, u32)

    cp_b().wait()
    cp_bo().wait()
    b_weights()
    for cpy in cp_wo():
        cpy.wait()
    a_finish(0, p_last, vm_last, True)


    def short_body(tau, c):
        @pl.when(tau == 2)
        def _():
            cp_x().wait()
        x_init(tau + 1)
        x_init(jnp.where(tau == 1, 2, jnp.minimum(nlead + tau, nseg - 1)))
        tick(tau, "short")
        return c
    jax.lax.fori_loop(1, nlead + 1, short_body, 0)

    un = UNROLL

    def body(it, c):
        tau = nlead + 1 + un * it
        for u in range(un):
            tick(tau + u, "normal")

        @pl.when(tau >= nseg + un)
        def _():
            out_copy(tau - nseg - un, un).start()
        return c
    assert (2 * nseg - nlead - 1) % un == 0 and 2 * nlead >= nseg - 1 and 2 <= nlead < nseg
    jax.lax.fori_loop(0, (2 * nseg - nlead - 1) // un, body, 0)
    for _ in b_steps(2 * nseg):
        pass
    t0 = nlead + 1 + un * (-(-(nseg + un - nlead - 1) // un))
    if t0 - nseg - un > 0:
        pltpu.make_async_copy(outv.at[0:(t0 - nseg - un) * SEG, :], out_hbm.at[0:(t0 - nseg - un) * SEG, :], out_sem).start()
    out_copy(nseg - un, un).start()
    pltpu.make_async_copy(outv, out_hbm, out_sem).wait()


@functools.partial(jax.jit, static_argnames=("A_seg_len",))
def pallas_interleave_layers__memory_aug_recurrent_mem_tr__sliding_local_dilated__prompt_kernel(
    A_x, A_mem0, A_Wq, A_Wk, A_Wv, A_Wo, A_seg_len, B_x, B_wqkv, B_wo,
):
    del B_x
    B, S, Dm = A_x.shape
    assert B == 1 and Dm == DM and A_seg_len == SEG and S % SEG == 0
    nseg = S // SEG
    x = A_x.reshape(nseg, SEG, DM)
    mem0 = A_mem0.reshape(MEM, DM)
    wt = lambda w: jnp.transpose(w, (1, 2, 0)).reshape(NH * DH, DM)
    any_spec = pl.BlockSpec(memory_space=pl.ANY)
    out = pl.pallas_call(
        functools.partial(_kernel, nseg=nseg, nlead=NLEAD),
        out_shape=jax.ShapeDtypeStruct((S, DM), A_x.dtype),
        in_specs=[any_spec] * 8,
        out_specs=any_spec,
        scratch_shapes=[
            pltpu.VMEM((PAD0 * 8, 128), f32),
            pltpu.VMEM((nseg, SEG, DM), bf16),
            pltpu.VMEM((NLEAD, 8, DM), bf16),
            pltpu.VMEM((MEM, DM), bf16),
            pltpu.VMEM((NP, 3, PW, DM), bf16),
            pltpu.VMEM((5, NH * DH, 128), bf16),
            pltpu.VMEM((DM, 3 * DM), bf16),
            pltpu.VMEM((DM, DM), bf16),
            pltpu.VMEM((3, 3 * DM, 128), u32),
            pltpu.VMEM((5, DM, 128), f32),
            pltpu.VMEM((NP // 2 + 1, DM // 2, 3 * PW), u32),
            pltpu.VMEM((NP // 2, DM // 2, 3 * PW), u32),
            pltpu.VMEM((5, NH * DH // 2, 128), u32),
            pltpu.VMEM((DM // 2, 3 * DM), u32),
            pltpu.VMEM((DM // 2, DM), u32),
            pltpu.VMEM((S, DM), f32),
            pltpu.VMEM((MEM, DM), f32),
            pltpu.VMEM((MEM, DM), f32),
            pltpu.VMEM((SEG, DM), f32),
            pltpu.VMEM((LL + 8 * NLEAD, DM), f32),
            pltpu.VMEM((NP, 8 * NLEAD, 3 * PW), f32),
            pltpu.VMEM((NP, LL, PW), f32),
            pltpu.VMEM((5, 16 + SEG, 128), f32),
            pltpu.VMEM((5, 16 + SEG, 128), f32),
            pltpu.VMEM((SEG, DM), f32),
            pltpu.VMEM((SEG, DM), f32),
            pltpu.VMEM((BW, SEG, 128), f32),
            pltpu.VMEM((S, DM), bf16),
            pltpu.SemaphoreType.DMA((11 + NP,)),
            pltpu.SemaphoreType.DMA(()),
        ],
        compiler_params=pltpu.CompilerParams(vmem_limit_bytes=124 * 1024 * 1024),
    )(x, mem0, wt(A_Wq), wt(A_Wk), wt(A_Wv), A_Wo.reshape(NH * DH, DM), B_wqkv, B_wo)
    return out.reshape(B, S, DM)
```

```python
import functools

import jax
import jax.numpy as jnp
import jax.experimental.pallas as pl
import jax.experimental.pallas.tpu as pltpu

f32 = jnp.float32
bf16 = jnp.bfloat16
u32 = jnp.uint32

DM = 640
NH = 32
DH = 192
NP = NH // 2
PW = 2 * DH
MEM = 8
SEG = 32
LL = MEM + SEG
BDH = DM // NH
BW, BDIL = 8, 2
LOG2E = 1.4426950408889634
EPS = 1e-5
NEG = -1e30
NLEAD = 34
UNROLL = 3
OSPLIT = 4


def _ln(x):
    m = jnp.mean(x, axis=-1, keepdims=True)
    d = x - m
    v = jnp.mean(d * d, axis=-1, keepdims=True)
    return d * jax.lax.rsqrt(v + EPS)


def _kernel(x_hbm, mem0_hbm, wq_hbm, wk_hbm, wv_hbm, wo_hbm, bqkv_hbm, bwo_hbm,
            out_hbm,
            xst, xlead, mem0_st, wst, wo_st, bst, bwo_st, tq, to,
            wq_even, wq_odd, wo, bw, bwo, xres, mem, mem0f, hn, h0, pre, obuf,
            kbuf, vbuf, hb, qb, lg, outv,
            sems, out_sem, *, nseg, nlead):
    def cp_mem0():
        return pltpu.make_async_copy(mem0_hbm, mem0_st, sems.at[0])

    def cp_b():
        return pltpu.make_async_copy(bqkv_hbm, bst, sems.at[1])

    def cp_bo():
        return pltpu.make_async_copy(bwo_hbm, bwo_st, sems.at[2])

    def cp_wo():
        return [pltpu.make_async_copy(wo_hbm.at[:, pl.ds(c * 128, 128)], wo_st.at[c], sems.at[3 + c])
                for c in range(5)]

    def cp_w(g, j):
        w = (wq_hbm, wk_hbm, wv_hbm)[j]
        return pltpu.make_async_copy(w.at[pl.ds(g * PW, PW), :], wst.at[g, j], sems.at[8 + g])

    def w_wait(g):
        pltpu.make_async_copy(wst.at[g], wst.at[g], sems.at[8 + g]).wait()

    def cp_xhead():
        return pltpu.make_async_copy(x_hbm.at[0:3], xst.at[0:3], sems.at[8 + NP])

    def cp_xlead():
        return pltpu.make_async_copy(x_hbm.at[1:nlead + 1, 0:8, :], xlead, sems.at[9 + NP])

    def cp_x():
        return pltpu.make_async_copy(x_hbm.at[3:nseg], xst.at[3:nseg], sems.at[10 + NP])

    def out_copy(j, n):
        r = pl.ds(pl.multiple_of(j * SEG, SEG), n * SEG)
        return pltpu.make_async_copy(outv.at[r, :], out_hbm.at[r, :], out_sem)

    for cpy in ([cp_xlead(), cp_xhead(), cp_mem0()] + [cp_w(g, j) for g in range(NP) for j in (1, 0, 2)]
                + [cp_b(), cp_bo()] + cp_wo() + [cp_x()]):
        cpy.start()

    kbuf[...] = jnp.zeros(kbuf.shape, f32)
    vbuf[...] = jnp.zeros(vbuf.shape, f32)
    cp_xlead().wait()
    cp_xhead().wait()
    cp_mem0().wait()
    mem0f[...] = mem0_st[...].astype(f32)
    h0[0:MEM, :] = mem0_st[...].astype(f32)
    h0[MEM:LL, :] = _ln(xst[0].astype(f32))
    for s in range(nlead):
        h0[LL + 8 * s:LL + 8 * s + 8, :] = _ln(xlead[s].astype(f32))
    for s in range(2):
        xres[s * SEG:(s + 1) * SEG, :] = xst[s].astype(f32)

    def x_init(s):
        xres[pl.ds(pl.multiple_of(s * SEG, SEG), SEG), :] = xst[s].astype(f32)

    lane = jax.lax.broadcasted_iota(jnp.int32, (LL, 128), 1)
    row = jax.lax.broadcasted_iota(jnp.int32, (LL, 128), 0)
    a_scale = DH ** -0.5 * LOG2E
    b_scale = BDH ** -0.5 * LOG2E
    lo = lane < 64
    first = lane < LL
    key = jnp.where(first, lane, lane - LL)
    valid = (lane < 2 * LL) & ((row < MEM) | (row >= key))
    m0 = valid & first
    m1 = valid & jnp.logical_not(first)

    def blk(t):
        z40 = jnp.zeros((LL, 128), f32)
        z48 = jnp.zeros((128 - 2 * LL, 128), f32)
        ta, tb, tc = t[:, 0:128], t[:, 128:256], t[:, 256:384]
        a = jnp.concatenate([ta, z40, z48], 0)
        b = jnp.concatenate([jnp.where(lo, tb, 0.), jnp.where(lo, 0., tb), z48], 0)
        c = jnp.concatenate([z40, tc, z48], 0)
        return jnp.concatenate([a, b, c], 1).astype(bf16)

    def scores(q, kmat):
        return jax.lax.dot_general(q, kmat, (((1,), (1,)), ((), ())), preferred_element_type=f32)

    def softmax(sc):
        sc = sc * a_scale
        mx0 = jnp.max(jnp.where(m0, sc, NEG), axis=1, keepdims=True)
        mx1 = jnp.max(jnp.where(m1, sc, NEG), axis=1, keepdims=True)
        p = jnp.where(valid, jnp.exp2(sc - jnp.where(first, mx0, mx1)), 0.)
        l0 = jnp.sum(jnp.where(first, p, 0.), axis=1, keepdims=True)
        l1 = jnp.sum(jnp.where(first, 0., p), axis=1, keepdims=True)
        return p * pl.reciprocal(jnp.where(first, l0, l1), approx=True)

    def pv(g, p, vmat):
        obuf[g] = jnp.dot(p, vmat, preferred_element_type=f32)

    def oproj(g0, g1, first_step):
        o = jnp.concatenate([obuf[g] for g in range(g0, g1)], axis=1)
        outs = []
        for c in range(5):
            if first_step:
                w = wo_st[c, g0 * PW:g1 * PW, :]
                wo[c, g0 * DH:g1 * DH, :] = pltpu.bitcast(w, u32)
            else:
                w = pltpu.bitcast(wo[c, g0 * DH:g1 * DH, :], bf16)
            outs.append(jnp.dot(o, w, preferred_element_type=f32))
        return jnp.concatenate(outs, axis=1)

    def a_finish(tau, p_last, vm_last, first_step):
        seg = tau & (nseg - 1)
        rows = pl.ds(pl.multiple_of(seg * SEG, SEG), SEG)
        nxt = (tau + 1) & (nseg - 1)
        hn[...] = _ln(xres[pl.ds(pl.multiple_of(nxt * SEG, SEG), SEG), :])
        r1 = oproj(0, OSPLIT, first_step)
        pv(NP - 1, p_last, vm_last)
        res = r1 + oproj(OSPLIT, NP, first_step)
        mem[...] = jnp.where(seg == nseg - 1, mem0f[...], res[0:MEM])
        xres[rows, :] = xres[rows, :] + res[MEM:LL]

    def a_steps(tau, short):
        if short:
            prow = pl.ds(pl.multiple_of((tau - 1) * 8, 8), 8)

        def proj(g, j):
            cols = slice(j * PW, (j + 1) * PW)
            w = pltpu.bitcast((wq_even, wq_odd)[g % 2][g // 2, :, cols], bf16)
            if short:
                h = jnp.concatenate([mem[...], hn[8:SEG, :]], axis=0)
                y = jnp.dot(h, w, preferred_element_type=f32)
                return jnp.concatenate([y[0:MEM], pre[g, prow, cols], y[MEM:SEG]], axis=0)
            h = jnp.concatenate([mem[...], hn[...]], axis=0)
            return jnp.dot(h, w, preferred_element_type=f32)

        scs, vms, ps = {}, {}, {}
        for g in range(NP):
            kmat = blk(proj(g, 1))
            q = proj(g, 0)
            vms[g] = blk(proj(g, 2))
            if g >= 1:
                ps[g - 1] = softmax(scs.pop(g - 1))
            scs[g] = scores(q, kmat)
            if g >= 1:
                pv(g - 1, ps.pop(g - 1), vms.pop(g - 1))
            yield
        a_finish(tau, softmax(scs.pop(NP - 1)), vms.pop(NP - 1), False)

    def b_steps(tau):
        j = (tau - 1) & (nseg - 1)
        rows = pl.ds(pl.multiple_of(j * SEG, SEG), SEG)

        def bproj(t):
            return jnp.dot(hb[...], pltpu.bitcast(bw[:, t * DM:(t + 1) * DM], bf16),
                           preferred_element_type=f32)

        hb[...] = _ln(xres[rows, :])
        for c in range(5):
            kbuf[c, 0:16, :] = kbuf[c, SEG:SEG + 16, :]
            vbuf[c, 0:16, :] = vbuf[c, SEG:SEG + 16, :]
        yield
        qb[...] = bproj(0) * b_scale
        yield
        k = bproj(1)
        for c in range(5):
            kbuf[c, 16:16 + SEG, :] = k[:, c * 128:(c + 1) * 128]
        yield
        v = bproj(2)
        for c in range(5):
            vbuf[c, 16:16 + SEG, :] = v[:, c * 128:(c + 1) * 128]
        yield
        pos = jax.lax.broadcasted_iota(jnp.int32, (SEG, 128), 0) + j * SEG
        for w in range(BW):
            off = 16 - w * BDIL
            acc = qb[:, 0:128] * kbuf[0, off:off + SEG, :]
            for c in range(1, 5):
                acc = acc + qb[:, c * 128:(c + 1) * 128] * kbuf[c, off:off + SEG, :]
            acc = acc + pltpu.roll(acc, 64, 1)
            acc = acc + pltpu.roll(acc, 32, 1)
            if w > 0:
                acc = jnp.where(pos >= w * BDIL, acc, NEG)
            lg[w] = acc
            if w % 2 == 1:
                yield
        lgs = [lg[w] for w in range(BW)]
        mx = functools.reduce(jnp.maximum, lgs)
        es = [jnp.exp2(l - mx) for l in lgs]
        inv = pl.reciprocal(functools.reduce(jnp.add, es), approx=True)
        for w in range(BW):
            lg[w] = es[w] * inv
        yield
        for c in range(5):
            acc = None
            for w in range(BW):
                off = 16 - w * BDIL
                t = lg[w] * vbuf[c, off:off + SEG, :]
                acc = t if acc is None else acc + t
            qb[:, c * 128:(c + 1) * 128] = acc
            if c in (1, 3):
                yield
        yield
        x2 = xres[rows, :] + jnp.dot(qb[...], pltpu.bitcast(bwo[...], bf16), preferred_element_type=f32)
        xres[rows, :] = x2
        outv[rows, :] = x2.astype(bf16)

    def b_weights():
        for ft in range(3 * DM // 128):
            w = pltpu.bitcast(bst[:, ft * 128:(ft + 1) * 128], u32)
            for kc in range(3):
                t = w[kc * 128:(kc + 1) * 128, :]
                if kc == 2:
                    t = jnp.concatenate([t, jnp.zeros((64, 128), u32)], 0)
                tq[kc, ft * 128:(ft + 1) * 128, :] = t.T
        for j in range(3):
            for t in range(5):
                for kc in range(3):
                    rows = [tq[kc, pl.ds(j * DM + 4 * t + dd, NH, stride=BDH), :] for dd in range(4)]
                    gt = jnp.concatenate(rows, 0).T
                    n = 128 if kc < 2 else 64
                    bw[kc * 128:kc * 128 + n, j * DM + t * 128:j * DM + (t + 1) * 128] = gt[0:n]
        for c5 in range(5):
            to[c5] = bwo_st[:, c5 * 128:(c5 + 1) * 128].astype(f32)
        for c5 in range(5):
            for t in range(5):
                rows = [to[c5, pl.ds(4 * t + dd, NH, stride=BDH), :] for dd in range(4)]
                gt = jnp.concatenate(rows, 0).astype(bf16)
                bwo[t * 64:(t + 1) * 64, c5 * 128:(c5 + 1) * 128] = pltpu.bitcast(gt, u32)

    def tick(tau, short):
        live = [b_steps(tau), a_steps(tau, short)]
        while live:
            for gen in list(live):
                try:
                    next(gen)
                except StopIteration:
                    live.remove(gen)

    def stage(g, dst, slot, t):
        j, r = divmod(t, 3)
        dst[slot, :, t * 128:(t + 1) * 128] = pltpu.bitcast(wst[g, j, r * 128:(r + 1) * 128, :].T, u32)

    def first_pair(g, cur, cur_slot, nxt, nxt_slot, sc_prev, vm_prev):
        gp = (g + NP - 1) & (NP - 1)
        gn = jnp.minimum(g + 1, NP - 1)
        nrow = h0.shape[0]

        def step(t, nsplit=1):
            cols = slice(t * 128, (t + 1) * 128)
            w = pltpu.bitcast(cur[cur_slot, :, cols], bf16)
            cuts = [8 * ((nrow // 8 * i) // nsplit) for i in range(nsplit + 1)]
            head = None
            for r0, r1 in zip(cuts[:-1], cuts[1:]):
                y = jnp.dot(h0[r0:r1, :], w, preferred_element_type=f32)
                if r0 == 0:
                    head, y, r0 = y[0:LL], y[LL:], LL
                pre[g, r0 - LL:r1 - LL, cols] = y
            stage(gn, nxt, nxt_slot, (t + 6) % 9)
            return head

        kmat = blk(jnp.concatenate([step(t) for t in (3, 4, 5)], axis=1))
        p = softmax(sc_prev)
        q = jnp.concatenate([step(t) for t in (0, 1, 2)], axis=1)
        v01 = [step(6), step(7)]
        sc = scores(q, kmat)
        pv(gp, p, vm_prev)
        vm = blk(jnp.concatenate(v01 + [step(8, 4)], axis=1))
        return sc, vm

    w_wait(0)
    for t in range(9):
        stage(0, wq_even, 0, t)

    def first_body(i, carry):
        w_wait(2 * i + 1)
        carry = first_pair(2 * i, wq_even, i, wq_odd, i, *carry)

        @pl.when(2 * i + 2 < NP)
        def _():
            w_wait(2 * i + 2)
        return first_pair(2 * i + 1, wq_odd, i, wq_even, i + 1, *carry)
    sc_last, vm_last = jax.lax.fori_loop(
        0, NP // 2, first_body, (jnp.zeros((LL, 128), f32), jnp.zeros((128, PW), bf16)))
    p_last = softmax(sc_last)

    cp_b().wait()
    cp_bo().wait()
    b_weights()
    for cpy in cp_wo():
        cpy.wait()
    a_finish(0, p_last, vm_last, True)

    def short_body(tau, c):
        @pl.when(tau == 2)
        def _():
            cp_x().wait()
        x_init(tau + 1)
        x_init(jnp.where(tau == 1, 2, jnp.minimum(nlead + tau, nseg - 1)))
        tick(tau, True)
        return c
    jax.lax.fori_loop(1, nlead + 1, short_body, 0)

    un = UNROLL

    def body(it, c):
        tau = nlead + 1 + un * it
        for u in range(un):
            tick(tau + u, False)

        @pl.when(tau >= nseg + un)
        def _():
            out_copy(tau - nseg - un, un).start()
        return c
    jax.lax.fori_loop(0, (2 * nseg - nlead - 1) // un, body, 0)
    for _ in b_steps(2 * nseg):
        pass
    t0 = nlead + 1 + un * (-(-(nseg + un - nlead - 1) // un))
    if t0 - nseg - un > 0:
        head = pl.ds(0, (t0 - nseg - un) * SEG)
        pltpu.make_async_copy(outv.at[head, :], out_hbm.at[head, :], out_sem).start()
    out_copy(nseg - un, un).start()
    pltpu.make_async_copy(outv, out_hbm, out_sem).wait()


@functools.partial(jax.jit, static_argnames=("A_seg_len",))
def pallas_interleave_layers__memory_aug_recurrent_mem_tr__sliding_local_dilated__prompt_kernel(
    A_x, A_mem0, A_Wq, A_Wk, A_Wv, A_Wo, A_seg_len, B_x, B_wqkv, B_wo,
):
    del B_x
    B, S, Dm = A_x.shape
    nseg = S // SEG
    assert B == 1 and Dm == DM and A_seg_len == SEG and S == nseg * SEG and nseg & (nseg - 1) == 0
    assert A_mem0.shape == (1, MEM, DM) and A_Wq.shape == (DM, NH, DH) and A_Wo.shape == (NH, DH, DM)
    assert (2 * nseg - NLEAD - 1) % UNROLL == 0 and nseg - 1 <= 2 * NLEAD and 2 <= NLEAD < nseg
    x = A_x.reshape(nseg, SEG, DM)
    mem0 = A_mem0.reshape(MEM, DM)
    wt = lambda w: jnp.transpose(w, (1, 2, 0)).reshape(NH * DH, DM)
    any_spec = pl.BlockSpec(memory_space=pl.ANY)
    out = pl.pallas_call(
        functools.partial(_kernel, nseg=nseg, nlead=NLEAD),
        out_shape=jax.ShapeDtypeStruct((S, DM), A_x.dtype),
        in_specs=[any_spec] * 8,
        out_specs=any_spec,
        scratch_shapes=[
            pltpu.VMEM((nseg, SEG, DM), bf16),
            pltpu.VMEM((NLEAD, 8, DM), bf16),
            pltpu.VMEM((MEM, DM), bf16),
            pltpu.VMEM((NP, 3, PW, DM), bf16),
            pltpu.VMEM((5, NH * DH, 128), bf16),
            pltpu.VMEM((DM, 3 * DM), bf16),
            pltpu.VMEM((DM, DM), bf16),
            pltpu.VMEM((3, 3 * DM, 128), u32),
            pltpu.VMEM((5, DM, 128), f32),
            pltpu.VMEM((NP // 2 + 1, DM // 2, 3 * PW), u32),
            pltpu.VMEM((NP // 2, DM // 2, 3 * PW), u32),
            pltpu.VMEM((5, NH * DH // 2, 128), u32),
            pltpu.VMEM((DM // 2, 3 * DM), u32),
            pltpu.VMEM((DM // 2, DM), u32),
            pltpu.VMEM((S, DM), f32),
            pltpu.VMEM((MEM, DM), f32),
            pltpu.VMEM((MEM, DM), f32),
            pltpu.VMEM((SEG, DM), f32),
            pltpu.VMEM((LL + 8 * NLEAD, DM), f32),
            pltpu.VMEM((NP, 8 * NLEAD, 3 * PW), f32),
            pltpu.VMEM((NP, LL, PW), f32),
            pltpu.VMEM((5, 16 + SEG, 128), f32),
            pltpu.VMEM((5, 16 + SEG, 128), f32),
            pltpu.VMEM((SEG, DM), f32),
            pltpu.VMEM((SEG, DM), f32),
            pltpu.VMEM((BW, SEG, 128), f32),
            pltpu.VMEM((S, DM), bf16),
            pltpu.SemaphoreType.DMA((11 + NP,)),
            pltpu.SemaphoreType.DMA(()),
        ],
        compiler_params=pltpu.CompilerParams(vmem_limit_bytes=124 * 1024 * 1024),
    )(x, mem0, wt(A_Wq), wt(A_Wk), wt(A_Wv), A_Wo.reshape(NH * DH, DM), B_wqkv, B_wo)
    return out.reshape(B, S, DM)
```

```python
import functools

import jax
import jax.numpy as jnp
import jax.experimental.pallas as pl
import jax.experimental.pallas.tpu as pltpu

f32 = jnp.float32
bf16 = jnp.bfloat16
u32 = jnp.uint32

DM = 640
NH = 32
DH = 192
NP = NH // 2
PW = 2 * DH
MEM = 8
SEG = 32
LL = MEM + SEG
BDH = DM // NH
BW, BDIL = 8, 2
LOG2E = 1.4426950408889634
EPS = 1e-5
NEG = -1e30
NLEAD = 34
UNROLL = 3
OSPLIT = 4
BS_NORM = (0, 1, 2, 3, 4, 6, 8, 10, 12)
BS_SHORT = (2, 3, 4, 5, 7, 9, 11, 13, 15)


def _ln(x):
    m = jnp.mean(x, axis=-1, keepdims=True)
    d = x - m
    v = jnp.mean(d * d, axis=-1, keepdims=True)
    return d * jax.lax.rsqrt(v + EPS)


def _kernel(x_hbm, mem0_hbm, wq_hbm, wk_hbm, wv_hbm, wo_hbm, bqkv_hbm, bwo_hbm,
            out_hbm,
            xst, xlead, mem0_st, wst, wo_st, bst, bwo_st, tq, to,
            wq_even, wq_odd, wo, bw, bwo, xres, mem, mem0f, hn, h0, pre, obuf,
            kbuf, vbuf, hb, qb, outv,
            sems, out_sem, *, nseg, nlead):
    def cp_mem0():
        return pltpu.make_async_copy(mem0_hbm, mem0_st, sems.at[0])

    def cp_b():
        return pltpu.make_async_copy(bqkv_hbm, bst, sems.at[1])

    def cp_bo():
        return pltpu.make_async_copy(bwo_hbm, bwo_st, sems.at[2])

    def cp_wo():
        return [pltpu.make_async_copy(wo_hbm.at[:, pl.ds(c * 128, 128)], wo_st.at[c], sems.at[3 + c])
                for c in range(5)]

    def cp_w(g, j):
        w = (wq_hbm, wk_hbm, wv_hbm)[j]
        return pltpu.make_async_copy(w.at[pl.ds(g * PW, PW), :], wst.at[g, j], sems.at[8 + g])

    def w_wait(g):
        pltpu.make_async_copy(wst.at[g], wst.at[g], sems.at[8 + g]).wait()

    def cp_xhead():
        return pltpu.make_async_copy(x_hbm.at[0:3], xst.at[0:3], sems.at[8 + NP])

    def cp_xlead():
        return pltpu.make_async_copy(x_hbm.at[1:nlead + 1, 0:8, :], xlead, sems.at[9 + NP])

    def cp_x():
        return pltpu.make_async_copy(x_hbm.at[3:nseg], xst.at[3:nseg], sems.at[10 + NP])

    def out_copy(j, n):
        r = pl.ds(pl.multiple_of(j * SEG, SEG), n * SEG)
        return pltpu.make_async_copy(outv.at[r, :], out_hbm.at[r, :], out_sem)

    for cpy in ([cp_xlead(), cp_xhead(), cp_mem0()] + [cp_w(g, j) for g in range(NP) for j in (1, 0, 2)]
                + [cp_b(), cp_bo()] + cp_wo() + [cp_x()]):
        cpy.start()

    kbuf[...] = jnp.zeros(kbuf.shape, f32)
    vbuf[...] = jnp.zeros(vbuf.shape, f32)
    cp_xlead().wait()
    cp_xhead().wait()
    cp_mem0().wait()
    mem0f[...] = mem0_st[...].astype(f32)
    h0[0:MEM, :] = mem0_st[...].astype(f32)
    h0[MEM:LL, :] = _ln(xst[0].astype(f32))
    for s in range(nlead):
        h0[LL + 8 * s:LL + 8 * s + 8, :] = _ln(xlead[s].astype(f32))
    for s in range(2):
        xres[s * SEG:(s + 1) * SEG, :] = xst[s].astype(f32)

    def x_init(s):
        xres[pl.ds(pl.multiple_of(s * SEG, SEG), SEG), :] = xst[s].astype(f32)

    lane = jax.lax.broadcasted_iota(jnp.int32, (LL, 128), 1)
    row = jax.lax.broadcasted_iota(jnp.int32, (LL, 128), 0)
    a_scale = DH ** -0.5 * LOG2E
    b_scale = BDH ** -0.5 * LOG2E
    lo = lane < 64
    first = lane < LL
    key = jnp.where(first, lane, lane - LL)
    valid = (lane < 2 * LL) & ((row < MEM) | (row >= key))
    m0 = valid & first
    m1 = valid & jnp.logical_not(first)

    def blk(t):
        z40 = jnp.zeros((LL, 128), f32)
        z48 = jnp.zeros((128 - 2 * LL, 128), f32)
        ta, tb, tc = t[:, 0:128], t[:, 128:256], t[:, 256:384]
        a = jnp.concatenate([ta, z40, z48], 0)
        b = jnp.concatenate([jnp.where(lo, tb, 0.), jnp.where(lo, 0., tb), z48], 0)
        c = jnp.concatenate([z40, tc, z48], 0)
        return jnp.concatenate([a, b, c], 1).astype(bf16)

    def scores(q, kmat):
        return jax.lax.dot_general(q, kmat, (((1,), (1,)), ((), ())), preferred_element_type=f32)

    def softmax(sc):
        sc = sc * a_scale
        mx0 = jnp.max(jnp.where(m0, sc, NEG), axis=1, keepdims=True)
        mx1 = jnp.max(jnp.where(m1, sc, NEG), axis=1, keepdims=True)
        p = jnp.where(valid, jnp.exp2(sc - jnp.where(first, mx0, mx1)), 0.)
        l0 = jnp.sum(jnp.where(first, p, 0.), axis=1, keepdims=True)
        l1 = jnp.sum(jnp.where(first, 0., p), axis=1, keepdims=True)
        return p * pl.reciprocal(jnp.where(first, l0, l1), approx=True)

    def pv(g, p, vmat):
        obuf[g] = jnp.dot(p, vmat, preferred_element_type=f32)

    def oproj(g0, g1, first_step):
        o = jnp.concatenate([obuf[g] for g in range(g0, g1)], axis=1)
        outs = []
        for c in range(5):
            if first_step:
                w = wo_st[c, g0 * PW:g1 * PW, :]
                wo[c, g0 * DH:g1 * DH, :] = pltpu.bitcast(w, u32)
            else:
                w = pltpu.bitcast(wo[c, g0 * DH:g1 * DH, :], bf16)
            outs.append(jnp.dot(o, w, preferred_element_type=f32))
        return jnp.concatenate(outs, axis=1)

    def a_finish(tau, p_last, vm_last, first_step):
        seg = tau & (nseg - 1)
        rows = pl.ds(pl.multiple_of(seg * SEG, SEG), SEG)
        nxt = (tau + 1) & (nseg - 1)
        hn[...] = _ln(xres[pl.ds(pl.multiple_of(nxt * SEG, SEG), SEG), :])
        r1 = oproj(0, OSPLIT, first_step)
        pv(NP - 1, p_last, vm_last)
        res = r1 + oproj(OSPLIT, NP, first_step)
        mem[...] = jnp.where(seg == nseg - 1, mem0f[...], res[0:MEM])
        xres[rows, :] = xres[rows, :] + res[MEM:LL]

    def a_steps(tau, short):
        if short:
            prow = pl.ds(pl.multiple_of((tau - 1) * 8, 8), 8)

        def proj(g, j):
            cols = slice(j * PW, (j + 1) * PW)
            w = pltpu.bitcast((wq_even, wq_odd)[g % 2][g // 2, :, cols], bf16)
            if short:
                h = jnp.concatenate([mem[...], hn[8:SEG, :]], axis=0)
                y = jnp.dot(h, w, preferred_element_type=f32)
                return jnp.concatenate([y[0:MEM], pre[g, prow, cols], y[MEM:SEG]], axis=0)
            h = jnp.concatenate([mem[...], hn[...]], axis=0)
            return jnp.dot(h, w, preferred_element_type=f32)

        scs, vms, ps = {}, {}, {}
        for g in range(NP):
            kmat = blk(proj(g, 1))
            q = proj(g, 0)
            vms[g] = blk(proj(g, 2))
            if g >= 1:
                ps[g - 1] = softmax(scs.pop(g - 1))
            scs[g] = scores(q, kmat)
            if g >= 1:
                pv(g - 1, ps.pop(g - 1), vms.pop(g - 1))
            yield
        a_finish(tau, softmax(scs.pop(NP - 1)), vms.pop(NP - 1), False)

    def b_steps(tau):
        j = (tau - 1) & (nseg - 1)
        rows = pl.ds(pl.multiple_of(j * SEG, SEG), SEG)

        def bproj(t):
            return jnp.dot(hb[...], pltpu.bitcast(bw[:, t * DM:(t + 1) * DM], bf16),
                           preferred_element_type=f32)

        hb[...] = _ln(xres[rows, :])
        for c in range(5):
            kbuf[c, 0:16, :] = kbuf[c, SEG:SEG + 16, :]
            vbuf[c, 0:16, :] = vbuf[c, SEG:SEG + 16, :]
        yield
        qb[...] = bproj(0) * b_scale
        yield
        k = bproj(1)
        for c in range(5):
            kbuf[c, 16:16 + SEG, :] = k[:, c * 128:(c + 1) * 128]
        yield
        v = bproj(2)
        for c in range(5):
            vbuf[c, 16:16 + SEG, :] = v[:, c * 128:(c + 1) * 128]
        yield
        for rg in range(SEG // 8):
            r0 = 8 * rg
            pos = jax.lax.broadcasted_iota(jnp.int32, (8, 128), 0) + (j * SEG + r0)
            q = [qb[r0:r0 + 8, c * 128:(c + 1) * 128] for c in range(5)]
            lgs = []
            for w in range(BW):
                off = 16 + r0 - w * BDIL
                acc = q[0] * kbuf[0, off:off + 8, :]
                for c in range(1, 5):
                    acc = acc + q[c] * kbuf[c, off:off + 8, :]
                acc = acc + pltpu.roll(acc, 64, 1)
                acc = acc + pltpu.roll(acc, 32, 1)
                if w * BDIL > r0:
                    acc = jnp.where(pos >= w * BDIL, acc, NEG)
                lgs.append(acc)
            mx = functools.reduce(jnp.maximum, lgs)
            es = [jnp.exp2(l - mx) for l in lgs]
            inv = pl.reciprocal(functools.reduce(jnp.add, es), approx=True)
            es = [e * inv for e in es]
            for c in range(5):
                acc = None
                for w in range(BW):
                    off = 16 + r0 - w * BDIL
                    t = es[w] * vbuf[c, off:off + 8, :]
                    acc = t if acc is None else acc + t
                qb[r0:r0 + 8, c * 128:(c + 1) * 128] = acc
            yield
        x2 = xres[rows, :] + jnp.dot(qb[...], pltpu.bitcast(bwo[...], bf16), preferred_element_type=f32)
        xres[rows, :] = x2
        outv[rows, :] = x2.astype(bf16)

    def b_weights():
        for ft in range(3 * DM // 128):
            w = pltpu.bitcast(bst[:, ft * 128:(ft + 1) * 128], u32)
            for kc in range(3):
                t = w[kc * 128:(kc + 1) * 128, :]
                if kc == 2:
                    t = jnp.concatenate([t, jnp.zeros((64, 128), u32)], 0)
                tq[kc, ft * 128:(ft + 1) * 128, :] = t.T
        for j in range(3):
            for t in range(5):
                for kc in range(3):
                    rows = [tq[kc, pl.ds(j * DM + 4 * t + dd, NH, stride=BDH), :] for dd in range(4)]
                    gt = jnp.concatenate(rows, 0).T
                    n = 128 if kc < 2 else 64
                    bw[kc * 128:kc * 128 + n, j * DM + t * 128:j * DM + (t + 1) * 128] = gt[0:n]
        for c5 in range(5):
            to[c5] = bwo_st[:, c5 * 128:(c5 + 1) * 128].astype(f32)
        for c5 in range(5):
            for t in range(5):
                rows = [to[c5, pl.ds(4 * t + dd, NH, stride=BDH), :] for dd in range(4)]
                gt = jnp.concatenate(rows, 0).astype(bf16)
                bwo[t * 64:(t + 1) * 64, c5 * 128:(c5 + 1) * 128] = pltpu.bitcast(gt, u32)

    def tick(tau, short):
        ga, gb = a_steps(tau, short), b_steps(tau)
        a_live = b_live = True
        n = i = 0
        slots = BS_SHORT if short else BS_NORM
        while a_live or b_live:
            while b_live and ((i < len(slots) and slots[i] <= n) or not a_live):
                b_live = next(gb, "done") != "done"
                i += 1
            if a_live:
                a_live = next(ga, "done") != "done"
            n += 1

    def stage(g, dst, slot, t):
        j, r = divmod(t, 3)
        dst[slot, :, t * 128:(t + 1) * 128] = pltpu.bitcast(wst[g, j, r * 128:(r + 1) * 128, :].T, u32)

    def first_pair(g, cur, cur_slot, nxt, nxt_slot, sc_prev, vm_prev):
        gp = (g + NP - 1) & (NP - 1)
        gn = jnp.minimum(g + 1, NP - 1)
        nrow = h0.shape[0]

        def step(t, nsplit=1):
            cols = slice(t * 128, (t + 1) * 128)
            w = pltpu.bitcast(cur[cur_slot, :, cols], bf16)
            cuts = [8 * ((nrow // 8 * i) // nsplit) for i in range(nsplit + 1)]
            head = None
            for r0, r1 in zip(cuts[:-1], cuts[1:]):
                y = jnp.dot(h0[r0:r1, :], w, preferred_element_type=f32)
                if r0 == 0:
                    head, y, r0 = y[0:LL], y[LL:], LL
                pre[g, r0 - LL:r1 - LL, cols] = y
            stage(gn, nxt, nxt_slot, (t + 6) % 9)
            return head

        kmat = blk(jnp.concatenate([step(t) for t in (3, 4, 5)], axis=1))
        p = softmax(sc_prev)
        q = jnp.concatenate([step(t) for t in (0, 1, 2)], axis=1)
        v01 = [step(6), step(7)]
        sc = scores(q, kmat)
        pv(gp, p, vm_prev)
        vm = blk(jnp.concatenate(v01 + [step(8, 4)], axis=1))
        return sc, vm

    w_wait(0)
    for t in range(9):
        stage(0, wq_even, 0, t)

    def first_body(i, carry):
        w_wait(2 * i + 1)
        carry = first_pair(2 * i, wq_even, i, wq_odd, i, *carry)

        @pl.when(2 * i + 2 < NP)
        def _():
            w_wait(2 * i + 2)
        return first_pair(2 * i + 1, wq_odd, i, wq_even, i + 1, *carry)
    sc_last, vm_last = jax.lax.fori_loop(
        0, NP // 2, first_body, (jnp.zeros((LL, 128), f32), jnp.zeros((128, PW), bf16)))
    p_last = softmax(sc_last)

    cp_b().wait()
    cp_bo().wait()
    b_weights()
    for cpy in cp_wo():
        cpy.wait()
    a_finish(0, p_last, vm_last, True)

    def short_body(tau, c):
        @pl.when(tau == 2)
        def _():
            cp_x().wait()
        x_init(tau + 1)
        x_init(jnp.where(tau == 1, 2, jnp.minimum(nlead + tau, nseg - 1)))
        tick(tau, True)
        return c
    jax.lax.fori_loop(1, nlead + 1, short_body, 0)

    un = UNROLL

    def body(it, c):
        tau = nlead + 1 + un * it
        for u in range(un):
            tick(tau + u, False)

        @pl.when(tau >= nseg + un)
        def _():
            out_copy(tau - nseg - un, un).start()
        return c
    jax.lax.fori_loop(0, (2 * nseg - nlead - 1) // un, body, 0)
    for _ in b_steps(2 * nseg):
        pass
    t0 = nlead + 1 + un * (-(-(nseg + un - nlead - 1) // un))
    if t0 - nseg - un > 0:
        head = pl.ds(0, (t0 - nseg - un) * SEG)
        pltpu.make_async_copy(outv.at[head, :], out_hbm.at[head, :], out_sem).start()
    out_copy(nseg - un, un).start()
    pltpu.make_async_copy(outv, out_hbm, out_sem).wait()


@functools.partial(jax.jit, static_argnames=("A_seg_len",))
def pallas_interleave_layers__memory_aug_recurrent_mem_tr__sliding_local_dilated__prompt_kernel(
    A_x, A_mem0, A_Wq, A_Wk, A_Wv, A_Wo, A_seg_len, B_x, B_wqkv, B_wo,
):
    del B_x
    B, S, Dm = A_x.shape
    nseg = S // SEG
    assert B == 1 and Dm == DM and A_seg_len == SEG and S == nseg * SEG and nseg & (nseg - 1) == 0
    assert A_mem0.shape == (1, MEM, DM) and A_Wq.shape == (DM, NH, DH) and A_Wo.shape == (NH, DH, DM)
    assert (2 * nseg - NLEAD - 1) % UNROLL == 0 and nseg - 1 <= 2 * NLEAD and 2 <= NLEAD < nseg
    x = A_x.reshape(nseg, SEG, DM)
    mem0 = A_mem0.reshape(MEM, DM)
    wt = lambda w: jnp.transpose(w, (1, 2, 0)).reshape(NH * DH, DM)
    any_spec = pl.BlockSpec(memory_space=pl.ANY)
    out = pl.pallas_call(
        functools.partial(_kernel, nseg=nseg, nlead=NLEAD),
        out_shape=jax.ShapeDtypeStruct((S, DM), A_x.dtype),
        in_specs=[any_spec] * 8,
        out_specs=any_spec,
        scratch_shapes=[
            pltpu.VMEM((nseg, SEG, DM), bf16),
            pltpu.VMEM((NLEAD, 8, DM), bf16),
            pltpu.VMEM((MEM, DM), bf16),
            pltpu.VMEM((NP, 3, PW, DM), bf16),
            pltpu.VMEM((5, NH * DH, 128), bf16),
            pltpu.VMEM((DM, 3 * DM), bf16),
            pltpu.VMEM((DM, DM), bf16),
            pltpu.VMEM((3, 3 * DM, 128), u32),
            pltpu.VMEM((5, DM, 128), f32),
            pltpu.VMEM((NP // 2 + 1, DM // 2, 3 * PW), u32),
            pltpu.VMEM((NP // 2, DM // 2, 3 * PW), u32),
            pltpu.VMEM((5, NH * DH // 2, 128), u32),
            pltpu.VMEM((DM // 2, 3 * DM), u32),
            pltpu.VMEM((DM // 2, DM), u32),
            pltpu.VMEM((S, DM), f32),
            pltpu.VMEM((MEM, DM), f32),
            pltpu.VMEM((MEM, DM), f32),
            pltpu.VMEM((SEG, DM), f32),
            pltpu.VMEM((LL + 8 * NLEAD, DM), f32),
            pltpu.VMEM((NP, 8 * NLEAD, 3 * PW), f32),
            pltpu.VMEM((NP, LL, PW), f32),
            pltpu.VMEM((5, 16 + SEG, 128), f32),
            pltpu.VMEM((5, 16 + SEG, 128), f32),
            pltpu.VMEM((SEG, DM), f32),
            pltpu.VMEM((SEG, DM), f32),
            pltpu.VMEM((S, DM), bf16),
            pltpu.SemaphoreType.DMA((11 + NP,)),
            pltpu.SemaphoreType.DMA(()),
        ],
        compiler_params=pltpu.CompilerParams(vmem_limit_bytes=124 * 1024 * 1024),
    )(x, mem0, wt(A_Wq), wt(A_Wk), wt(A_Wv), A_Wo.reshape(NH * DH, DM), B_wqkv, B_wo)
    return out.reshape(B, S, DM)
```

```python
import functools

import jax
import jax.numpy as jnp
import jax.experimental.pallas as pl
import jax.experimental.pallas.tpu as pltpu

f32 = jnp.float32
bf16 = jnp.bfloat16
u32 = jnp.uint32

DM = 640
NH = 32
DH = 192
NP = NH // 2
PW = 2 * DH
MEM = 8
SEG = 32
LL = MEM + SEG
BDH = DM // NH
BW, BDIL = 8, 2
LOG2E = 1.4426950408889634
EPS = 1e-5
NEG = -1e30
NLEAD = 34
UNROLL = 3
OSPLIT = 4
BS_NORM = (0, 1, 2, 4, 6, 8, 10, 12, 14)
BS_SHORT = (2, 3, 4, 5, 7, 9, 11, 13, 15)


def _ln(x):
    m = jnp.mean(x, axis=-1, keepdims=True)
    d = x - m
    v = jnp.mean(d * d, axis=-1, keepdims=True)
    return d * jax.lax.rsqrt(v + EPS)


def _kernel(x_hbm, mem0_hbm, wq_hbm, wk_hbm, wv_hbm, wo_hbm, bqkv_hbm, bwo_hbm,
            out_hbm,
            xst, xlead, mem0_st, wst, wo_st, bst, bwo_st, tq, to,
            wq_even, wq_odd, wo, bw, bwo, xres, mem, mem0f, hn, h0, pre, obuf,
            kbuf, vbuf, hb, qb, outv,
            sems, out_sem, *, nseg, nlead):
    def cp_mem0():
        return pltpu.make_async_copy(mem0_hbm, mem0_st, sems.at[0])

    def cp_b():
        return pltpu.make_async_copy(bqkv_hbm, bst, sems.at[1])

    def cp_bo():
        return pltpu.make_async_copy(bwo_hbm, bwo_st, sems.at[2])

    def cp_wo():
        return [pltpu.make_async_copy(wo_hbm.at[:, pl.ds(c * 128, 128)], wo_st.at[c], sems.at[3 + c])
                for c in range(5)]

    def cp_w(g, j):
        w = (wq_hbm, wk_hbm, wv_hbm)[j]
        return pltpu.make_async_copy(w.at[pl.ds(g * PW, PW), :], wst.at[g, j], sems.at[8 + g])

    def w_wait(g):
        pltpu.make_async_copy(wst.at[g], wst.at[g], sems.at[8 + g]).wait()

    def cp_xhead():
        return pltpu.make_async_copy(x_hbm.at[0:3], xst.at[0:3], sems.at[8 + NP])

    def cp_xlead():
        return pltpu.make_async_copy(x_hbm.at[1:nlead + 1, 0:8, :], xlead, sems.at[9 + NP])

    def cp_x():
        return pltpu.make_async_copy(x_hbm.at[3:nseg], xst.at[3:nseg], sems.at[10 + NP])

    def out_copy(j, n):
        r = pl.ds(pl.multiple_of(j * SEG, SEG), n * SEG)
        return pltpu.make_async_copy(outv.at[r, :], out_hbm.at[r, :], out_sem)

    for cpy in ([cp_xlead(), cp_xhead(), cp_mem0()] + [cp_w(g, j) for g in range(NP) for j in (1, 0, 2)]
                + [cp_b(), cp_bo()] + cp_wo() + [cp_x()]):
        cpy.start()

    kbuf[...] = jnp.zeros(kbuf.shape, f32)
    vbuf[...] = jnp.zeros(vbuf.shape, f32)
    cp_xlead().wait()
    cp_xhead().wait()
    cp_mem0().wait()
    mem0f[...] = mem0_st[...].astype(f32)
    h0[0:MEM, :] = mem0_st[...].astype(f32)
    h0[MEM:LL, :] = _ln(xst[0].astype(f32))
    for s in range(nlead):
        h0[LL + 8 * s:LL + 8 * s + 8, :] = _ln(xlead[s].astype(f32))
    for s in range(2):
        xres[s * SEG:(s + 1) * SEG, :] = xst[s].astype(f32)

    def x_init(s):
        xres[pl.ds(pl.multiple_of(s * SEG, SEG), SEG), :] = xst[s].astype(f32)

    lane = jax.lax.broadcasted_iota(jnp.int32, (LL, 128), 1)
    row = jax.lax.broadcasted_iota(jnp.int32, (LL, 128), 0)
    a_scale = DH ** -0.5 * LOG2E
    b_scale = BDH ** -0.5 * LOG2E
    lo = lane < 64
    first = lane < LL
    key = jnp.where(first, lane, lane - LL)
    valid = (lane < 2 * LL) & ((row < MEM) | (row >= key))
    m0 = valid & first
    m1 = valid & jnp.logical_not(first)

    def blk(t):
        z40 = jnp.zeros((LL, 128), f32)
        z48 = jnp.zeros((128 - 2 * LL, 128), f32)
        ta, tb, tc = t[:, 0:128], t[:, 128:256], t[:, 256:384]
        a = jnp.concatenate([ta, z40, z48], 0)
        b = jnp.concatenate([jnp.where(lo, tb, 0.), jnp.where(lo, 0., tb), z48], 0)
        c = jnp.concatenate([z40, tc, z48], 0)
        return jnp.concatenate([a, b, c], 1).astype(bf16)

    def scores(q, kmat):
        return jax.lax.dot_general(q, kmat, (((1,), (1,)), ((), ())), preferred_element_type=f32)

    def softmax(sc):
        sc = sc * a_scale
        mx0 = jnp.max(jnp.where(m0, sc, NEG), axis=1, keepdims=True)
        mx1 = jnp.max(jnp.where(m1, sc, NEG), axis=1, keepdims=True)
        p = jnp.where(valid, jnp.exp2(sc - jnp.where(first, mx0, mx1)), 0.)
        l0 = jnp.sum(jnp.where(first, p, 0.), axis=1, keepdims=True)
        l1 = jnp.sum(jnp.where(first, 0., p), axis=1, keepdims=True)
        return p * pl.reciprocal(jnp.where(first, l0, l1), approx=True)

    def pv(g, p, vmat):
        obuf[g] = jnp.dot(p, vmat, preferred_element_type=f32)

    def oproj(g0, g1, first_step):
        o = jnp.concatenate([obuf[g] for g in range(g0, g1)], axis=1)
        outs = []
        for c in range(5):
            if first_step:
                w = wo_st[c, g0 * PW:g1 * PW, :]
                wo[c, g0 * DH:g1 * DH, :] = pltpu.bitcast(w, u32)
            else:
                w = pltpu.bitcast(wo[c, g0 * DH:g1 * DH, :], bf16)
            outs.append(jnp.dot(o, w, preferred_element_type=f32))
        return jnp.concatenate(outs, axis=1)

    def a_finish(tau, p_last, vm_last, first_step):
        seg = tau & (nseg - 1)
        rows = pl.ds(pl.multiple_of(seg * SEG, SEG), SEG)
        nxt = (tau + 1) & (nseg - 1)
        hn[...] = _ln(xres[pl.ds(pl.multiple_of(nxt * SEG, SEG), SEG), :])
        r1 = oproj(0, OSPLIT, first_step)
        pv(NP - 1, p_last, vm_last)
        res = r1 + oproj(OSPLIT, NP, first_step)
        mem[...] = jnp.where(seg == nseg - 1, mem0f[...], res[0:MEM])
        xres[rows, :] = xres[rows, :] + res[MEM:LL]

    def a_steps(tau, short):
        if short:
            prow = pl.ds(pl.multiple_of((tau - 1) * 8, 8), 8)

        def proj(g, j):
            cols = slice(j * PW, (j + 1) * PW)
            w = pltpu.bitcast((wq_even, wq_odd)[g % 2][g // 2, :, cols], bf16)
            if short:
                h = jnp.concatenate([mem[...], hn[8:SEG, :]], axis=0)
                y = jnp.dot(h, w, preferred_element_type=f32)
                return jnp.concatenate([y[0:MEM], pre[g, prow, cols], y[MEM:SEG]], axis=0)
            h = jnp.concatenate([mem[...], hn[...]], axis=0)
            return jnp.dot(h, w, preferred_element_type=f32)

        scs, vms, ps = {}, {}, {}
        for g in range(NP):
            kmat = blk(proj(g, 1))
            q = proj(g, 0)
            vms[g] = blk(proj(g, 2))
            if g >= 1:
                ps[g - 1] = softmax(scs.pop(g - 1))
            scs[g] = scores(q, kmat)
            if g >= 1:
                pv(g - 1, ps.pop(g - 1), vms.pop(g - 1))
            yield
        a_finish(tau, softmax(scs.pop(NP - 1)), vms.pop(NP - 1), False)

    def b_steps(tau):
        j = (tau - 1) & (nseg - 1)
        rows = pl.ds(pl.multiple_of(j * SEG, SEG), SEG)

        def bproj(t):
            return jnp.dot(hb[...], pltpu.bitcast(bw[:, t * DM:(t + 1) * DM], bf16),
                           preferred_element_type=f32)

        hb[...] = _ln(xres[rows, :])
        for c in range(5):
            kbuf[c, 0:16, :] = kbuf[c, SEG:SEG + 16, :]
            vbuf[c, 0:16, :] = vbuf[c, SEG:SEG + 16, :]
        yield
        qb[...] = bproj(0) * b_scale
        yield
        k = bproj(1)
        for c in range(5):
            kbuf[c, 16:16 + SEG, :] = k[:, c * 128:(c + 1) * 128]
        yield
        v = bproj(2)
        for c in range(5):
            vbuf[c, 16:16 + SEG, :] = v[:, c * 128:(c + 1) * 128]
        yield
        for rg in range(SEG // 8):
            r0 = 8 * rg
            pos = jax.lax.broadcasted_iota(jnp.int32, (8, 128), 0) + (j * SEG + r0)
            q = [qb[r0:r0 + 8, c * 128:(c + 1) * 128] for c in range(5)]
            lgs = []
            for w in range(BW):
                off = 16 + r0 - w * BDIL
                acc = q[0] * kbuf[0, off:off + 8, :]
                for c in range(1, 5):
                    acc = acc + q[c] * kbuf[c, off:off + 8, :]
                acc = acc + pltpu.roll(acc, 64, 1)
                acc = acc + pltpu.roll(acc, 32, 1)
                if w * BDIL > r0:
                    acc = jnp.where(pos >= w * BDIL, acc, NEG)
                lgs.append(acc)
            mx = functools.reduce(jnp.maximum, lgs)
            es = [jnp.exp2(l - mx) for l in lgs]
            inv = pl.reciprocal(functools.reduce(jnp.add, es), approx=True)
            es = [e * inv for e in es]
            for c in range(5):
                acc = None
                for w in range(BW):
                    off = 16 + r0 - w * BDIL
                    t = es[w] * vbuf[c, off:off + 8, :]
                    acc = t if acc is None else acc + t
                qb[r0:r0 + 8, c * 128:(c + 1) * 128] = acc
            yield
        x2 = xres[rows, :] + jnp.dot(qb[...], pltpu.bitcast(bwo[...], bf16), preferred_element_type=f32)
        xres[rows, :] = x2
        outv[rows, :] = x2.astype(bf16)

    def b_weights():
        for ft in range(3 * DM // 128):
            w = pltpu.bitcast(bst[:, ft * 128:(ft + 1) * 128], u32)
            for kc in range(3):
                t = w[kc * 128:(kc + 1) * 128, :]
                if kc == 2:
                    t = jnp.concatenate([t, jnp.zeros((64, 128), u32)], 0)
                tq[kc, ft * 128:(ft + 1) * 128, :] = t.T
        for j in range(3):
            for t in range(5):
                for kc in range(3):
                    rows = [tq[kc, pl.ds(j * DM + 4 * t + dd, NH, stride=BDH), :] for dd in range(4)]
                    gt = jnp.concatenate(rows, 0).T
                    n = 128 if kc < 2 else 64
                    bw[kc * 128:kc * 128 + n, j * DM + t * 128:j * DM + (t + 1) * 128] = gt[0:n]
        for c5 in range(5):
            to[c5] = bwo_st[:, c5 * 128:(c5 + 1) * 128].astype(f32)
        for c5 in range(5):
            for t in range(5):
                rows = [to[c5, pl.ds(4 * t + dd, NH, stride=BDH), :] for dd in range(4)]
                gt = jnp.concatenate(rows, 0).astype(bf16)
                bwo[t * 64:(t + 1) * 64, c5 * 128:(c5 + 1) * 128] = pltpu.bitcast(gt, u32)

    def tick(tau, short):
        ga, gb = a_steps(tau, short), b_steps(tau)
        a_live = b_live = True
        n = i = 0
        slots = BS_SHORT if short else BS_NORM
        while a_live or b_live:
            while b_live and ((i < len(slots) and slots[i] <= n) or not a_live):
                b_live = next(gb, "done") != "done"
                i += 1
            if a_live:
                a_live = next(ga, "done") != "done"
            n += 1

    def stage(g, dst, slot, t):
        j, r = divmod(t, 3)
        dst[slot, :, t * 128:(t + 1) * 128] = pltpu.bitcast(wst[g, j, r * 128:(r + 1) * 128, :].T, u32)

    def first_pair(g, cur, cur_slot, nxt, nxt_slot, sc_prev, vm_prev):
        gp = (g + NP - 1) & (NP - 1)
        gn = jnp.minimum(g + 1, NP - 1)
        nrow = h0.shape[0]

        def step(t, nsplit=1):
            cols = slice(t * 128, (t + 1) * 128)
            w = pltpu.bitcast(cur[cur_slot, :, cols], bf16)
            cuts = [8 * ((nrow // 8 * i) // nsplit) for i in range(nsplit + 1)]
            head = None
            for r0, r1 in zip(cuts[:-1], cuts[1:]):
                y = jnp.dot(h0[r0:r1, :], w, preferred_element_type=f32)
                if r0 == 0:
                    head, y, r0 = y[0:LL], y[LL:], LL
                pre[g, r0 - LL:r1 - LL, cols] = y
            stage(gn, nxt, nxt_slot, (t + 6) % 9)
            return head

        kmat = blk(jnp.concatenate([step(t) for t in (3, 4, 5)], axis=1))
        p = softmax(sc_prev)
        q = jnp.concatenate([step(t) for t in (0, 1, 2)], axis=1)
        v01 = [step(6), step(7)]
        sc = scores(q, kmat)
        pv(gp, p, vm_prev)
        vm = blk(jnp.concatenate(v01 + [step(8, 4)], axis=1))
        return sc, vm

    w_wait(0)
    for t in range(9):
        stage(0, wq_even, 0, t)

    def first_body(i, carry):
        w_wait(2 * i + 1)
        carry = first_pair(2 * i, wq_even, i, wq_odd, i, *carry)

        @pl.when(2 * i + 2 < NP)
        def _():
            w_wait(2 * i + 2)
        return first_pair(2 * i + 1, wq_odd, i, wq_even, i + 1, *carry)
    sc_last, vm_last = jax.lax.fori_loop(
        0, NP // 2, first_body, (jnp.zeros((LL, 128), f32), jnp.zeros((128, PW), bf16)))
    p_last = softmax(sc_last)

    cp_b().wait()
    cp_bo().wait()
    b_weights()
    for cpy in cp_wo():
        cpy.wait()
    a_finish(0, p_last, vm_last, True)

    def short_body(tau, c):
        @pl.when(tau == 2)
        def _():
            cp_x().wait()
        x_init(tau + 1)
        x_init(jnp.where(tau == 1, 2, jnp.minimum(nlead + tau, nseg - 1)))
        tick(tau, True)
        return c
    jax.lax.fori_loop(1, nlead + 1, short_body, 0)

    un = UNROLL

    def body(it, c):
        tau = nlead + 1 + un * it
        for u in range(un):
            tick(tau + u, False)

        @pl.when(tau >= nseg + un)
        def _():
            out_copy(tau - nseg - un, un).start()
        return c
    jax.lax.fori_loop(0, (2 * nseg - nlead - 1) // un, body, 0)
    for _ in b_steps(2 * nseg):
        pass
    t0 = nlead + 1 + un * (-(-(nseg + un - nlead - 1) // un))
    if t0 - nseg - un > 0:
        head = pl.ds(0, (t0 - nseg - un) * SEG)
        pltpu.make_async_copy(outv.at[head, :], out_hbm.at[head, :], out_sem).start()
    out_copy(nseg - un, un).start()
    pltpu.make_async_copy(outv, out_hbm, out_sem).wait()


@functools.partial(jax.jit, static_argnames=("A_seg_len",))
def pallas_interleave_layers__memory_aug_recurrent_mem_tr__sliding_local_dilated__prompt_kernel(
    A_x, A_mem0, A_Wq, A_Wk, A_Wv, A_Wo, A_seg_len, B_x, B_wqkv, B_wo,
):
    del B_x
    B, S, Dm = A_x.shape
    nseg = S // SEG
    assert B == 1 and Dm == DM and A_seg_len == SEG and S == nseg * SEG and nseg & (nseg - 1) == 0
    assert A_mem0.shape == (1, MEM, DM) and A_Wq.shape == (DM, NH, DH) and A_Wo.shape == (NH, DH, DM)
    assert (2 * nseg - NLEAD - 1) % UNROLL == 0 and nseg - 1 <= 2 * NLEAD and 2 <= NLEAD < nseg
    x = A_x.reshape(nseg, SEG, DM)
    mem0 = A_mem0.reshape(MEM, DM)
    wt = lambda w: jnp.transpose(w, (1, 2, 0)).reshape(NH * DH, DM)
    any_spec = pl.BlockSpec(memory_space=pl.ANY)
    out = pl.pallas_call(
        functools.partial(_kernel, nseg=nseg, nlead=NLEAD),
        out_shape=jax.ShapeDtypeStruct((S, DM), A_x.dtype),
        in_specs=[any_spec] * 8,
        out_specs=any_spec,
        scratch_shapes=[
            pltpu.VMEM((nseg, SEG, DM), bf16),
            pltpu.VMEM((NLEAD, 8, DM), bf16),
            pltpu.VMEM((MEM, DM), bf16),
            pltpu.VMEM((NP, 3, PW, DM), bf16),
            pltpu.VMEM((5, NH * DH, 128), bf16),
            pltpu.VMEM((DM, 3 * DM), bf16),
            pltpu.VMEM((DM, DM), bf16),
            pltpu.VMEM((3, 3 * DM, 128), u32),
            pltpu.VMEM((5, DM, 128), f32),
            pltpu.VMEM((NP // 2 + 1, DM // 2, 3 * PW), u32),
            pltpu.VMEM((NP // 2, DM // 2, 3 * PW), u32),
            pltpu.VMEM((5, NH * DH // 2, 128), u32),
            pltpu.VMEM((DM // 2, 3 * DM), u32),
            pltpu.VMEM((DM // 2, DM), u32),
            pltpu.VMEM((S, DM), f32),
            pltpu.VMEM((MEM, DM), f32),
            pltpu.VMEM((MEM, DM), f32),
            pltpu.VMEM((SEG, DM), f32),
            pltpu.VMEM((LL + 8 * NLEAD, DM), f32),
            pltpu.VMEM((NP, 8 * NLEAD, 3 * PW), f32),
            pltpu.VMEM((NP, LL, PW), f32),
            pltpu.VMEM((5, 16 + SEG, 128), f32),
            pltpu.VMEM((5, 16 + SEG, 128), f32),
            pltpu.VMEM((SEG, DM), f32),
            pltpu.VMEM((SEG, DM), f32),
            pltpu.VMEM((S, DM), bf16),
            pltpu.SemaphoreType.DMA((11 + NP,)),
            pltpu.SemaphoreType.DMA(()),
        ],
        compiler_params=pltpu.CompilerParams(
            vmem_limit_bytes=124 * 1024 * 1024,
            flags={"XLA_TPU_FORCE_LP_LLO_SCHEDULER": True}),
    )(x, mem0, wt(A_Wq), wt(A_Wk), wt(A_Wv), A_Wo.reshape(NH * DH, DM), B_wqkv, B_wo)
    return out.reshape(B, S, DM)
```

```python
import functools

import jax
import jax.numpy as jnp
import jax.experimental.pallas as pl
import jax.experimental.pallas.tpu as pltpu

f32 = jnp.float32
bf16 = jnp.bfloat16
u32 = jnp.uint32

DM = 640
NH = 32
DH = 192
NP = NH // 2
PW = 2 * DH
MEM = 8
SEG = 32
LL = MEM + SEG
BDH = DM // NH
BW, BDIL = 8, 2
LOG2E = 1.4426950408889634
EPS = 1e-5
NEG = -1e30
NLEAD = 37
XPAD = 44
UNROLL = 3
OSPLIT = 4
BS_NORM = (0, 1, 2, 4, 6, 8, 10, 12, 14)
BS_SHORT = (2, 3, 4, 5, 7, 9, 11, 13, 15)


def _ln(x):
    m = jnp.mean(x, axis=-1, keepdims=True)
    d = x - m
    v = jnp.mean(d * d, axis=-1, keepdims=True)
    return d * jax.lax.rsqrt(v + EPS)


def _kernel(x_hbm, mem0_hbm, wq_hbm, wk_hbm, wv_hbm, wo_hbm, bqkv_hbm, bwo_hbm,
            out_hbm,
            xst, xlead, mem0_st, wst, wo_st, bst, bwo_st, tq, to,
            wq_even, wq_odd, wo, bw, bwo, xres, mem, mem0f, hn, h0, pre, obuf,
            kbuf, vbuf, hb, qb, outv,
            sems, out_sem, *, nseg, nlead):
    def cp_mem0():
        return pltpu.make_async_copy(mem0_hbm, mem0_st, sems.at[0])

    def cp_b():
        return pltpu.make_async_copy(bqkv_hbm, bst, sems.at[1])

    def cp_bo():
        return pltpu.make_async_copy(bwo_hbm, bwo_st, sems.at[2])

    def cp_wo():
        return [pltpu.make_async_copy(wo_hbm.at[:, pl.ds(c * 128, 128)], wo_st.at[c], sems.at[3 + c])
                for c in range(5)]

    def cp_w(g, j):
        w = (wq_hbm, wk_hbm, wv_hbm)[j]
        return pltpu.make_async_copy(w.at[pl.ds(g * PW, PW), :], wst.at[g, j], sems.at[8 + g])

    def w_wait(g):
        pltpu.make_async_copy(wst.at[g], wst.at[g], sems.at[8 + g]).wait()

    def cp_xhead():
        return pltpu.make_async_copy(x_hbm.at[0:3], xst.at[0:3], sems.at[8 + NP])

    def cp_xlead():
        return pltpu.make_async_copy(x_hbm.at[1:nlead + 1, 0:8, :], xlead.at[0:nlead], sems.at[9 + NP])

    def cp_x():
        return pltpu.make_async_copy(x_hbm.at[3:nseg], xst.at[3:nseg], sems.at[10 + NP])

    def out_copy(j, n):
        r = pl.ds(pl.multiple_of(j * SEG, SEG), n * SEG)
        return pltpu.make_async_copy(outv.at[r, :], out_hbm.at[r, :], out_sem)

    for cpy in ([cp_xlead(), cp_xhead(), cp_mem0()] + [cp_w(g, j) for g in range(NP) for j in (1, 0, 2)]
                + [cp_b(), cp_bo()] + cp_wo() + [cp_x()]):
        cpy.start()

    kbuf[...] = jnp.zeros(kbuf.shape, f32)
    vbuf[...] = jnp.zeros(vbuf.shape, f32)
    cp_xlead().wait()
    cp_xhead().wait()
    cp_mem0().wait()
    mem0f[...] = mem0_st[...].astype(f32)
    h0[0:MEM, :] = mem0_st[...].astype(f32)
    h0[MEM:LL, :] = _ln(xst[0].astype(f32))
    for s in range(nlead):
        h0[LL + 8 * s:LL + 8 * s + 8, :] = _ln(xlead[s].astype(f32))
    for s in range(2):
        xres[s * SEG:(s + 1) * SEG, :] = xst[s].astype(f32)

    def x_init(s):
        xres[pl.ds(pl.multiple_of(s * SEG, SEG), SEG), :] = xst[s].astype(f32)

    lane = jax.lax.broadcasted_iota(jnp.int32, (LL, 128), 1)
    row = jax.lax.broadcasted_iota(jnp.int32, (LL, 128), 0)
    a_scale = DH ** -0.5 * LOG2E
    b_scale = BDH ** -0.5 * LOG2E
    lo = lane < 64
    first = lane < LL
    key = jnp.where(first, lane, lane - LL)
    valid = (lane < 2 * LL) & ((row < MEM) | (row >= key))
    m0 = valid & first
    m1 = valid & jnp.logical_not(first)

    def blk(t):
        z40 = jnp.zeros((LL, 128), f32)
        z48 = jnp.zeros((128 - 2 * LL, 128), f32)
        ta, tb, tc = t[:, 0:128], t[:, 128:256], t[:, 256:384]
        a = jnp.concatenate([ta, z40, z48], 0)
        b = jnp.concatenate([jnp.where(lo, tb, 0.), jnp.where(lo, 0., tb), z48], 0)
        c = jnp.concatenate([z40, tc, z48], 0)
        return jnp.concatenate([a, b, c], 1).astype(bf16)

    def scores(q, kmat):
        return jax.lax.dot_general(q, kmat, (((1,), (1,)), ((), ())), preferred_element_type=f32)

    def softmax(sc):
        sc = sc * a_scale
        mx0 = jnp.max(jnp.where(m0, sc, NEG), axis=1, keepdims=True)
        mx1 = jnp.max(jnp.where(m1, sc, NEG), axis=1, keepdims=True)
        p = jnp.where(valid, jnp.exp2(sc - jnp.where(first, mx0, mx1)), 0.)
        l0 = jnp.sum(jnp.where(first, p, 0.), axis=1, keepdims=True)
        l1 = jnp.sum(jnp.where(first, 0., p), axis=1, keepdims=True)
        return p * pl.reciprocal(jnp.where(first, l0, l1), approx=True)

    def pv(g, p, vmat):
        obuf[g] = jnp.dot(p, vmat, preferred_element_type=f32)

    def oproj(g0, g1, first_step):
        o = jnp.concatenate([obuf[g] for g in range(g0, g1)], axis=1)
        outs = []
        for c in range(5):
            if first_step:
                w = wo_st[c, g0 * PW:g1 * PW, :]
                wo[c, g0 * DH:g1 * DH, :] = pltpu.bitcast(w, u32)
            else:
                w = pltpu.bitcast(wo[c, g0 * DH:g1 * DH, :], bf16)
            outs.append(jnp.dot(o, w, preferred_element_type=f32))
        return jnp.concatenate(outs, axis=1)

    def a_finish(tau, p_last, vm_last, first_step):
        seg = tau & (nseg - 1)
        rows = pl.ds(pl.multiple_of(seg * SEG, SEG), SEG)
        nxt = (tau + 1) & (nseg - 1)
        hn[...] = _ln(xres[pl.ds(pl.multiple_of(nxt * SEG, SEG), SEG), :])
        r1 = oproj(0, OSPLIT, first_step)
        pv(NP - 1, p_last, vm_last)
        res = r1 + oproj(OSPLIT, NP, first_step)
        mem[...] = jnp.where(seg == nseg - 1, mem0f[...], res[0:MEM])
        xres[rows, :] = xres[rows, :] + res[MEM:LL]

    def a_steps(tau, short):
        if short:
            prow = pl.ds(pl.multiple_of((tau - 1) * 8, 8), 8)

        def proj(g, j):
            cols = slice(j * PW, (j + 1) * PW)
            w = pltpu.bitcast((wq_even, wq_odd)[g % 2][g // 2, :, cols], bf16)
            if short:
                h = jnp.concatenate([mem[...], hn[8:SEG, :]], axis=0)
                y = jnp.dot(h, w, preferred_element_type=f32)
                return jnp.concatenate([y[0:MEM], pre[g, prow, cols], y[MEM:SEG]], axis=0)
            h = jnp.concatenate([mem[...], hn[...]], axis=0)
            return jnp.dot(h, w, preferred_element_type=f32)

        scs, vms, ps = {}, {}, {}
        for g in range(NP):
            kmat = blk(proj(g, 1))
            q = proj(g, 0)
            vms[g] = blk(proj(g, 2))
            if g >= 1:
                ps[g - 1] = softmax(scs.pop(g - 1))
            scs[g] = scores(q, kmat)
            if g >= 1:
                pv(g - 1, ps.pop(g - 1), vms.pop(g - 1))
            yield
        a_finish(tau, softmax(scs.pop(NP - 1)), vms.pop(NP - 1), False)

    def b_steps(tau):
        j = (tau - 1) & (nseg - 1)
        rows = pl.ds(pl.multiple_of(j * SEG, SEG), SEG)

        def bproj(t):
            return jnp.dot(hb[...], pltpu.bitcast(bw[:, t * DM:(t + 1) * DM], bf16),
                           preferred_element_type=f32)

        hb[...] = _ln(xres[rows, :])
        for c in range(5):
            kbuf[c, 0:16, :] = kbuf[c, SEG:SEG + 16, :]
            vbuf[c, 0:16, :] = vbuf[c, SEG:SEG + 16, :]
        yield
        qb[...] = bproj(0) * b_scale
        yield
        k = bproj(1)
        for c in range(5):
            kbuf[c, 16:16 + SEG, :] = k[:, c * 128:(c + 1) * 128]
        yield
        v = bproj(2)
        for c in range(5):
            vbuf[c, 16:16 + SEG, :] = v[:, c * 128:(c + 1) * 128]
        yield
        for rg in range(SEG // 8):
            r0 = 8 * rg
            pos = jax.lax.broadcasted_iota(jnp.int32, (8, 128), 0) + (j * SEG + r0)
            q = [qb[r0:r0 + 8, c * 128:(c + 1) * 128] for c in range(5)]
            lgs = []
            for w in range(BW):
                off = 16 + r0 - w * BDIL
                acc = q[0] * kbuf[0, off:off + 8, :]
                for c in range(1, 5):
                    acc = acc + q[c] * kbuf[c, off:off + 8, :]
                acc = acc + pltpu.roll(acc, 64, 1)
                acc = acc + pltpu.roll(acc, 32, 1)
                if w * BDIL > r0:
                    acc = jnp.where(pos >= w * BDIL, acc, NEG)
                lgs.append(acc)
            mx = functools.reduce(jnp.maximum, lgs)
            es = [jnp.exp2(l - mx) for l in lgs]
            inv = pl.reciprocal(functools.reduce(jnp.add, es), approx=True)
            es = [e * inv for e in es]
            for c in range(5):
                acc = None
                for w in range(BW):
                    off = 16 + r0 - w * BDIL
                    t = es[w] * vbuf[c, off:off + 8, :]
                    acc = t if acc is None else acc + t
                qb[r0:r0 + 8, c * 128:(c + 1) * 128] = acc
            yield
        x2 = xres[rows, :] + jnp.dot(qb[...], pltpu.bitcast(bwo[...], bf16), preferred_element_type=f32)
        xres[rows, :] = x2
        outv[rows, :] = x2.astype(bf16)

    def b_weights():
        for ft in range(3 * DM // 128):
            w = pltpu.bitcast(bst[:, ft * 128:(ft + 1) * 128], u32)
            for kc in range(3):
                t = w[kc * 128:(kc + 1) * 128, :]
                if kc == 2:
                    t = jnp.concatenate([t, jnp.zeros((64, 128), u32)], 0)
                tq[kc, ft * 128:(ft + 1) * 128, :] = t.T
        for j in range(3):
            for t in range(5):
                for kc in range(3):
                    rows = [tq[kc, pl.ds(j * DM + 4 * t + dd, NH, stride=BDH), :] for dd in range(4)]
                    gt = jnp.concatenate(rows, 0).T
                    n = 128 if kc < 2 else 64
                    bw[kc * 128:kc * 128 + n, j * DM + t * 128:j * DM + (t + 1) * 128] = gt[0:n]
        for c5 in range(5):
            to[c5] = bwo_st[:, c5 * 128:(c5 + 1) * 128].astype(f32)
        for c5 in range(5):
            for t in range(5):
                rows = [to[c5, pl.ds(4 * t + dd, NH, stride=BDH), :] for dd in range(4)]
                gt = jnp.concatenate(rows, 0).astype(bf16)
                bwo[t * 64:(t + 1) * 64, c5 * 128:(c5 + 1) * 128] = pltpu.bitcast(gt, u32)

    def tick(tau, short):
        ga, gb = a_steps(tau, short), b_steps(tau)
        a_live = b_live = True
        n = i = 0
        slots = BS_SHORT if short else BS_NORM
        while a_live or b_live:
            while b_live and ((i < len(slots) and slots[i] <= n) or not a_live):
                b_live = next(gb, "done") != "done"
                i += 1
            if a_live:
                a_live = next(ga, "done") != "done"
            n += 1

    def stage(g, dst, slot, t):
        j, r = divmod(t, 3)
        dst[slot, :, t * 128:(t + 1) * 128] = pltpu.bitcast(wst[g, j, r * 128:(r + 1) * 128, :].T, u32)

    def first_pair(g, cur, cur_slot, nxt, nxt_slot, sc_prev, vm_prev):
        gp = (g + NP - 1) & (NP - 1)
        gn = jnp.minimum(g + 1, NP - 1)
        nrow = h0.shape[0]

        def step(t, nsplit=1):
            cols = slice(t * 128, (t + 1) * 128)
            w = pltpu.bitcast(cur[cur_slot, :, cols], bf16)
            cuts = [8 * ((nrow // 8 * i) // nsplit) for i in range(nsplit + 1)]
            head = None
            for r0, r1 in zip(cuts[:-1], cuts[1:]):
                y = jnp.dot(h0[r0:r1, :], w, preferred_element_type=f32)
                if r0 == 0:
                    head, y, r0 = y[0:LL], y[LL:], LL
                pre[g, r0 - LL:r1 - LL, cols] = y
            stage(gn, nxt, nxt_slot, (t + 6) % 9)
            return head

        kmat = blk(jnp.concatenate([step(t) for t in (3, 4, 5)], axis=1))
        p = softmax(sc_prev)
        q = jnp.concatenate([step(t) for t in (0, 1, 2)], axis=1)
        v01 = [step(6), step(7)]
        sc = scores(q, kmat)
        pv(gp, p, vm_prev)
        vm = blk(jnp.concatenate(v01 + [step(8, 4)], axis=1))
        return sc, vm

    w_wait(0)
    for t in range(9):
        stage(0, wq_even, 0, t)

    def first_body(i, carry):
        w_wait(2 * i + 1)
        carry = first_pair(2 * i, wq_even, i, wq_odd, i, *carry)

        @pl.when(2 * i + 2 < NP)
        def _():
            w_wait(2 * i + 2)
        return first_pair(2 * i + 1, wq_odd, i, wq_even, i + 1, *carry)
    sc_last, vm_last = jax.lax.fori_loop(
        0, NP // 2, first_body, (jnp.zeros((LL, 128), f32), jnp.zeros((128, PW), bf16)))
    p_last = softmax(sc_last)

    cp_b().wait()
    cp_bo().wait()
    for cpy in cp_wo():
        cpy.wait()
    a_finish(0, p_last, vm_last, True)
    b_weights()

    def short_body(tau, c):
        @pl.when(tau == 2)
        def _():
            cp_x().wait()
        x_init(tau + 1)
        x_init(jnp.where(tau == 1, 2, jnp.minimum(nlead + tau, nseg - 1)))
        tick(tau, True)
        return c
    jax.lax.fori_loop(1, nlead + 1, short_body, 0)

    un = UNROLL

    def body(it, c):
        tau = nlead + 1 + un * it
        for u in range(un):
            tick(tau + u, False)

        @pl.when(tau >= nseg + un)
        def _():
            out_copy(tau - nseg - un, un).start()
        return c
    jax.lax.fori_loop(0, (2 * nseg - nlead - 1) // un, body, 0)
    for _ in b_steps(2 * nseg):
        pass
    t0 = nlead + 1 + un * (-(-(nseg + un - nlead - 1) // un))
    if t0 - nseg - un > 0:
        head = pl.ds(0, (t0 - nseg - un) * SEG)
        pltpu.make_async_copy(outv.at[head, :], out_hbm.at[head, :], out_sem).start()
    out_copy(nseg - un, un).start()
    pltpu.make_async_copy(outv, out_hbm, out_sem).wait()


@functools.partial(jax.jit, static_argnames=("A_seg_len",))
def pallas_interleave_layers__memory_aug_recurrent_mem_tr__sliding_local_dilated__prompt_kernel(
    A_x, A_mem0, A_Wq, A_Wk, A_Wv, A_Wo, A_seg_len, B_x, B_wqkv, B_wo,
):
    del B_x
    B, S, Dm = A_x.shape
    nseg = S // SEG
    assert B == 1 and Dm == DM and A_seg_len == SEG and S == nseg * SEG and nseg & (nseg - 1) == 0
    assert A_mem0.shape == (1, MEM, DM) and A_Wq.shape == (DM, NH, DH) and A_Wo.shape == (NH, DH, DM)
    assert (2 * nseg - NLEAD - 1) % UNROLL == 0 and nseg - 1 <= 2 * NLEAD and 2 <= NLEAD < nseg
    x = A_x.reshape(nseg, SEG, DM)
    mem0 = A_mem0.reshape(MEM, DM)
    wt = lambda w: jnp.transpose(w, (1, 2, 0)).reshape(NH * DH, DM)
    any_spec = pl.BlockSpec(memory_space=pl.ANY)
    out = pl.pallas_call(
        functools.partial(_kernel, nseg=nseg, nlead=NLEAD),
        out_shape=jax.ShapeDtypeStruct((S, DM), A_x.dtype),
        in_specs=[any_spec] * 8,
        out_specs=any_spec,
        scratch_shapes=[
            pltpu.VMEM((nseg, SEG, DM), bf16),
            pltpu.VMEM((XPAD, 8, DM), bf16),
            pltpu.VMEM((MEM, DM), bf16),
            pltpu.VMEM((NP, 3, PW, DM), bf16),
            pltpu.VMEM((5, NH * DH, 128), bf16),
            pltpu.VMEM((DM, 3 * DM), bf16),
            pltpu.VMEM((DM, DM), bf16),
            pltpu.VMEM((3, 3 * DM, 128), u32),
            pltpu.VMEM((5, DM, 128), f32),
            pltpu.VMEM((NP // 2 + 1, DM // 2, 3 * PW), u32),
            pltpu.VMEM((NP // 2, DM // 2, 3 * PW), u32),
            pltpu.VMEM((5, NH * DH // 2, 128), u32),
            pltpu.VMEM((DM // 2, 3 * DM), u32),
            pltpu.VMEM((DM // 2, DM), u32),
            pltpu.VMEM((S, DM), f32),
            pltpu.VMEM((MEM, DM), f32),
            pltpu.VMEM((MEM, DM), f32),
            pltpu.VMEM((SEG, DM), f32),
            pltpu.VMEM((LL + 8 * NLEAD, DM), f32),
            pltpu.VMEM((NP, 8 * NLEAD, 3 * PW), f32),
            pltpu.VMEM((NP, LL, PW), f32),
            pltpu.VMEM((5, 16 + SEG, 128), f32),
            pltpu.VMEM((5, 16 + SEG, 128), f32),
            pltpu.VMEM((SEG, DM), f32),
            pltpu.VMEM((SEG, DM), f32),
            pltpu.VMEM((S, DM), bf16),
            pltpu.SemaphoreType.DMA((11 + NP,)),
            pltpu.SemaphoreType.DMA(()),
        ],
        compiler_params=pltpu.CompilerParams(
            vmem_limit_bytes=124 * 1024 * 1024,
            flags={"XLA_TPU_FORCE_LP_LLO_SCHEDULER": True}),
    )(x, mem0, wt(A_Wq), wt(A_Wk), wt(A_Wv), A_Wo.reshape(NH * DH, DM), B_wqkv, B_wo)
    return out.reshape(B, S, DM)
```

```python
import functools

import jax
import jax.numpy as jnp
import jax.experimental.pallas as pl
import jax.experimental.pallas.tpu as pltpu

f32 = jnp.float32
bf16 = jnp.bfloat16
u32 = jnp.uint32

DM = 640
NH = 32
DH = 192
NP = NH // 2
PW = 2 * DH
MEM = 8
SEG = 32
LL = MEM + SEG
BDH = DM // NH
BW, BDIL = 8, 2
LOG2E = 1.4426950408889634
EPS = 1e-5
NEG = -1e30
NLEAD = 37
XPAD = 44
UNROLL = 3
OSPLIT = 4
BS_NORM = (0, 1, 2, 4, 6, 8, 10, 12, 14)
BS_SHORT = (2, 3, 4, 5, 7, 9, 11, 13, 15)


def _ln(x):
    m = jnp.mean(x, axis=-1, keepdims=True)
    d = x - m
    v = jnp.mean(d * d, axis=-1, keepdims=True)
    return d * jax.lax.rsqrt(v + EPS)


_rcp_estimate = getattr(pltpu, "reciprocal", None) or pl.reciprocal


def _recip(x):
    r = _rcp_estimate(x, approx=True)
    return r * (2.0 - x * r)


def _kernel(x_hbm, mem0_hbm, wq_hbm, wk_hbm, wv_hbm, wo_hbm, bqkv_hbm, bwo_hbm,
            out_hbm,
            xst, xlead, mem0_st, wst, wo_st, bst, bwo_st, tq, to,
            wq_even, wq_odd, wo, bw, bwo, xres, mem, mem0f, hn, h0, pre, obuf,
            kbuf, vbuf, hb, qb, outv,
            sems, out_sem, *, nseg, nlead):
    def cp_mem0():
        return pltpu.make_async_copy(mem0_hbm, mem0_st, sems.at[0])

    def cp_b():
        return pltpu.make_async_copy(bqkv_hbm, bst, sems.at[1])

    def cp_bo():
        return pltpu.make_async_copy(bwo_hbm, bwo_st, sems.at[2])

    def cp_wo():
        return [pltpu.make_async_copy(wo_hbm.at[:, pl.ds(c * 128, 128)], wo_st.at[c], sems.at[3 + c])
                for c in range(5)]

    def cp_w(g, j):
        w = (wq_hbm, wk_hbm, wv_hbm)[j]
        return pltpu.make_async_copy(w.at[pl.ds(g * PW, PW), :], wst.at[g, j], sems.at[8 + g])

    def w_wait(g):
        pltpu.make_async_copy(wst.at[g], wst.at[g], sems.at[8 + g]).wait()

    def cp_xhead():
        return pltpu.make_async_copy(x_hbm.at[0:3], xst.at[0:3], sems.at[8 + NP])

    def cp_xlead():
        return pltpu.make_async_copy(x_hbm.at[1:nlead + 1, 0:8, :], xlead.at[0:nlead], sems.at[9 + NP])

    def cp_x():
        return pltpu.make_async_copy(x_hbm.at[3:nseg], xst.at[3:nseg], sems.at[10 + NP])

    def out_copy(j, n):
        r = pl.ds(pl.multiple_of(j * SEG, SEG), n * SEG)
        return pltpu.make_async_copy(outv.at[r, :], out_hbm.at[r, :], out_sem)

    for cpy in ([cp_xlead(), cp_xhead(), cp_mem0()] + [cp_w(g, j) for g in range(NP) for j in (1, 0, 2)]
                + [cp_b(), cp_bo()] + cp_wo() + [cp_x()]):
        cpy.start()

    kbuf[...] = jnp.zeros(kbuf.shape, f32)
    vbuf[...] = jnp.zeros(vbuf.shape, f32)
    cp_xlead().wait()
    cp_xhead().wait()
    cp_mem0().wait()
    mem0f[...] = mem0_st[...].astype(f32)
    h0[0:MEM, :] = mem0_st[...].astype(f32)
    h0[MEM:LL, :] = _ln(xst[0].astype(f32))
    for s in range(nlead):
        h0[LL + 8 * s:LL + 8 * s + 8, :] = _ln(xlead[s].astype(f32))
    for s in range(2):
        xres[s * SEG:(s + 1) * SEG, :] = xst[s].astype(f32)

    def x_init(s):
        xres[pl.ds(pl.multiple_of(s * SEG, SEG), SEG), :] = xst[s].astype(f32)

    lane = jax.lax.broadcasted_iota(jnp.int32, (LL, 128), 1)
    row = jax.lax.broadcasted_iota(jnp.int32, (LL, 128), 0)
    a_scale = DH ** -0.5 * LOG2E
    b_scale = BDH ** -0.5 * LOG2E
    lo = lane < 64
    first = lane < LL
    key = jnp.where(first, lane, lane - LL)
    valid = (lane < 2 * LL) & ((row < MEM) | (row >= key))
    m0 = valid & first
    m1 = valid & jnp.logical_not(first)

    def blk(t):
        z40 = jnp.zeros((LL, 128), f32)
        z48 = jnp.zeros((128 - 2 * LL, 128), f32)
        ta, tb, tc = t[:, 0:128], t[:, 128:256], t[:, 256:384]
        a = jnp.concatenate([ta, z40, z48], 0)
        b = jnp.concatenate([jnp.where(lo, tb, 0.), jnp.where(lo, 0., tb), z48], 0)
        c = jnp.concatenate([z40, tc, z48], 0)
        return jnp.concatenate([a, b, c], 1).astype(bf16)

    def scores(q, kmat):
        return jax.lax.dot_general(q, kmat, (((1,), (1,)), ((), ())), preferred_element_type=f32)

    def softmax(sc):
        sc = sc * a_scale
        mx0 = jnp.max(jnp.where(m0, sc, NEG), axis=1, keepdims=True)
        mx1 = jnp.max(jnp.where(m1, sc, NEG), axis=1, keepdims=True)
        p = jnp.where(valid, jnp.exp2(sc - jnp.where(first, mx0, mx1)), 0.)
        l0 = jnp.sum(jnp.where(first, p, 0.), axis=1, keepdims=True)
        l1 = jnp.sum(jnp.where(first, 0., p), axis=1, keepdims=True)
        return p * _recip(jnp.where(first, l0, l1))

    def pv(g, p, vmat):
        obuf[g] = jnp.dot(p, vmat, preferred_element_type=f32)

    def oproj(g0, g1, first_step):
        o = jnp.concatenate([obuf[g] for g in range(g0, g1)], axis=1)
        outs = []
        for c in range(5):
            if first_step:
                w = wo_st[c, g0 * PW:g1 * PW, :]
                wo[c, g0 * DH:g1 * DH, :] = pltpu.bitcast(w, u32)
            else:
                w = pltpu.bitcast(wo[c, g0 * DH:g1 * DH, :], bf16)
            outs.append(jnp.dot(o, w, preferred_element_type=f32))
        return jnp.concatenate(outs, axis=1)

    def a_finish(tau, p_last, vm_last, first_step):
        seg = tau & (nseg - 1)
        rows = pl.ds(pl.multiple_of(seg * SEG, SEG), SEG)
        nxt = (tau + 1) & (nseg - 1)
        hn[...] = _ln(xres[pl.ds(pl.multiple_of(nxt * SEG, SEG), SEG), :])
        r1 = oproj(0, OSPLIT, first_step)
        pv(NP - 1, p_last, vm_last)
        res = r1 + oproj(OSPLIT, NP, first_step)
        mem[...] = jnp.where(seg == nseg - 1, mem0f[...], res[0:MEM])
        xres[rows, :] = xres[rows, :] + res[MEM:LL]

    def a_steps(tau, short):
        if short:
            prow = pl.ds(pl.multiple_of((tau - 1) * 8, 8), 8)

        def proj(g, j):
            cols = slice(j * PW, (j + 1) * PW)
            w = pltpu.bitcast((wq_even, wq_odd)[g % 2][g // 2, :, cols], bf16)
            if short:
                h = jnp.concatenate([mem[...], hn[8:SEG, :]], axis=0)
                y = jnp.dot(h, w, preferred_element_type=f32)
                return jnp.concatenate([y[0:MEM], pre[g, prow, cols], y[MEM:SEG]], axis=0)
            h = jnp.concatenate([mem[...], hn[...]], axis=0)
            return jnp.dot(h, w, preferred_element_type=f32)

        scs, vms, ps = {}, {}, {}
        for g in range(NP):
            kmat = blk(proj(g, 1))
            q = proj(g, 0)
            vms[g] = blk(proj(g, 2))
            if g >= 1:
                ps[g - 1] = softmax(scs.pop(g - 1))
            scs[g] = scores(q, kmat)
            if g >= 1:
                pv(g - 1, ps.pop(g - 1), vms.pop(g - 1))
            yield
        a_finish(tau, softmax(scs.pop(NP - 1)), vms.pop(NP - 1), False)

    def b_steps(tau):
        j = (tau - 1) & (nseg - 1)
        rows = pl.ds(pl.multiple_of(j * SEG, SEG), SEG)

        def bproj(t):
            return jnp.dot(hb[...], pltpu.bitcast(bw[:, t * DM:(t + 1) * DM], bf16),
                           preferred_element_type=f32)

        hb[...] = _ln(xres[rows, :])
        for c in range(5):
            kbuf[c, 0:16, :] = kbuf[c, SEG:SEG + 16, :]
            vbuf[c, 0:16, :] = vbuf[c, SEG:SEG + 16, :]
        yield
        qb[...] = bproj(0) * b_scale
        yield
        k = bproj(1)
        for c in range(5):
            kbuf[c, 16:16 + SEG, :] = k[:, c * 128:(c + 1) * 128]
        yield
        v = bproj(2)
        for c in range(5):
            vbuf[c, 16:16 + SEG, :] = v[:, c * 128:(c + 1) * 128]
        yield
        for rg in range(SEG // 8):
            r0 = 8 * rg
            pos = jax.lax.broadcasted_iota(jnp.int32, (8, 128), 0) + (j * SEG + r0)
            q = [qb[r0:r0 + 8, c * 128:(c + 1) * 128] for c in range(5)]
            lgs = []
            for w in range(BW):
                off = 16 + r0 - w * BDIL
                acc = q[0] * kbuf[0, off:off + 8, :]
                for c in range(1, 5):
                    acc = acc + q[c] * kbuf[c, off:off + 8, :]
                acc = acc + pltpu.roll(acc, 64, 1)
                acc = acc + pltpu.roll(acc, 32, 1)
                if w * BDIL > r0:
                    acc = jnp.where(pos >= w * BDIL, acc, NEG)
                lgs.append(acc)
            mx = functools.reduce(jnp.maximum, lgs)
            es = [jnp.exp2(l - mx) for l in lgs]
            inv = _recip(functools.reduce(jnp.add, es))
            es = [e * inv for e in es]
            for c in range(5):
                acc = None
                for w in range(BW):
                    off = 16 + r0 - w * BDIL
                    t = es[w] * vbuf[c, off:off + 8, :]
                    acc = t if acc is None else acc + t
                qb[r0:r0 + 8, c * 128:(c + 1) * 128] = acc
            yield
        x2 = xres[rows, :] + jnp.dot(qb[...], pltpu.bitcast(bwo[...], bf16), preferred_element_type=f32)
        xres[rows, :] = x2
        outv[rows, :] = x2.astype(bf16)

    def b_weights():
        for ft in range(3 * DM // 128):
            w = pltpu.bitcast(bst[:, ft * 128:(ft + 1) * 128], u32)
            for kc in range(3):
                t = w[kc * 128:(kc + 1) * 128, :]
                if kc == 2:
                    t = jnp.concatenate([t, jnp.zeros((64, 128), u32)], 0)
                tq[kc, ft * 128:(ft + 1) * 128, :] = t.T
        for j in range(3):
            for t in range(5):
                for kc in range(3):
                    rows = [tq[kc, pl.ds(j * DM + 4 * t + dd, NH, stride=BDH), :] for dd in range(4)]
                    gt = jnp.concatenate(rows, 0).T
                    n = 128 if kc < 2 else 64
                    bw[kc * 128:kc * 128 + n, j * DM + t * 128:j * DM + (t + 1) * 128] = gt[0:n]
        for c5 in range(5):
            to[c5] = bwo_st[:, c5 * 128:(c5 + 1) * 128].astype(f32)
        for c5 in range(5):
            for t in range(5):
                rows = [to[c5, pl.ds(4 * t + dd, NH, stride=BDH), :] for dd in range(4)]
                gt = jnp.concatenate(rows, 0).astype(bf16)
                bwo[t * 64:(t + 1) * 64, c5 * 128:(c5 + 1) * 128] = pltpu.bitcast(gt, u32)

    def tick(tau, short):
        ga, gb = a_steps(tau, short), b_steps(tau)
        a_live = b_live = True
        n = i = 0
        slots = BS_SHORT if short else BS_NORM
        while a_live or b_live:
            while b_live and ((i < len(slots) and slots[i] <= n) or not a_live):
                b_live = next(gb, "done") != "done"
                i += 1
            if a_live:
                a_live = next(ga, "done") != "done"
            n += 1

    def stage(g, dst, slot, t):
        j, r = divmod(t, 3)
        dst[slot, :, t * 128:(t + 1) * 128] = pltpu.bitcast(wst[g, j, r * 128:(r + 1) * 128, :].T, u32)

    def first_pair(g, cur, cur_slot, nxt, nxt_slot, sc_prev, vm_prev):
        gp = (g + NP - 1) & (NP - 1)
        gn = jnp.minimum(g + 1, NP - 1)
        nrow = h0.shape[0]

        def step(t, nsplit=1):
            cols = slice(t * 128, (t + 1) * 128)
            w = pltpu.bitcast(cur[cur_slot, :, cols], bf16)
            cuts = [8 * ((nrow // 8 * i) // nsplit) for i in range(nsplit + 1)]
            head = None
            for r0, r1 in zip(cuts[:-1], cuts[1:]):
                y = jnp.dot(h0[r0:r1, :], w, preferred_element_type=f32)
                if r0 == 0:
                    head, y, r0 = y[0:LL], y[LL:], LL
                pre[g, r0 - LL:r1 - LL, cols] = y
            stage(gn, nxt, nxt_slot, (t + 6) % 9)
            return head

        kmat = blk(jnp.concatenate([step(t) for t in (3, 4, 5)], axis=1))
        p = softmax(sc_prev)
        q = jnp.concatenate([step(t) for t in (0, 1, 2)], axis=1)
        v01 = [step(6), step(7)]
        sc = scores(q, kmat)
        pv(gp, p, vm_prev)
        vm = blk(jnp.concatenate(v01 + [step(8, 4)], axis=1))
        return sc, vm

    w_wait(0)
    for t in range(9):
        stage(0, wq_even, 0, t)

    def first_body(i, carry):
        w_wait(2 * i + 1)
        carry = first_pair(2 * i, wq_even, i, wq_odd, i, *carry)

        @pl.when(2 * i + 2 < NP)
        def _():
            w_wait(2 * i + 2)
        return first_pair(2 * i + 1, wq_odd, i, wq_even, i + 1, *carry)
    sc_last, vm_last = jax.lax.fori_loop(
        0, NP // 2, first_body, (jnp.zeros((LL, 128), f32), jnp.zeros((128, PW), bf16)))
    p_last = softmax(sc_last)

    cp_b().wait()
    cp_bo().wait()
    for cpy in cp_wo():
        cpy.wait()
    a_finish(0, p_last, vm_last, True)
    b_weights()

    def short_body(tau, c):
        @pl.when(tau == 2)
        def _():
            cp_x().wait()
        x_init(tau + 1)
        x_init(jnp.where(tau == 1, 2, jnp.minimum(nlead + tau, nseg - 1)))
        tick(tau, True)
        return c
    jax.lax.fori_loop(1, nlead + 1, short_body, 0)

    un = UNROLL

    def body(it, c):
        tau = nlead + 1 + un * it
        for u in range(un):
            tick(tau + u, False)

        @pl.when(tau >= nseg + un)
        def _():
            out_copy(tau - nseg - un, un).start()
        return c
    jax.lax.fori_loop(0, (2 * nseg - nlead - 1) // un, body, 0)
    t0 = nlead + 1 + un * (-(-(nseg + un - nlead - 1) // un))
    if t0 - nseg - un > 0:
        head = pl.ds(0, (t0 - nseg - un) * SEG)
        pltpu.make_async_copy(outv.at[head, :], out_hbm.at[head, :], out_sem).start()
    out_copy(nseg - un, un - 1).start()
    for _ in b_steps(2 * nseg):
        pass
    out_copy(nseg - 1, 1).start()
    pltpu.make_async_copy(outv, out_hbm, out_sem).wait()


@functools.partial(jax.jit, static_argnames=("A_seg_len",))
def pallas_interleave_layers__memory_aug_recurrent_mem_tr__sliding_local_dilated__prompt_kernel(
    A_x, A_mem0, A_Wq, A_Wk, A_Wv, A_Wo, A_seg_len, B_x, B_wqkv, B_wo,
):
    del B_x
    B, S, Dm = A_x.shape
    nseg = S // SEG
    assert B == 1 and Dm == DM and A_seg_len == SEG and S == nseg * SEG and nseg & (nseg - 1) == 0
    assert A_mem0.shape == (1, MEM, DM) and A_Wq.shape == (DM, NH, DH) and A_Wo.shape == (NH, DH, DM)
    assert (2 * nseg - NLEAD - 1) % UNROLL == 0 and nseg - 1 <= 2 * NLEAD and 2 <= NLEAD < nseg
    x = A_x.reshape(nseg, SEG, DM)
    mem0 = A_mem0.reshape(MEM, DM)
    wt = lambda w: jnp.transpose(w, (1, 2, 0)).reshape(NH * DH, DM)
    any_spec = pl.BlockSpec(memory_space=pl.ANY)
    out = pl.pallas_call(
        functools.partial(_kernel, nseg=nseg, nlead=NLEAD),
        out_shape=jax.ShapeDtypeStruct((S, DM), A_x.dtype),
        in_specs=[any_spec] * 8,
        out_specs=any_spec,
        scratch_shapes=[
            pltpu.VMEM((nseg, SEG, DM), bf16),
            pltpu.VMEM((XPAD, 8, DM), bf16),
            pltpu.VMEM((MEM, DM), bf16),
            pltpu.VMEM((NP, 3, PW, DM), bf16),
            pltpu.VMEM((5, NH * DH, 128), bf16),
            pltpu.VMEM((DM, 3 * DM), bf16),
            pltpu.VMEM((DM, DM), bf16),
            pltpu.VMEM((3, 3 * DM, 128), u32),
            pltpu.VMEM((5, DM, 128), f32),
            pltpu.VMEM((NP // 2 + 1, DM // 2, 3 * PW), u32),
            pltpu.VMEM((NP // 2, DM // 2, 3 * PW), u32),
            pltpu.VMEM((5, NH * DH // 2, 128), u32),
            pltpu.VMEM((DM // 2, 3 * DM), u32),
            pltpu.VMEM((DM // 2, DM), u32),
            pltpu.VMEM((S, DM), f32),
            pltpu.VMEM((MEM, DM), f32),
            pltpu.VMEM((MEM, DM), f32),
            pltpu.VMEM((SEG, DM), f32),
            pltpu.VMEM((LL + 8 * NLEAD, DM), f32),
            pltpu.VMEM((NP, 8 * NLEAD, 3 * PW), f32),
            pltpu.VMEM((NP, LL, PW), f32),
            pltpu.VMEM((5, 16 + SEG, 128), f32),
            pltpu.VMEM((5, 16 + SEG, 128), f32),
            pltpu.VMEM((SEG, DM), f32),
            pltpu.VMEM((SEG, DM), f32),
            pltpu.VMEM((S, DM), bf16),
            pltpu.SemaphoreType.DMA((11 + NP,)),
            pltpu.SemaphoreType.DMA(()),
        ],
        compiler_params=pltpu.CompilerParams(
            vmem_limit_bytes=124 * 1024 * 1024,
            flags={"XLA_TPU_FORCE_LP_LLO_SCHEDULER": True}),
    )(x, mem0, wt(A_Wq), wt(A_Wk), wt(A_Wv), A_Wo.reshape(NH * DH, DM), B_wqkv, B_wo)
    return out.reshape(B, S, DM)
```
